```python
import jax
import jax.numpy as jnp

def _softmax(x, axis=-1):
    return jax.nn.softmax(x, axis=axis)

def _gelu(x):
    return jax.nn.gelu(x, approximate=True)

def _silu(x):
    return jax.nn.silu(x)

def _sigmoid(x):
    return jax.nn.sigmoid(x)

def _layernorm(x, axis=-1, eps=1e-05):
    m = jnp.mean(x, axis=axis, keepdims=True)
    v = jnp.var(x, axis=axis, keepdims=True)
    return (x - m) / jnp.sqrt(v + eps)

def _scatter_add(tgt, idx, src, axis=0):
    return tgt.at[idx].add(src)

def _segment_sum(src, seg, n):
    return jax.ops.segment_sum(src, seg, n)

class _Rng:

    def __init__(self, key):
        self._k = key

    def _next(self):
        self._k, sub = jax.random.split(self._k)
        return sub

    def normal(self, shape):
        return jax.random.normal(self._next(), shape, dtype=jnp.bfloat16)

    def randint(self, lo, hi, shape):
        return jax.random.randint(self._next(), shape, lo, hi, dtype=jnp.int32)

    def uniform(self, shape, lo=0.0, hi=1.0):
        return jax.random.uniform(self._next(), shape, jnp.bfloat16, lo, hi)

    def permutation(self, n):
        return jax.random.permutation(self._next(), n)
kernel_name = 'interleave_layers__memory_aug_recurrent_mem_tr__sliding_local_dilated__prompt'

def setup_inputs():
    _rng = _Rng(jax.random.key(int.from_bytes(__import__("os").urandom(4), "little")))
    _w = lambda a: (lambda t: t.astype(jnp.bfloat16) if jnp.issubdtype(t.dtype, jnp.floating) else t)(jnp.asarray(a))

    def _A_setup():
        B, S, Dm = (1, 2048, 640)
        H, Dh = (32, 192)
        M, seg = (8, 32)
        seg = min(seg, S)
        S = S // seg * seg
        return {'x': _w((lambda *s: _rng.normal(s) * 0.05)(B, S, Dm)), 'mem0': _w((lambda *s: _rng.normal(s) * 0.05)(B, M, Dm)), 'Wq': _w((lambda *s: _rng.normal(s) * 0.05)(Dm, H, Dh) * Dm ** (-0.5)), 'Wk': _w((lambda *s: _rng.normal(s) * 0.05)(Dm, H, Dh) * Dm ** (-0.5)), 'Wv': _w((lambda *s: _rng.normal(s) * 0.05)(Dm, H, Dh) * Dm ** (-0.5)), 'Wo': _w((lambda *s: _rng.normal(s) * 0.05)(H, Dh, Dm) * (H * Dh) ** (-0.5)), 'seg_len': seg}
    _A_in = _A_setup()

    def _B_setup():
        B, S, D = (1, 2048, 640)
        return {'x': _w((lambda *s: _rng.normal(s) * 0.05)(B, S, D)), 'wqkv': _w((lambda *s: _rng.normal(s) * 0.05)(D, 3 * D)), 'wo': _w((lambda *s: _rng.normal(s) * 0.05)(D, D))}
    _B_in = _B_setup()
    return {'A_x': _A_in['x'], 'A_mem0': _A_in['mem0'], 'A_Wq': _A_in['Wq'], 'A_Wk': _A_in['Wk'], 'A_Wv': _A_in['Wv'], 'A_Wo': _A_in['Wo'], 'A_seg_len': _A_in['seg_len'], 'B_x': _B_in['x'], 'B_wqkv': _B_in['wqkv'], 'B_wo': _B_in['wo']}

def reference(A_x, A_mem0, A_Wq, A_Wk, A_Wv, A_Wo, A_seg_len, B_x, B_wqkv, B_wo):

    def _A_ref(x, mem0, Wq, Wk, Wv, Wo, seg_len):
        B, S, Dm = x.shape
        H, Dh = (Wq.shape[1], Wq.shape[2])
        M = mem0.shape[1]
        scale = Dh ** (-0.5)
        n_seg = S // seg_len
        L = M + seg_len
        idx = jnp.arange(L)
        mask = (idx[:, None] < M) | (idx[:, None] >= idx[None, :])
        mem = mem0
        outs = []
        for s in range(n_seg):
            xs = x[:, s * seg_len:(s + 1) * seg_len, :].copy()
            h = jnp.concatenate([mem, xs], axis=1)
            q = jnp.einsum('btd,dhe->bhte', h, Wq)
            k = jnp.einsum('btd,dhe->bhte', h, Wk)
            v = jnp.einsum('btd,dhe->bhte', h, Wv)
            scores = jnp.einsum('bhqe,bhke->bhqk', q, k) * scale
            scores = jnp.where(mask[None, None], scores, -1000000000.0)
            p = _softmax(scores, axis=-1)
            o = jnp.einsum('bhqk,bhke->bhqe', p, v)
            o = jnp.einsum('bhte,hed->btd', o, Wo)
            mem = o[:, :M, :].copy()
            outs.append(o[:, M:, :])
        return jnp.concatenate(outs, axis=1)

    def _B_ref(x, wqkv, wo):
        B, S, D = x.shape
        H = 32
        Dh = D // H
        W, dil = (8, 2)
        qkv = (lambda x, *d: x.transpose(*d))((x @ wqkv).reshape(B, S, 3, H, Dh), 2, 0, 3, 1, 4)
        q, k, v = (qkv[0], qkv[1], qkv[2])
        scale = Dh ** (-0.5)
        pos = jnp.arange(S)
        off = jnp.arange(W) * dil
        idx = pos[:, None] - off[None, :]
        mask = idx >= 0
        idx_c = jnp.where(mask, idx, 0).reshape(-1)
        kg = k[:, :, idx_c, :].reshape(B, H, S, W, Dh)
        vg = v[:, :, idx_c, :].reshape(B, H, S, W, Dh)
        logits = jnp.einsum('bhsd,bhswd->bhsw', q, kg) * scale
        logits = jnp.where(mask[None, None, :, :], logits, -1000000000.0)
        attn = _softmax(logits, axis=-1)
        o = jnp.einsum('bhsw,bhswd->bhsd', attn, vg)
        return (lambda x, *d: x.transpose(*d))(o, 0, 2, 1, 3).reshape(B, S, D) @ wo
    x = A_x
    x = x + _A_ref(_layernorm(x, axis=-1), A_mem0, A_Wq, A_Wk, A_Wv, A_Wo, A_seg_len)
    x = x + _B_ref(_layernorm(x, axis=-1), B_wqkv, B_wo)
    x = x + _A_ref(_layernorm(x, axis=-1), A_mem0, A_Wq, A_Wk, A_Wv, A_Wo, A_seg_len)
    x = x + _B_ref(_layernorm(x, axis=-1), B_wqkv, B_wo)
    return x
```

```python
import functools
import jax
import jax.numpy as jnp
import numpy as np
from jax.experimental import pallas as pl
from jax.experimental.pallas import tpu as pltpu

S = 2048; D = 640; H = 32; DH = 192; M = 8; SEG = 32; NSEG = S // SEG
NPAIR = H // 2; PW = 2 * DH
BH = 32; BDH = D // BH; BW = 8; BDIL = 2
LOG2E = 1.4426950408889634
NEG = -1e30
f32 = jnp.float32; bf16 = jnp.bfloat16

def _dot(a, b):
    return jnp.dot(a, b, preferred_element_type=f32)
def _dot_nt(a, b):
    return lax_dot(a, b, (((1,), (1,)), ((), ())))
def lax_dot(a, b, dn):
    return jax.lax.dot_general(a, b, dn, preferred_element_type=f32)

def _recip(x):
    r = pl.reciprocal(x, approx=True)
    return r * (2.0 - x * r)

def _ln(x):
    m = jnp.mean(x, axis=-1, keepdims=True)
    xc = x - m
    v = jnp.mean(xc * xc, axis=-1, keepdims=True)
    return xc * jax.lax.rsqrt(v + 1e-5)

def _perm_mat():
    r = jax.lax.broadcasted_iota(jnp.int32, (D, D), 0)
    c = jax.lax.broadcasted_iota(jnp.int32, (D, D), 1)
    h = c % BH
    d = c // BH
    return (r == h * BDH + d).astype(bf16)

def kernel(x_ref, mem0_ref, wq_hbm, wk_hbm, wv_hbm, wo_hbm, bqkv_ref, bwo_ref, out_ref,
           wq, wk, wv, wo, bqkv_p, bwo_p, h_ref, qkv_ref, o_ref, xa_ref, xb_ref, kb_ref, vb_ref, sems):
    cps = [pltpu.make_async_copy(s, d, sems.at[i]) for i, (s, d) in enumerate(
        [(wq_hbm, wq), (wk_hbm, wk), (wv_hbm, wv), (wo_hbm, wo)])]
    for c in cps: c.start()

    pm = _perm_mat()
    for j in range(3):
        bqkv_p[:, j * D:(j + 1) * D] = _dot(bqkv_ref[:, j * D:(j + 1) * D], pm).astype(bf16)
    bwo_p[...] = lax_dot(pm, bwo_ref[...], (((0,), (0,)), ((), ()))).astype(bf16)

    mem0 = mem0_ref[...]
    mem00 = jnp.concatenate([mem0.astype(f32), mem0.astype(f32)], axis=0)
    h_ref[0, 0:16, :] = mem00.astype(bf16)
    x00 = x_ref[0:SEG, :].astype(f32)
    h_ref[0, 16:48, :] = _ln(x00).astype(bf16)
    h_ref[0, 48:80, :] = jnp.zeros((SEG, D), bf16)
    xa_ref[0:SEG, :] = x00
    xa_ref[SEG:2 * SEG, :] = jnp.zeros((SEG, D), f32)
    xb_ref[...] = jnp.zeros((2 * SEG, D), f32)
    kb_ref[...] = jnp.zeros(kb_ref.shape, f32)
    vb_ref[...] = jnp.zeros(vb_ref.shape, f32)
    for c in cps: c.wait()

    lane = jax.lax.broadcasted_iota(jnp.int32, (48, 128), 1)
    lo64 = lane < 64
    rr = jax.lax.broadcasted_iota(jnp.int32, (48, 96), 0)
    cc = jax.lax.broadcasted_iota(jnp.int32, (48, 96), 1)
    ck = jnp.where(cc >= 48, cc - 48, cc)
    first = cc < 48
    def smask(l):
        memk = (ck >= 8 * l) & (ck < 8 * l + 8)
        tokk = (ck >= 16) & ((rr < 16) | (ck <= rr))
        return memk | tokk
    masks = [smask(0), smask(1)]
    row16 = jax.lax.broadcasted_iota(jnp.int32, (16, PW), 0)
    sc = (DH ** -0.5) * LOG2E
    ws = (wq, wk, wv)

    def bd(a):
        z = jnp.zeros((48, 128), bf16)
        a0, a1, a2 = a[:, 0:128], a[:, 128:256], a[:, 256:384]
        top = jnp.concatenate([a0, jnp.where(lo64, a1, z), z], axis=1)
        bot = jnp.concatenate([z, jnp.where(lo64, z, a1), a2], axis=1)
        return jnp.concatenate([top, bot], axis=0)

    def proj(hs, g, j):
        qkv_ref[j, :, g * PW:(g + 1) * PW] = _dot_nt(h_ref[hs], ws[j][g * PW:(g + 1) * PW, :]).astype(bf16)
    def rows(j, g, l):
        return jnp.concatenate([qkv_ref[j, 0:16, g * PW:(g + 1) * PW],
                                qkv_ref[j, 16 + 32 * l:48 + 32 * l, g * PW:(g + 1) * PW]], axis=0)
    def qk(g, l):
        return _dot_nt(rows(0, g, l), bd(rows(1, g, l)))
    def sm(s, l):
        s = jnp.where(masks[l], s * sc, NEG)
        m0 = jnp.max(jnp.where(first, s, NEG), axis=1, keepdims=True)
        m1 = jnp.max(jnp.where(first, NEG, s), axis=1, keepdims=True)
        p = jnp.exp2(s - jnp.where(first, m0, m1))
        s0 = jnp.sum(jnp.where(first, p, 0.0), axis=1, keepdims=True)
        s1 = jnp.sum(jnp.where(first, 0.0, p), axis=1, keepdims=True)
        p = p * _recip(jnp.where(first, s0, s1))
        return p.astype(bf16)
    def pv(g, ps):
        os_ = [_dot(ps[l], bd(rows(2, g, l))) for l in range(2)]
        om = jnp.where(row16 < 8, os_[0][0:16], os_[1][0:16])
        o = jnp.concatenate([om, os_[0][16:48], os_[1][16:48]], axis=0)
        o_ref[:, g * PW:(g + 1) * PW] = o.astype(bf16)

    r8 = jax.lax.broadcasted_iota(jnp.int32, (2 * SEG, 128), 0)
    bsc = (BDH ** -0.5) * LOG2E

    def b_qkv():
        xb = xb_ref[...]
        return _dot(_ln(xb).astype(bf16), bqkv_p[...])
    def b_attn(t, y):
        q = y[:, 0:D]
        for l in range(2):
            kb_ref[l, 16:48, :] = y[32 * l:32 * l + 32, D:2 * D]
            vb_ref[l, 16:48, :] = y[32 * l:32 * l + 32, 2 * D:3 * D]
        seg = jnp.where(r8 < SEG, t - 1, t - 3)
        pos = seg * SEG + jnp.where(r8 < SEG, r8, r8 - SEG)
        lg = []
        for w in range(BW):
            off = 16 - BDIL * w
            ks = jnp.concatenate([kb_ref[0, off:off + 32, :], kb_ref[1, off:off + 32, :]], axis=0)
            pr = q * ks
            a = pr[:, 0:128] + pr[:, 128:256] + pr[:, 256:384] + pr[:, 384:512] + pr[:, 512:640]
            a = a + pltpu.roll(a, 64, 1)
            a = a + pltpu.roll(a, 32, 1)
            a = a * bsc
            if w > 0:
                a = jnp.where(pos >= BDIL * w, a, NEG)
            lg.append(a)
        m = lg[0]
        for w in range(1, BW): m = jnp.maximum(m, lg[w])
        ps = [jnp.exp2(a - m) for a in lg]
        den = ps[0]
        for w in range(1, BW): den = den + ps[w]
        inv = _recip(den)
        acc = None
        for w in range(BW):
            off = 16 - BDIL * w
            vs = jnp.concatenate([vb_ref[0, off:off + 32, :], vb_ref[1, off:off + 32, :]], axis=0)
            pw = ps[w] * inv
            pw5 = jnp.concatenate([pw] * 5, axis=1)
            acc = pw5 * vs if acc is None else acc + pw5 * vs
        for l in range(2):
            kb_ref[l, 0:16, :] = kb_ref[l, 32:48, :]
            vb_ref[l, 0:16, :] = vb_ref[l, 32:48, :]
        return acc.astype(bf16)
    def b_out(acc):
        return xb_ref[...] + _dot(acc, bwo_p[...])

    def step(t, c):
        hs = t % 2
        st = {}
        ss = {}; pp = {}
        for i in range(-2, NPAIR):
            g2, g1, g0 = i + 2, i + 1, i
            if g2 < NPAIR: proj(hs, g2, 0)
            if 0 <= g1 < NPAIR: ss[(g1, 0)] = qk(g1, 0)
            if g2 < NPAIR: proj(hs, g2, 1)
            if 0 <= g1 < NPAIR: ss[(g1, 1)] = qk(g1, 1)
            if g2 < NPAIR: proj(hs, g2, 2)
            if 0 <= g1 < NPAIR:
                pp[g1] = [sm(ss.pop((g1, 0)), 0), sm(ss.pop((g1, 1)), 1)]
            if i == 0:
                st['y'] = b_qkv()
            if i == 3:
                st['acc'] = b_attn(t, st['y'])
            if i == 8:
                xo = b_out(st['acc'])
                out_ref[pl.ds(pl.multiple_of(jnp.maximum(t - 3, 0) * SEG, SEG), SEG), :] = xo[SEG:].astype(bf16)
                xn = x_ref[pl.ds(pl.multiple_of(jnp.minimum(t + 1, NSEG - 1) * SEG, SEG), SEG), :].astype(f32)
                xan = jnp.concatenate([xn, xo[:SEG]], axis=0)
                h_ref[1 - hs, 16:80, :] = _ln(xan).astype(bf16)
                st['xan'] = xan
            if 0 <= g0: pv(g0, pp.pop(g0))
        oa = _dot(o_ref[...], wo[...])
        xb_ref[...] = xa_ref[...] + oa[16:80]
        xa_ref[...] = st['xan']
        r16 = jax.lax.broadcasted_iota(jnp.int32, (16, D), 0)
        memn = jnp.where((r16 >= 8) & (t < 2), mem00, oa[0:16])
        h_ref[1 - hs, 0:16, :] = memn.astype(bf16)
        return c

    jax.lax.fori_loop(0, NSEG + 2, step, 0)
    xo = b_out(b_attn(NSEG + 2, b_qkv()))
    out_ref[S - SEG:S, :] = xo[SEG:].astype(bf16)

@functools.partial(jax.jit, static_argnames=("A_seg_len",))
def pallas_interleave_layers__memory_aug_recurrent_mem_tr__sliding_local_dilated__prompt_kernel(
        A_x, A_mem0, A_Wq, A_Wk, A_Wv, A_Wo, A_seg_len, B_x, B_wqkv, B_wo):
    assert A_seg_len == SEG
    x = A_x.reshape(S, D)
    mem0 = A_mem0.reshape(M, D)
    tr = lambda w: jnp.transpose(w, (1, 2, 0)).reshape(H * DH, D)
    wo = A_Wo.reshape(H * DH, D)
    vm = pl.BlockSpec(memory_space=pltpu.VMEM)
    hbm = pl.BlockSpec(memory_space=pl.ANY)
    out = pl.pallas_call(
        kernel,
        out_shape=jax.ShapeDtypeStruct((S, D), bf16),
        in_specs=[vm, vm, hbm, hbm, hbm, hbm, vm, vm],
        out_specs=vm,
        scratch_shapes=[
            pltpu.VMEM((H * DH, D), bf16), pltpu.VMEM((H * DH, D), bf16), pltpu.VMEM((H * DH, D), bf16), pltpu.VMEM((H * DH, D), bf16),
            pltpu.VMEM((D, 3 * D), bf16), pltpu.VMEM((D, D), bf16),
            pltpu.VMEM((2, 80, D), bf16), pltpu.VMEM((3, 80, H * DH), bf16), pltpu.VMEM((80, H * DH), bf16),
            pltpu.VMEM((64, D), f32), pltpu.VMEM((64, D), f32),
            pltpu.VMEM((2, 48, D), f32), pltpu.VMEM((2, 48, D), f32),
            pltpu.SemaphoreType.DMA((4,)),
        ],
        compiler_params=pltpu.CompilerParams(vmem_limit_bytes=100 * 1024 * 1024),
    )(x, mem0, tr(A_Wq), tr(A_Wk), tr(A_Wv), wo, B_wqkv, B_wo)
    return out.reshape(1, S, D)
```

```python
import functools
import jax
import jax.numpy as jnp
import numpy as np
from jax.experimental import pallas as pl
from jax.experimental.pallas import tpu as pltpu

S = 2048; D = 640; H = 32; DH = 192; M = 8; SEG = 32; NSEG = S // SEG
NPAIR = H // 2; PW = 2 * DH
BH = 32; BDH = D // BH; BW = 8; BDIL = 2
LOG2E = 1.4426950408889634
NEG = -1e30
f32 = jnp.float32; bf16 = jnp.bfloat16; u32 = jnp.uint32

SCHED = {
    (0, 'post'): ['bqkv'],
    (2, 'post'): [('battn', 0, 0)],
    (3, 'post'): [('battn', 0, 1)],
    (4, 'post'): [('battn', 1, 0)],
    (5, 'post'): [('battn', 1, 1), 'bhist'],
    (7, 'post'): ['b1fin'],
    (13, 'post'): ['hcopy', ('wo', 0, 5)],
    (14, 'k'): [('wo', 5, 10)],
    (14, 'post'): [('wo', 10, 14)],
    (15, 'post'): [('wo', 14, 16), 'b2fin'],
}
ORDER = 'B'

def _dot(a, b):
    return jnp.dot(a, b, preferred_element_type=f32)
def _dot_nt(a, b):
    return lax_dot(a, b, (((1,), (1,)), ((), ())))
def lax_dot(a, b, dn):
    return jax.lax.dot_general(a, b, dn, preferred_element_type=f32)

def _recip(x):
    r = pl.reciprocal(x, approx=True)
    return r * (2.0 - x * r)

def _ln(x):
    m = jnp.mean(x, axis=-1, keepdims=True)
    xc = x - m
    v = jnp.mean(xc * xc, axis=-1, keepdims=True)
    return xc * jax.lax.rsqrt(v + 1e-5)

def _perm_mat():
    r = jax.lax.broadcasted_iota(jnp.int32, (D, D), 0)
    c = jax.lax.broadcasted_iota(jnp.int32, (D, D), 1)
    h = c % BH
    d = c // BH
    return (r == h * BDH + d).astype(bf16)

def _pk(x):
    return pltpu.bitcast(x.astype(bf16), u32)
def _up(x):
    return pltpu.bitcast(x, bf16)

def kernel(nsteps, x_hbm, mem0_hbm, wq_hbm, wk_hbm, wv_hbm, wo_hbm, bqkv_hbm, bwo_hbm, out_hbm,
           wq, wk, wv, wo, bqkv_raw, bwo_raw, bqkv_p, bwo_p, x_ref, mem0_ref, out_ref,
           h_ref, qkv_ref, o_ref, xa_ref, xb_ref, kb_ref, vb_ref, xan_ref, bq_ref, bo_ref, hn_ref,
           sem_w, sem_m, sem_o):
    RW = PW // 2
    ws = (wq, wk, wv)
    ws_hbm = (wq_hbm.bitcast(u32), wk_hbm.bitcast(u32), wv_hbm.bitcast(u32))
    NWO = 4
    RO = H * DH // 2 // NWO
    def cp_w(j, g):
        sl = pl.ds(pl.multiple_of(g * RW, RW), RW) if not isinstance(g, int) else pl.ds(g * RW, RW)
        return pltpu.make_async_copy(ws_hbm[j].at[sl], ws[j].at[sl], sem_w.at[g])
    cp_x0 = pltpu.make_async_copy(x_hbm.at[0:2 * SEG], x_ref.at[0:2 * SEG], sem_m.at[0])
    cp_mem = pltpu.make_async_copy(mem0_hbm, mem0_ref, sem_m.at[1])
    cp_bqkv = pltpu.make_async_copy(bqkv_hbm, bqkv_raw, sem_m.at[2])
    cp_bwo = pltpu.make_async_copy(bwo_hbm, bwo_raw, sem_m.at[3])
    cp_wo = [pltpu.make_async_copy(wo_hbm.bitcast(u32).at[i * RO:(i + 1) * RO], wo.at[i * RO:(i + 1) * RO], sem_m.at[4 + i])
             for i in range(NWO)]
    cp_x1 = pltpu.make_async_copy(x_hbm.at[2 * SEG:S], x_ref.at[2 * SEG:S], sem_m.at[4 + NWO])
    def cp_out(s):
        sl = pl.ds(pl.multiple_of(s * SEG, SEG), SEG) if not isinstance(s, int) else pl.ds(s * SEG, SEG)
        return pltpu.make_async_copy(out_ref.at[sl], out_hbm.at[sl], sem_o.at[0])

    cp_x0.start(); cp_mem.start(); cp_bqkv.start(); cp_bwo.start()
    for g in range(NPAIR):
        for j in range(3): cp_w(j, g).start()
    for c in cp_wo: c.start()
    cp_x1.start()

    xb_ref[...] = jnp.zeros((2 * SEG, D), f32)
    kb_ref[...] = jnp.zeros(kb_ref.shape, f32)
    vb_ref[...] = jnp.zeros(vb_ref.shape, f32)
    xa_ref[SEG:2 * SEG, :] = jnp.zeros((SEG, D), f32)
    h_ref[24:40, :] = jnp.zeros((16, D), u32)
    cp_x0.wait(); cp_mem.wait()
    mem0 = mem0_ref[...]
    mem00 = jnp.concatenate([mem0.astype(f32), mem0.astype(f32)], axis=0)
    h_ref[0:8, :] = _pk(mem00)
    x00 = x_ref[0:SEG, :].astype(f32)
    h_ref[8:24, :] = _pk(_ln(x00))
    xa_ref[0:SEG, :] = x00

    pm = _perm_mat()
    cp_bqkv.wait()
    for j in range(3):
        bqkv_p[:, j * D:(j + 1) * D] = _pk(_dot(bqkv_raw[:, j * D:(j + 1) * D], pm))
    cp_bwo.wait()
    bwo_p[...] = _pk(lax_dot(pm, bwo_raw[...], (((0,), (0,)), ((), ()))))

    lane = jax.lax.broadcasted_iota(jnp.int32, (48, 128), 1)
    lo64 = lane < 64
    rr = jax.lax.broadcasted_iota(jnp.int32, (48, 96), 0)
    cc = jax.lax.broadcasted_iota(jnp.int32, (48, 96), 1)
    ck = jnp.where(cc >= 48, cc - 48, cc)
    first = cc < 48
    def smask(l):
        memk = (ck >= 8 * l) & (ck < 8 * l + 8)
        tokk = (ck >= 16) & ((rr < 16) | (ck <= rr))
        return jnp.where(memk | tokk, 0.0, NEG).astype(f32)
    bias = [smask(0), smask(1)]
    row16 = jax.lax.broadcasted_iota(jnp.int32, (16, PW), 0)
    sc = (DH ** -0.5) * LOG2E

    def bd(a):
        z = jnp.zeros((48, 128), bf16)
        a0, a1, a2 = a[:, 0:128], a[:, 128:256], a[:, 256:384]
        top = jnp.concatenate([a0, jnp.where(lo64, a1, z), z], axis=1)
        bot = jnp.concatenate([z, jnp.where(lo64, z, a1), a2], axis=1)
        return jnp.concatenate([top, bot], axis=0)

    def proj(g, j):
        sl = pl.ds(pl.multiple_of(g * RW, RW), RW) if not isinstance(g, int) else pl.ds(g * RW, RW)
        qkv_ref[g, j] = _pk(_dot_nt(_up(h_ref[...]), _up(ws[j][sl, :])))
    def rows(j, g, l):
        return jnp.concatenate([_up(qkv_ref[g, j, 0:8, :]), _up(qkv_ref[g, j, 8 + 16 * l:24 + 16 * l, :])], axis=0)
    def qk(g, l):
        return _dot_nt(rows(0, g, l), bd(rows(1, g, l)))
    def sm(s, l):
        s = s * sc + bias[l]
        m0 = jnp.max(jnp.where(first, s, NEG), axis=1, keepdims=True)
        m1 = jnp.max(jnp.where(first, NEG, s), axis=1, keepdims=True)
        p = jnp.exp2(s - jnp.where(first, m0, m1))
        s0 = jnp.sum(jnp.where(first, p, 0.0), axis=1, keepdims=True)
        s1 = jnp.sum(jnp.where(first, 0.0, p), axis=1, keepdims=True)
        p = p * _recip(jnp.where(first, s0, s1))
        return p.astype(bf16)
    def pv(g, ps):
        os_ = [_dot(ps[l], bd(rows(2, g, l))) for l in range(2)]
        om = jnp.where(row16 < 8, os_[0][0:16], os_[1][0:16])
        o = jnp.concatenate([om, os_[0][16:48], os_[1][16:48]], axis=0)
        o_ref[g] = _pk(o)

    rC = jax.lax.broadcasted_iota(jnp.int32, (16, 128), 0)
    bsc = (BDH ** -0.5) * LOG2E

    def b_qkv():
        y = _dot(_ln(xb_ref[...]).astype(bf16), _up(bqkv_p[...]))
        bq_ref[...] = y[:, 0:D]
        for l in range(2):
            kb_ref[l, 16:48, :] = y[32 * l:32 * l + 32, D:2 * D]
            vb_ref[l, 16:48, :] = y[32 * l:32 * l + 32, 2 * D:3 * D]
    def b_attn(t, l, c):
        r0 = 16 * c
        q = bq_ref[32 * l + r0:32 * l + r0 + 16, :]
        seg = t - 1 - 2 * l
        pos = seg * SEG + r0 + rC
        lg = []
        for w in range(BW):
            off = 16 - BDIL * w + r0
            pr = q * kb_ref[l, off:off + 16, :]
            a = pr[:, 0:128] + pr[:, 128:256] + pr[:, 256:384] + pr[:, 384:512] + pr[:, 512:640]
            a = a + pltpu.roll(a, 64, 1)
            a = a + pltpu.roll(a, 32, 1)
            a = a * bsc
            if w > 0:
                a = jnp.where(pos >= BDIL * w, a, NEG)
            lg.append(a)
        m = lg[0]
        for w in range(1, BW): m = jnp.maximum(m, lg[w])
        ps = [jnp.exp2(a - m) for a in lg]
        den = ps[0]
        for w in range(1, BW): den = den + ps[w]
        inv = _recip(den)
        acc = None
        for w in range(BW):
            off = 16 - BDIL * w + r0
            pw = ps[w] * inv
            pw5 = jnp.concatenate([pw] * 5, axis=1)
            tt = pw5 * vb_ref[l, off:off + 16, :]
            acc = tt if acc is None else acc + tt
        bo_ref[16 * l + r0 // 2:16 * l + r0 // 2 + 8, :] = _pk(acc)
    def b_hist():
        for l in range(2):
            kb_ref[l, 0:16, :] = kb_ref[l, 32:48, :]
            vb_ref[l, 0:16, :] = vb_ref[l, 32:48, :]
    def b_out(l):
        return xb_ref[32 * l:32 * l + 32, :] + _dot(_up(bo_ref[16 * l:16 * l + 16, :]), _up(bwo_p[...]))
    def b1_finish(t):
        x2 = b_out(0)
        xn = x_ref[pl.ds(pl.multiple_of(jnp.minimum(t + 1, NSEG - 1) * SEG, SEG), SEG), :].astype(f32)
        xan_ref[0:SEG, :] = xn
        xan_ref[SEG:2 * SEG, :] = x2
        hn_ref[0:16, :] = _pk(_ln(xn))
        hn_ref[16:32, :] = _pk(_ln(x2))
    def b2_finish(t):
        x4 = b_out(1)
        out_ref[pl.ds(pl.multiple_of(jnp.maximum(t - 3, 0) * SEG, SEG), SEG), :] = x4.astype(bf16)
    def wo_part(g0, g1):
        o = jnp.concatenate([_up(o_ref[g]) for g in range(g0, g1)], axis=1)
        return _dot(o, _up(wo[g0 * PW // 2:g1 * PW // 2, :]))

    def step(t, c):
        st = {}
        ss = {}; pp = {}
        def ex(i, pos):
            for name in SCHED.get((i, pos), ()): run_extra(name, t, st)
        for i in range(-2, NPAIR):
            g2, g1, g0 = i + 2, i + 1, i
            ex(i, 'pre')
            if ORDER == 'A':
                if g2 < NPAIR: proj(g2, 0)
                ex(i, 'q')
                if 0 <= g1 < NPAIR: ss[(g1, 0)] = qk(g1, 0)
                if g2 < NPAIR: proj(g2, 1)
                ex(i, 'k')
                if 0 <= g1 < NPAIR: ss[(g1, 1)] = qk(g1, 1)
                if g2 < NPAIR: proj(g2, 2)
                ex(i, 'v')
            else:
                if g2 < NPAIR: proj(g2, 0)
                ex(i, 'q')
                if g2 < NPAIR: proj(g2, 1)
                ex(i, 'k')
                if g2 < NPAIR: proj(g2, 2)
                ex(i, 'v')
                if 0 <= g1 < NPAIR:
                    ss[(g1, 0)] = qk(g1, 0); ss[(g1, 1)] = qk(g1, 1)
            if 0 <= g1 < NPAIR:
                pp[g1] = [sm(ss.pop((g1, 0)), 0), sm(ss.pop((g1, 1)), 1)]
            if 0 <= g0: pv(g0, pp.pop(g0))
            ex(i, 'post')
        end_step(t, st['oa'])
        @pl.when(t >= 3)
        def _():
            cp_out(jnp.maximum(t - 3, 0)).start()
        return c

    def end_step(t, oa):
        xb_ref[...] = xa_ref[...] + oa[16:80]
        xa_ref[...] = xan_ref[...]
        r16 = jax.lax.broadcasted_iota(jnp.int32, (16, D), 0)
        memn = jnp.where((r16 >= 8) & (t < 2), mem00, oa[0:16])
        h_ref[0:8, :] = _pk(memn)

    def run_extra(name, t, st):
        if name == 'bqkv': b_qkv()
        elif name[0] == 'battn': b_attn(t, name[1], name[2])
        elif name == 'bhist': b_hist()
        elif name == 'hcopy': h_ref[8:40, :] = hn_ref[...]
        elif name == 'b1fin': b1_finish(t)
        elif name == 'b2fin': b2_finish(t)
        elif name[0] == 'wo':
            part = wo_part(name[1], name[2])
            st['oa'] = part if 'oa' not in st else st['oa'] + part
        else: raise ValueError(name)

    def pair0(g, c):
        for j in range(3): cp_w(j, g).wait()
        for j in range(3): proj(g, j)
        pv(g, [sm(qk(g, l), l) for l in range(2)])
        return c
    jax.lax.fori_loop(0, NPAIR, pair0, 0)
    oa = None
    for i in range(NWO):
        cp_wo[i].wait()
        part = wo_part(i * NPAIR // NWO, (i + 1) * NPAIR // NWO)
        oa = part if oa is None else oa + part
    xn = x_ref[SEG:2 * SEG, :].astype(f32)
    xan_ref[0:SEG, :] = xn
    xan_ref[SEG:2 * SEG, :] = jnp.zeros((SEG, D), f32)
    h_ref[8:24, :] = _pk(_ln(xn))
    end_step(0, oa)
    cp_x1.wait()

    jax.lax.fori_loop(1, nsteps, step, 0)
    b_qkv()
    for c_ in range(2): b_attn(NSEG + 2, 1, c_)
    b2_finish(NSEG + 2)
    cp_out(NSEG - 1).start()
    def wait_out(s, c):
        cp_out(s).wait()
        return c
    jax.lax.fori_loop(0, min(nsteps - 3, NSEG - 1) + 1 if nsteps > 3 else 1, wait_out, 0)

@functools.partial(jax.jit, static_argnames=("A_seg_len",))
def pallas_interleave_layers__memory_aug_recurrent_mem_tr__sliding_local_dilated__prompt_kernel(
        A_x, A_mem0, A_Wq, A_Wk, A_Wv, A_Wo, A_seg_len, B_x, B_wqkv, B_wo):
    assert A_seg_len == SEG
    del B_x
    nsteps = NSEG + 2
    x = A_x.reshape(S, D)
    mem0 = A_mem0.reshape(M, D)
    tr = lambda w: jnp.transpose(w, (1, 2, 0)).reshape(H * DH, D)
    wo = A_Wo.reshape(H * DH, D)
    hbm = pl.BlockSpec(memory_space=pl.ANY)
    out = pl.pallas_call(
        functools.partial(kernel, nsteps),
        out_shape=jax.ShapeDtypeStruct((S, D), bf16),
        in_specs=[hbm] * 8,
        out_specs=hbm,
        scratch_shapes=[
            pltpu.VMEM((H * DH // 2, D), u32), pltpu.VMEM((H * DH // 2, D), u32), pltpu.VMEM((H * DH // 2, D), u32), pltpu.VMEM((H * DH // 2, D), u32),
            pltpu.VMEM((D, 3 * D), bf16), pltpu.VMEM((D, D), bf16),
            pltpu.VMEM((D // 2, 3 * D), u32), pltpu.VMEM((D // 2, D), u32),
            pltpu.VMEM((S, D), bf16), pltpu.VMEM((M, D), bf16), pltpu.VMEM((S, D), bf16),
            pltpu.VMEM((40, D), u32), pltpu.VMEM((NPAIR, 3, 40, PW), u32), pltpu.VMEM((NPAIR, 40, PW), u32),
            pltpu.VMEM((64, D), f32), pltpu.VMEM((64, D), f32),
            pltpu.VMEM((2, 48, D), f32), pltpu.VMEM((2, 48, D), f32),
            pltpu.VMEM((64, D), f32), pltpu.VMEM((64, D), f32), pltpu.VMEM((32, D), u32),
            pltpu.VMEM((32, D), u32),
            pltpu.SemaphoreType.DMA((NPAIR,)), pltpu.SemaphoreType.DMA((9,)), pltpu.SemaphoreType.DMA((1,)),
        ],
        compiler_params=pltpu.CompilerParams(vmem_limit_bytes=100 * 1024 * 1024),
    )(x, mem0, tr(A_Wq), tr(A_Wk), tr(A_Wv), wo, B_wqkv, B_wo)
    return out.reshape(1, S, D)
```

```python
import functools
import jax
import jax.numpy as jnp
import numpy as np
from jax.experimental import pallas as pl
from jax.experimental.pallas import tpu as pltpu

S = 2048; D = 640; H = 32; DH = 192; M = 8; SEG = 32; NSEG = S // SEG
NPAIR = H // 2; PW = 2 * DH
BH = 32; BDH = D // BH; BW = 8; BDIL = 2
LOG2E = 1.4426950408889634
NEG = -1e30
f32 = jnp.float32; bf16 = jnp.bfloat16; u32 = jnp.uint32

SCHED = {
    (0, 'post'): ['bqkv'],
    (12, 'post'): ['bhist'],
    (5, 'post'): ['b1fin'],
    (13, 'post'): ['hcopy', ('wo', 0, 5)],
    (14, 'k'): [('wo', 5, 10)],
    (14, 'post'): [('wo', 10, 14)],
    (15, 'post'): [('wo', 14, 16), 'b2fin'],
}
BDEP = {1: [(0, 0, 8)], 2: [(0, 8, 8)], 3: [(0, 16, 8)], 4: [(0, 24, 8)], 8: [(1, 0, 8)], 9: [(1, 8, 8)], 10: [(1, 16, 8)], 11: [(1, 24, 8)]}
HALF = 1
UNROLL = 1
ORDER = 'B'

def _dot(a, b):
    return jnp.dot(a, b, preferred_element_type=f32)
def _dot_nt(a, b):
    return lax_dot(a, b, (((1,), (1,)), ((), ())))
def lax_dot(a, b, dn):
    return jax.lax.dot_general(a, b, dn, preferred_element_type=f32)

def _recip(x):
    r = pl.reciprocal(x, approx=True)
    return r * (2.0 - x * r)

def _ln(x):
    m = jnp.mean(x, axis=-1, keepdims=True)
    xc = x - m
    v = jnp.mean(xc * xc, axis=-1, keepdims=True)
    return xc * jax.lax.rsqrt(v + 1e-5)

def _perm_mat():
    r = jax.lax.broadcasted_iota(jnp.int32, (D, D), 0)
    c = jax.lax.broadcasted_iota(jnp.int32, (D, D), 1)
    h = c % BH
    d = c // BH
    return (r == h * BDH + d).astype(bf16)

def _pk(x):
    return pltpu.bitcast(x.astype(bf16), u32)
def _up(x):
    return pltpu.bitcast(x, bf16)

def kernel(nsteps, x_hbm, mem0_hbm, wq_hbm, wk_hbm, wv_hbm, wo_hbm, bqkv_hbm, bwo_hbm, out_hbm,
           wq, wk, wv, wo, bqkv_raw, bwo_raw, bqkv_p, bwo_p, x_ref, mem0_ref, out_ref,
           h_ref, qkv_ref, o_ref, xa_ref, xb_ref, kb_ref, vb_ref, xan_ref, bq_ref, bo_ref, hn_ref,
           sem_w, sem_m, sem_o):
    RW = PW // 2
    ws = (wq, wk, wv)
    ws_hbm = (wq_hbm.bitcast(u32), wk_hbm.bitcast(u32), wv_hbm.bitcast(u32))
    NWO = 4
    RO = H * DH // 2 // NWO
    def cp_w(j, g):
        sl = pl.ds(pl.multiple_of(g * RW, RW), RW) if not isinstance(g, int) else pl.ds(g * RW, RW)
        return pltpu.make_async_copy(ws_hbm[j].at[sl], ws[j].at[sl], sem_w.at[g])
    cp_x0 = pltpu.make_async_copy(x_hbm.at[0:2 * SEG], x_ref.at[0:2 * SEG], sem_m.at[0])
    cp_mem = pltpu.make_async_copy(mem0_hbm, mem0_ref, sem_m.at[1])
    cp_bqkv = pltpu.make_async_copy(bqkv_hbm, bqkv_raw, sem_m.at[2])
    cp_bwo = pltpu.make_async_copy(bwo_hbm, bwo_raw, sem_m.at[3])
    cp_wo = [pltpu.make_async_copy(wo_hbm.bitcast(u32).at[i * RO:(i + 1) * RO], wo.at[i * RO:(i + 1) * RO], sem_m.at[4 + i])
             for i in range(NWO)]
    cp_x1 = pltpu.make_async_copy(x_hbm.at[2 * SEG:S], x_ref.at[2 * SEG:S], sem_m.at[4 + NWO])
    def cp_out(s):
        sl = pl.ds(pl.multiple_of(s * SEG, SEG), SEG) if not isinstance(s, int) else pl.ds(s * SEG, SEG)
        return pltpu.make_async_copy(out_ref.at[sl], out_hbm.at[sl], sem_o.at[0])

    cp_x0.start(); cp_mem.start(); cp_bqkv.start(); cp_bwo.start()
    for g in range(NPAIR):
        for j in range(3): cp_w(j, g).start()
    for c in cp_wo: c.start()
    cp_x1.start()

    xb_ref[...] = jnp.zeros((2 * SEG, D), f32)
    kb_ref[...] = jnp.zeros(kb_ref.shape, f32)
    vb_ref[...] = jnp.zeros(vb_ref.shape, f32)
    xa_ref[SEG:2 * SEG, :] = jnp.zeros((SEG, D), f32)
    h_ref[24:40, :] = jnp.zeros((16, D), u32)
    cp_x0.wait(); cp_mem.wait()
    mem0 = mem0_ref[...]
    mem00 = jnp.concatenate([mem0.astype(f32), mem0.astype(f32)], axis=0)
    h_ref[0:8, :] = _pk(mem00)
    x00 = x_ref[0:SEG, :].astype(f32)
    h_ref[8:24, :] = _pk(_ln(x00))
    xa_ref[0:SEG, :] = x00

    pm = _perm_mat()
    cp_bqkv.wait()
    for j in range(3):
        bqkv_p[:, j * D:(j + 1) * D] = _pk(_dot(bqkv_raw[:, j * D:(j + 1) * D], pm))
    cp_bwo.wait()
    bwo_p[...] = _pk(lax_dot(pm, bwo_raw[...], (((0,), (0,)), ((), ()))))

    lane = jax.lax.broadcasted_iota(jnp.int32, (48, 128), 1)
    lo64 = lane < 64
    rr = jax.lax.broadcasted_iota(jnp.int32, (48, 96), 0)
    cc = jax.lax.broadcasted_iota(jnp.int32, (48, 96), 1)
    ck = jnp.where(cc >= 48, cc - 48, cc)
    first = cc < 48
    def smask(l):
        memk = (ck >= 8 * l) & (ck < 8 * l + 8)
        tokk = (ck >= 16) & ((rr < 16) | (ck <= rr))
        return jnp.where(memk | tokk, 0.0, NEG).astype(f32)
    bias = [smask(0), smask(1)]
    row16 = jax.lax.broadcasted_iota(jnp.int32, (16, PW), 0)
    sc = (DH ** -0.5) * LOG2E

    def bd(a):
        z = jnp.zeros((48, 128), bf16)
        a0, a1, a2 = a[:, 0:128], a[:, 128:256], a[:, 256:384]
        top = jnp.concatenate([a0, jnp.where(lo64, a1, z), z], axis=1)
        bot = jnp.concatenate([z, jnp.where(lo64, z, a1), a2], axis=1)
        return jnp.concatenate([top, bot], axis=0)

    def lhs_h(lh):
        if lh is None:
            return _up(h_ref[...])
        return _up(jnp.concatenate([h_ref[0:8, :], h_ref[pl.ds(pl.multiple_of(8 + 16 * lh, 8), 16), :]], axis=0))
    def proj(g, j, lh=None):
        sl = pl.ds(pl.multiple_of(g * RW, RW), RW) if not isinstance(g, int) else pl.ds(g * RW, RW)
        y = _pk(_dot_nt(lhs_h(lh), _up(ws[j][sl, :])))
        if lh is None: qkv_ref[g, j] = y
        else: qkv_ref[g, j, 0:24, :] = y
    def rows(j, g, l):
        if l is None: return _up(qkv_ref[g, j, 0:24, :])
        return jnp.concatenate([_up(qkv_ref[g, j, 0:8, :]), _up(qkv_ref[g, j, 8 + 16 * l:24 + 16 * l, :])], axis=0)
    def qk(g, l):
        return _dot_nt(rows(0, g, l), bd(rows(1, g, l)))
    def sm(s, bias_l):
        s = s * sc + bias_l
        m0 = jnp.max(jnp.where(first, s, NEG), axis=1, keepdims=True)
        m1 = jnp.max(jnp.where(first, NEG, s), axis=1, keepdims=True)
        p = jnp.exp2(s - jnp.where(first, m0, m1))
        s0 = jnp.sum(jnp.where(first, p, 0.0), axis=1, keepdims=True)
        s1 = jnp.sum(jnp.where(first, 0.0, p), axis=1, keepdims=True)
        p = p * _recip(jnp.where(first, s0, s1))
        return p.astype(bf16)
    def pv(g, ps):
        if len(ps) == 1:
            o_ref[g, 0:24, :] = _pk(_dot(ps[0], bd(rows(2, g, None))))
            return
        os_ = [_dot(ps[l], bd(rows(2, g, l))) for l in range(2)]
        om = jnp.where(row16 < 8, os_[0][0:16], os_[1][0:16])
        o = jnp.concatenate([om, os_[0][16:48], os_[1][16:48]], axis=0)
        o_ref[g] = _pk(o)

    rC = jax.lax.broadcasted_iota(jnp.int32, (16, 128), 0)
    bsc = (BDH ** -0.5) * LOG2E

    def b_qkv():
        y = _dot(_ln(xb_ref[...]).astype(bf16), _up(bqkv_p[...]))
        bq_ref[...] = y[:, 0:D]
        for l in range(2):
            kb_ref[l, 16:48, :] = y[32 * l:32 * l + 32, D:2 * D]
            vb_ref[l, 16:48, :] = y[32 * l:32 * l + 32, 2 * D:3 * D]
    def b_attn(t, l, r0, nr):
        q = bq_ref[32 * l + r0:32 * l + r0 + nr, :]
        seg = t - 1 - 2 * l
        pos = seg * SEG + r0 + rC[0:nr]
        lg = []
        for w in range(BW):
            off = 16 - BDIL * w + r0
            pr = q * kb_ref[l, off:off + nr, :]
            a = pr[:, 0:128] + pr[:, 128:256] + pr[:, 256:384] + pr[:, 384:512] + pr[:, 512:640]
            a = a + pltpu.roll(a, 64, 1)
            a = a + pltpu.roll(a, 32, 1)
            a = a * bsc
            if w > 0:
                a = jnp.where(pos >= BDIL * w, a, NEG)
            lg.append(a)
        m = lg[0]
        for w in range(1, BW): m = jnp.maximum(m, lg[w])
        ps = [jnp.exp2(a - m) for a in lg]
        den = ps[0]
        for w in range(1, BW): den = den + ps[w]
        inv = _recip(den)
        acc = None
        for w in range(BW):
            off = 16 - BDIL * w + r0
            pw = ps[w] * inv
            pw5 = jnp.concatenate([pw] * 5, axis=1)
            tt = pw5 * vb_ref[l, off:off + nr, :]
            acc = tt if acc is None else acc + tt
        bo_ref[32 * l + r0:32 * l + r0 + nr, :] = acc
        z = acc[0:8, 0:128]
        for rr_ in range(nr // 8):
            for cc_ in range(5):
                if rr_ or cc_: z = jnp.maximum(z, acc[8 * rr_:8 * rr_ + 8, 128 * cc_:128 * cc_ + 128])
        return z
    def b_hist():
        for l in range(2):
            kb_ref[l, 0:16, :] = kb_ref[l, 32:48, :]
            vb_ref[l, 0:16, :] = vb_ref[l, 32:48, :]
    def b_out(l):
        return xb_ref[32 * l:32 * l + 32, :] + _dot(bo_ref[32 * l:32 * l + 32, :].astype(bf16), _up(bwo_p[...]))
    def b1_finish(t):
        x2 = b_out(0)
        xn = x_ref[pl.ds(pl.multiple_of(jnp.minimum(t + 1, NSEG - 1) * SEG, SEG), SEG), :].astype(f32)
        xan_ref[0:SEG, :] = xn
        xan_ref[SEG:2 * SEG, :] = x2
        hn_ref[0:16, :] = _pk(_ln(xn))
        hn_ref[16:32, :] = _pk(_ln(x2))
    def b2_finish(t):
        x4 = b_out(1)
        out_ref[pl.ds(pl.multiple_of(jnp.maximum(t - 3, 0) * SEG, SEG), SEG), :] = x4.astype(bf16)
    def wo_part(g0, g1, half=False):
        o = jnp.concatenate([_up(o_ref[g, 0:24, :] if half else o_ref[g]) for g in range(g0, g1)], axis=1)
        return _dot(o, _up(wo[g0 * PW // 2:g1 * PW // 2, :]))

    def step_body(t, half):
        st = {}
        ss = {}; pp = {}
        lh = jnp.where(t < 2, 0, 1) if half else None
        bias_h = smask(lh) if half else None
        def ex(i, pos):
            for name in SCHED.get((i, pos), ()): run_extra(name, t, st, half)
        for i in range(-2, NPAIR):
            g2, g1, g0 = i + 2, i + 1, i
            ex(i, 'pre')
            if g2 < NPAIR: proj(g2, 0, lh)
            ex(i, 'q')
            if g2 < NPAIR: proj(g2, 1, lh)
            ex(i, 'k')
            if g2 < NPAIR: proj(g2, 2, lh)
            ex(i, 'v')
            if 0 <= g1 < NPAIR:
                if half:
                    pp[g1] = [sm(qk(g1, None), bias_h)]
                else:
                    s_ = [qk(g1, 0), qk(g1, 1)]
                    pp[g1] = [sm(s_[0], bias[0]), sm(s_[1], bias[1])]
            if 0 <= g0:
                pg = pp.pop(g0)
                for (l_, r0_, nr_) in BDEP.get(g0, ()):
                    z = b_attn(t, l_, r0_, nr_)
                    p0 = jnp.where(t < 0, z[:, 0:96].astype(bf16), pg[0][0:8])
                    pg[0] = jnp.concatenate([p0, pg[0][8:]], axis=0)
                pv(g0, pg)
            ex(i, 'post')
        end_step(t, st['oa'], lh)

    def step(t, c):
        if HALF:
            is_half = (t < 2) | (t >= NSEG)
            pl.when(is_half)(lambda: step_body(t, True))
            pl.when(jnp.logical_not(is_half))(lambda: step_body(t, False))
        else:
            step_body(t, False)
        @pl.when(t >= 3)
        def _():
            cp_out(jnp.maximum(t - 3, 0)).start()
        return c

    def end_step(t, oa, lh=None):
        if lh is None:
            xb_ref[...] = xa_ref[...] + oa[16:80]
        else:
            sl = pl.ds(pl.multiple_of(SEG * lh, SEG), SEG)
            xb_ref[sl, :] = xa_ref[sl, :] + oa[16:48]
        xa_ref[...] = xan_ref[...]
        r16 = jax.lax.broadcasted_iota(jnp.int32, (16, D), 0)
        memn = jnp.where((r16 >= 8) & (t < 2), mem00, oa[0:16])
        h_ref[0:8, :] = _pk(memn)

    def run_extra(name, t, st, half):
        if name == 'bqkv': b_qkv()
        elif name[0] == 'battn': b_attn(t, name[1], name[2], name[3])
        elif name == 'bhist': b_hist()
        elif name == 'hcopy': h_ref[8:40, :] = hn_ref[...]
        elif name == 'b1fin': b1_finish(t)
        elif name == 'b2fin': b2_finish(t)
        elif name[0] == 'wo':
            part = wo_part(name[1], name[2], half)
            st['oa'] = part if 'oa' not in st else st['oa'] + part
        else: raise ValueError(name)

    def pair0(g, c):
        for j in range(3): cp_w(j, g).wait()
        for j in range(3): proj(g, j)
        pv(g, [sm(qk(g, l), bias[l]) for l in range(2)])
        return c
    jax.lax.fori_loop(0, NPAIR, pair0, 0)
    oa = None
    for i in range(NWO):
        cp_wo[i].wait()
        part = wo_part(i * NPAIR // NWO, (i + 1) * NPAIR // NWO)
        oa = part if oa is None else oa + part
    xn = x_ref[SEG:2 * SEG, :].astype(f32)
    xan_ref[0:SEG, :] = xn
    xan_ref[SEG:2 * SEG, :] = jnp.zeros((SEG, D), f32)
    h_ref[8:24, :] = _pk(_ln(xn))
    end_step(0, oa)
    cp_x1.wait()

    jax.lax.fori_loop(1, nsteps, step, 0, unroll=UNROLL)
    b_qkv()
    for c_ in range(2): b_attn(NSEG + 2, 1, 16 * c_, 16)
    b2_finish(NSEG + 2)
    cp_out(NSEG - 1).start()
    def wait_out(s, c):
        cp_out(s).wait()
        return c
    jax.lax.fori_loop(0, min(nsteps - 3, NSEG - 1) + 1 if nsteps > 3 else 1, wait_out, 0)

@functools.partial(jax.jit, static_argnames=("A_seg_len",))
def pallas_interleave_layers__memory_aug_recurrent_mem_tr__sliding_local_dilated__prompt_kernel(
        A_x, A_mem0, A_Wq, A_Wk, A_Wv, A_Wo, A_seg_len, B_x, B_wqkv, B_wo):
    assert A_seg_len == SEG
    del B_x
    nsteps = NSEG + 2
    x = A_x.reshape(S, D)
    mem0 = A_mem0.reshape(M, D)
    tr = lambda w: jnp.transpose(w, (1, 2, 0)).reshape(H * DH, D)
    wo = A_Wo.reshape(H * DH, D)
    hbm = pl.BlockSpec(memory_space=pl.ANY)
    out = pl.pallas_call(
        functools.partial(kernel, nsteps),
        out_shape=jax.ShapeDtypeStruct((S, D), bf16),
        in_specs=[hbm] * 8,
        out_specs=hbm,
        scratch_shapes=[
            pltpu.VMEM((H * DH // 2, D), u32), pltpu.VMEM((H * DH // 2, D), u32), pltpu.VMEM((H * DH // 2, D), u32), pltpu.VMEM((H * DH // 2, D), u32),
            pltpu.VMEM((D, 3 * D), bf16), pltpu.VMEM((D, D), bf16),
            pltpu.VMEM((D // 2, 3 * D), u32), pltpu.VMEM((D // 2, D), u32),
            pltpu.VMEM((S, D), bf16), pltpu.VMEM((M, D), bf16), pltpu.VMEM((S, D), bf16),
            pltpu.VMEM((40, D), u32), pltpu.VMEM((NPAIR, 3, 40, PW), u32), pltpu.VMEM((NPAIR, 40, PW), u32),
            pltpu.VMEM((64, D), f32), pltpu.VMEM((64, D), f32),
            pltpu.VMEM((2, 48, D), f32), pltpu.VMEM((2, 48, D), f32),
            pltpu.VMEM((64, D), f32), pltpu.VMEM((64, D), f32), pltpu.VMEM((64, D), f32),
            pltpu.VMEM((32, D), u32),
            pltpu.SemaphoreType.DMA((NPAIR,)), pltpu.SemaphoreType.DMA((9,)), pltpu.SemaphoreType.DMA((1,)),
        ],
        compiler_params=pltpu.CompilerParams(vmem_limit_bytes=100 * 1024 * 1024),
    )(x, mem0, tr(A_Wq), tr(A_Wk), tr(A_Wv), wo, B_wqkv, B_wo)
    return out.reshape(1, S, D)
```

```python
import functools
import jax
import jax.numpy as jnp
import numpy as np
from jax.experimental import pallas as pl
from jax.experimental.pallas import tpu as pltpu

S = 2048; D = 640; H = 32; DH = 192; M = 8; SEG = 32; NSEG = S // SEG
NPAIR = H // 2; PW = 2 * DH
BH = 32; BDH = D // BH; BW = 8; BDIL = 2
LOG2E = 1.4426950408889634
NEG = -1e30
f32 = jnp.float32; bf16 = jnp.bfloat16; u32 = jnp.uint32

SCHED = {
    (0, 'post'): ['bqkv'],
    (12, 'post'): ['bhist'],
    (5, 'post'): ['b1fin'],
    (13, 'post'): ['hcopy', ('wo', 0, 5)],
    (14, 'k'): [('wo', 5, 10)],
    (14, 'post'): [('wo', 10, 14)],
    (15, 'post'): [('wo', 14, 16), 'b2fin'],
}
BDEP = {1: [(0, 0, 8)], 2: [(0, 8, 8)], 3: [(0, 16, 8)], 4: [(0, 24, 8)], 8: [(1, 0, 8)], 9: [(1, 8, 8)], 10: [(1, 16, 8)], 11: [(1, 24, 8)]}
NPRE = 14
HALF = 1
UNROLL = 1
ORDER = 'B'

def _dot(a, b):
    return jnp.dot(a, b, preferred_element_type=f32)
def _dot_nt(a, b):
    return lax_dot(a, b, (((1,), (1,)), ((), ())))
def lax_dot(a, b, dn):
    return jax.lax.dot_general(a, b, dn, preferred_element_type=f32)

def _recip(x):
    r = pl.reciprocal(x, approx=True)
    return r * (2.0 - x * r)

def _ln(x):
    m = jnp.mean(x, axis=-1, keepdims=True)
    xc = x - m
    v = jnp.mean(xc * xc, axis=-1, keepdims=True)
    return xc * jax.lax.rsqrt(v + 1e-5)

def _perm_mat():
    r = jax.lax.broadcasted_iota(jnp.int32, (D, D), 0)
    c = jax.lax.broadcasted_iota(jnp.int32, (D, D), 1)
    h = c % BH
    d = c // BH
    return (r == h * BDH + d).astype(bf16)

def _pk(x):
    return pltpu.bitcast(x.astype(bf16), u32)
def _up(x):
    return pltpu.bitcast(x, bf16)

def kernel(nsteps, x_hbm, mem0_hbm, wq_hbm, wk_hbm, wv_hbm, wo_hbm, bqkv_hbm, bwo_hbm, out_hbm,
           wq, wk, wv, wo, bqkv_raw, bwo_raw, bqkv_p, bwo_p, x_ref, mem0_ref, out_ref,
           h_ref, qkv_ref, o_ref, xa_ref, xb_ref, kb_ref, vb_ref, xan_ref, bq_ref, bo_ref, hn_ref, hp_ref, pre_ref, wof_ref,
           sem_w, sem_m, sem_o):
    RW = PW // 2
    ws = (wq, wk, wv)
    ws_hbm = (wq_hbm.bitcast(u32), wk_hbm.bitcast(u32), wv_hbm.bitcast(u32))
    NWO = 4
    RO = H * DH // 2 // NWO
    def cp_w(j, g):
        sl = pl.ds(pl.multiple_of(g * RW, RW), RW) if not isinstance(g, int) else pl.ds(g * RW, RW)
        return pltpu.make_async_copy(ws_hbm[j].at[sl], ws[j].at[sl], sem_w.at[g])
    X0R = (NPRE + 2) * SEG
    cp_x0 = pltpu.make_async_copy(x_hbm.at[0:X0R], x_ref.at[0:X0R], sem_m.at[0])
    cp_mem = pltpu.make_async_copy(mem0_hbm, mem0_ref, sem_m.at[1])
    cp_bqkv = pltpu.make_async_copy(bqkv_hbm.bitcast(u32), bqkv_raw, sem_m.at[2])
    cp_bwo = pltpu.make_async_copy(bwo_hbm, bwo_raw, sem_m.at[3])
    def cp_wo(i):
        sl = pl.ds(pl.multiple_of(i * RO, RO), RO) if not isinstance(i, int) else pl.ds(i * RO, RO)
        return pltpu.make_async_copy(wo_hbm.bitcast(u32).at[sl], wo.at[sl], sem_m.at[4 + i])
    cp_x1 = pltpu.make_async_copy(x_hbm.at[X0R:S], x_ref.at[X0R:S], sem_m.at[4 + NWO])
    def cp_out(s):
        sl = pl.ds(pl.multiple_of(s * SEG, SEG), SEG) if not isinstance(s, int) else pl.ds(s * SEG, SEG)
        return pltpu.make_async_copy(out_ref.at[sl], out_hbm.at[sl], sem_o.at[0])

    cp_bwo.start(); cp_x0.start(); cp_mem.start(); cp_bqkv.start()
    for g in range(NPAIR):
        for j in range(3): cp_w(j, g).start()
    for i_ in range(NWO): cp_wo(i_).start()
    cp_x1.start()

    xb_ref[...] = jnp.zeros((2 * SEG, D), f32)
    kb_ref[...] = jnp.zeros(kb_ref.shape, f32)
    vb_ref[...] = jnp.zeros(vb_ref.shape, f32)
    xa_ref[SEG:2 * SEG, :] = jnp.zeros((SEG, D), f32)
    h_ref[24:40, :] = jnp.zeros((16, D), u32)
    cp_x0.wait(); cp_mem.wait()
    mem0 = mem0_ref[...]
    mem00 = jnp.concatenate([mem0.astype(f32), mem0.astype(f32)], axis=0)
    h_ref[0:8, :] = _pk(mem00)
    x00 = x_ref[0:SEG, :].astype(f32)
    h_ref[8:24, :] = _pk(_ln(x00))
    xa_ref[0:SEG, :] = x00
    hp_ref[0:8, :] = _pk(mem00)
    hp_ref[8:24, :] = _pk(_ln(x00))
    for i_ in range(NPRE):
        hp_ref[24 + 8 * i_:32 + 8 * i_, :] = _pk(_ln(x_ref[(i_ + 2) * SEG:(i_ + 2) * SEG + 16, :].astype(f32)))

    cp_bwo.wait()
    def cvt_wo(i, c):
        r = pl.ds(pl.multiple_of(i * 64, 64), 64)
        v_ = bwo_raw[r, :].astype(f32)
        for k_ in range(5): wof_ref[k_, r, :] = v_[:, k_ * 128:(k_ + 1) * 128]
        return c
    jax.lax.fori_loop(0, D // 64, cvt_wo, 0)
    def perm_wo(d, c):
        blk = jnp.concatenate([wof_ref[k_, pl.ds(d, BH, stride=BDH), :] for k_ in range(5)], axis=1)
        bwo_p[pl.ds(pl.multiple_of(d * (BH // 2), BH // 2), BH // 2), :] = _pk(blk)
        return c
    jax.lax.fori_loop(0, BDH, perm_wo, 0)

    lane8 = jax.lax.broadcasted_iota(jnp.int32, (8, 128), 1)
    def perm_unit(u):
        j = u // 40
        r = pl.ds(pl.multiple_of((u - 40 * j) * 8, 8), 8)
        srcs = [bqkv_raw[r, pl.ds(pl.multiple_of(j * D + k_ * 128, 128), 128)] for k_ in range(5)]
        for n in range(5):
            col = lane8 + n * 128
            s = (col % BH) * BDH + col // BH
            acc = None
            for k_ in range(5):
                g_ = jnp.take_along_axis(srcs[k_], s % 128, axis=1)
                acc = g_ if acc is None else jnp.where(s // 128 == k_, g_, acc)
            bqkv_p[r, pl.ds(pl.multiple_of(j * D + n * 128, 128), 128)] = acc

    lane = jax.lax.broadcasted_iota(jnp.int32, (48, 128), 1)
    lo64 = lane < 64
    rr = jax.lax.broadcasted_iota(jnp.int32, (48, 96), 0)
    cc = jax.lax.broadcasted_iota(jnp.int32, (48, 96), 1)
    ck = jnp.where(cc >= 48, cc - 48, cc)
    first = cc < 48
    def smask(l):
        memk = (ck >= 8 * l) & (ck < 8 * l + 8)
        tokk = (ck >= 16) & ((rr < 16) | (ck <= rr))
        return jnp.where(memk | tokk, 0.0, NEG).astype(f32)
    bias = [smask(0), smask(1)]
    row16 = jax.lax.broadcasted_iota(jnp.int32, (16, PW), 0)
    sc = (DH ** -0.5) * LOG2E

    def bd(a):
        z = jnp.zeros((48, 128), bf16)
        a0, a1, a2 = a[:, 0:128], a[:, 128:256], a[:, 256:384]
        top = jnp.concatenate([a0, jnp.where(lo64, a1, z), z], axis=1)
        bot = jnp.concatenate([z, jnp.where(lo64, z, a1), a2], axis=1)
        return jnp.concatenate([top, bot], axis=0)

    def lhs_h(var, lh):
        if var == 'full':
            return _up(h_ref[...])
        if var == 'v64':
            return _up(jnp.concatenate([h_ref[0:8, :], h_ref[16:40, :]], axis=0))
        return _up(jnp.concatenate([h_ref[0:8, :], h_ref[pl.ds(pl.multiple_of(8 + 16 * lh, 8), 16), :]], axis=0))
    def proj(g, j, var='full', lh=None):
        sl = pl.ds(pl.multiple_of(g * RW, RW), RW) if not isinstance(g, int) else pl.ds(g * RW, RW)
        y = _pk(_dot_nt(lhs_h(var, lh), _up(ws[j][sl, :])))
        if var == 'full': qkv_ref[g, j] = y
        elif var == 'v64':
            qkv_ref[g, j, 0:8, :] = y[0:8]
            qkv_ref[g, j, 16:40, :] = y[8:32]
        else: qkv_ref[g, j, 0:24, :] = y
    def rows(j, g, l, pre=None):
        if l is None: return _up(qkv_ref[g, j, 0:24, :])
        if l == 0 and pre is not None:
            return jnp.concatenate([_up(qkv_ref[g, j, 0:8, :]), _up(pre_ref[g, j, pl.ds(pl.multiple_of(8 * pre, 8), 8), :]),
                                    _up(qkv_ref[g, j, 16:24, :])], axis=0)
        return jnp.concatenate([_up(qkv_ref[g, j, 0:8, :]), _up(qkv_ref[g, j, 8 + 16 * l:24 + 16 * l, :])], axis=0)
    def qk(g, l, pre=None):
        return _dot_nt(rows(0, g, l, pre), bd(rows(1, g, l, pre)))
    def sm(s, bias_l):
        s = s * sc + bias_l
        m0 = jnp.max(jnp.where(first, s, NEG), axis=1, keepdims=True)
        m1 = jnp.max(jnp.where(first, NEG, s), axis=1, keepdims=True)
        p = jnp.exp2(s - jnp.where(first, m0, m1))
        s0 = jnp.sum(jnp.where(first, p, 0.0), axis=1, keepdims=True)
        s1 = jnp.sum(jnp.where(first, 0.0, p), axis=1, keepdims=True)
        p = p * _recip(jnp.where(first, s0, s1))
        return p.astype(bf16)
    def pv(g, ps, pre=None):
        if len(ps) == 1:
            o_ref[g, 0:24, :] = _pk(_dot(ps[0], bd(rows(2, g, None))))
            return
        os_ = [_dot(ps[l], bd(rows(2, g, l, pre))) for l in range(2)]
        om = jnp.where(row16 < 8, os_[0][0:16], os_[1][0:16])
        o = jnp.concatenate([om, os_[0][16:48], os_[1][16:48]], axis=0)
        o_ref[g] = _pk(o)

    rC = jax.lax.broadcasted_iota(jnp.int32, (16, 128), 0)
    bsc = (BDH ** -0.5) * LOG2E

    def b_qkv():
        y = _dot(_ln(xb_ref[...]).astype(bf16), _up(bqkv_p[...]))
        bq_ref[...] = y[:, 0:D]
        for l in range(2):
            kb_ref[l, 16:48, :] = y[32 * l:32 * l + 32, D:2 * D]
            vb_ref[l, 16:48, :] = y[32 * l:32 * l + 32, 2 * D:3 * D]
    def b_attn(t, l, r0, nr):
        q = bq_ref[32 * l + r0:32 * l + r0 + nr, :]
        seg = t - 1 - 2 * l
        pos = seg * SEG + r0 + rC[0:nr]
        lg = []
        for w in range(BW):
            off = 16 - BDIL * w + r0
            pr = q * kb_ref[l, off:off + nr, :]
            a = pr[:, 0:128] + pr[:, 128:256] + pr[:, 256:384] + pr[:, 384:512] + pr[:, 512:640]
            a = a + pltpu.roll(a, 64, 1)
            a = a + pltpu.roll(a, 32, 1)
            a = a * bsc
            if w > 0:
                a = jnp.where(pos >= BDIL * w, a, NEG)
            lg.append(a)
        m = lg[0]
        for w in range(1, BW): m = jnp.maximum(m, lg[w])
        ps = [jnp.exp2(a - m) for a in lg]
        den = ps[0]
        for w in range(1, BW): den = den + ps[w]
        inv = _recip(den)
        acc = None
        for w in range(BW):
            off = 16 - BDIL * w + r0
            pw = ps[w] * inv
            pw5 = jnp.concatenate([pw] * 5, axis=1)
            tt = pw5 * vb_ref[l, off:off + nr, :]
            acc = tt if acc is None else acc + tt
        bo_ref[32 * l + r0:32 * l + r0 + nr, :] = acc
        z = acc[0:8, 0:128]
        for rr_ in range(nr // 8):
            for cc_ in range(5):
                if rr_ or cc_: z = jnp.maximum(z, acc[8 * rr_:8 * rr_ + 8, 128 * cc_:128 * cc_ + 128])
        return z
    def b_hist():
        for l in range(2):
            kb_ref[l, 0:16, :] = kb_ref[l, 32:48, :]
            vb_ref[l, 0:16, :] = vb_ref[l, 32:48, :]
    def b_out(l):
        return xb_ref[32 * l:32 * l + 32, :] + _dot(bo_ref[32 * l:32 * l + 32, :].astype(bf16), _up(bwo_p[...]))
    def b1_finish(t):
        x2 = b_out(0)
        xn = x_ref[pl.ds(pl.multiple_of(jnp.minimum(t + 1, NSEG - 1) * SEG, SEG), SEG), :].astype(f32)
        xan_ref[0:SEG, :] = xn
        xan_ref[SEG:2 * SEG, :] = x2
        hn_ref[0:16, :] = _pk(_ln(xn))
        hn_ref[16:32, :] = _pk(_ln(x2))
    def b2_finish(t):
        x4 = b_out(1)
        out_ref[pl.ds(pl.multiple_of(jnp.maximum(t - 3, 0) * SEG, SEG), SEG), :] = x4.astype(bf16)
    def wo_part(g0, g1, half=False):
        o = jnp.concatenate([_up(o_ref[g, 0:24, :] if half else o_ref[g]) for g in range(g0, g1)], axis=1)
        return _dot(o, _up(wo[g0 * PW // 2:g1 * PW // 2, :]))

    def step_body(t, var):
        st = {}
        pp = {}
        half = var == 'half'
        lh = jnp.where(t < 2, 0, 1) if half else None
        bias_h = smask(lh) if half else None
        pre = jnp.clip(t - 2, 0, NPRE - 1) if var == 'v64' else None
        def ex(i, pos):
            for name in SCHED.get((i, pos), ()): run_extra(name, t, st, half)
        for i in range(-2, NPAIR):
            g2, g1, g0 = i + 2, i + 1, i
            ex(i, 'pre')
            if g2 < NPAIR: proj(g2, 0, var, lh)
            ex(i, 'q')
            if g2 < NPAIR: proj(g2, 1, var, lh)
            ex(i, 'k')
            if g2 < NPAIR: proj(g2, 2, var, lh)
            ex(i, 'v')
            if 0 <= g1 < NPAIR:
                if half:
                    pp[g1] = [sm(qk(g1, None), bias_h)]
                else:
                    s_ = [qk(g1, 0, pre), qk(g1, 1, pre)]
                    pp[g1] = [sm(s_[0], bias[0]), sm(s_[1], bias[1])]
            if 0 <= g0:
                pg = pp.pop(g0)
                for (l_, r0_, nr_) in BDEP.get(g0, ()):
                    z = b_attn(t, l_, r0_, nr_)
                    p0 = jnp.where(t < 0, z[:, 0:96].astype(bf16), pg[0][0:8])
                    pg[0] = jnp.concatenate([p0, pg[0][8:]], axis=0)
                pv(g0, pg, pre)
            ex(i, 'post')
        end_step(t, st['oa'], lh)

    def step(t, c):
        is_half = (t < 2) | (t >= NSEG)
        is_v64 = (t >= 2) & (t < NPRE + 2)
        pl.when(is_half)(lambda: step_body(t, 'half'))
        pl.when(is_v64)(lambda: step_body(t, 'v64'))
        pl.when(jnp.logical_not(is_half | is_v64))(lambda: step_body(t, 'full'))
        @pl.when(t >= 3)
        def _():
            cp_out(jnp.maximum(t - 3, 0)).start()
        return c

    def end_step(t, oa, lh=None):
        if lh is None:
            xb_ref[...] = xa_ref[...] + oa[16:80]
        else:
            sl = pl.ds(pl.multiple_of(SEG * lh, SEG), SEG) if not isinstance(lh, int) else pl.ds(SEG * lh, SEG)
            xb_ref[sl, :] = xa_ref[sl, :] + oa[16:48]
        xa_ref[...] = xan_ref[...]
        r16 = jax.lax.broadcasted_iota(jnp.int32, (16, D), 0)
        memn = jnp.where((r16 >= 8) & (t < 2), mem00, oa[0:16])
        h_ref[0:8, :] = _pk(memn)

    def run_extra(name, t, st, half):
        if name == 'bqkv': b_qkv()
        elif name[0] == 'battn': b_attn(t, name[1], name[2], name[3])
        elif name == 'bhist': b_hist()
        elif name == 'hcopy': h_ref[8:40, :] = hn_ref[...]
        elif name == 'b1fin': b1_finish(t)
        elif name == 'b2fin': b2_finish(t)
        elif name[0] == 'wo':
            part = wo_part(name[1], name[2], half)
            st['oa'] = part if 'oa' not in st else st['oa'] + part
        else: raise ValueError(name)

    def wproj(g, j):
        sl = pl.ds(pl.multiple_of(g * RW, RW), RW)
        y = _pk(_dot_nt(_up(hp_ref[...]), _up(ws[j][sl, :])))
        qkv_ref[g, j, 0:24, :] = y[0:24]
        pre_ref[g, j] = y[24:]
    for j in range(3): qkv_ref[0, j, 0:24, :] = jnp.zeros((24, PW), u32)
    cp_bqkv.wait()
    def pair0(g, c):
        gp = jnp.maximum(g - 1, 0)
        for j in range(3): cp_w(j, g).wait()
        p = sm(qk(gp, None), bias[0])
        wproj(g, 0); wproj(g, 1)
        pv(gp, [p])
        wproj(g, 2)
        for k_ in range(8): perm_unit(jnp.minimum(8 * g + k_, 119))
        return c
    jax.lax.fori_loop(0, NPAIR, pair0, 0)
    pv(NPAIR - 1, [sm(qk(NPAIR - 1, None), bias[0])])
    xan_ref[0:48, :] = jnp.zeros((48, D), f32)
    def wo0(i, c):
        cp_wo(i).wait()
        GP = NPAIR // NWO
        o = jnp.concatenate([_up(o_ref[i * GP + g, 0:24, :]) for g in range(GP)], axis=1)
        xan_ref[0:48, :] += _dot(o, _up(wo[pl.ds(pl.multiple_of(i * RO, RO), RO), :]))
        return c
    jax.lax.fori_loop(0, NWO, wo0, 0)
    oa = xan_ref[0:48, :]
    xn = x_ref[SEG:2 * SEG, :].astype(f32)
    xan_ref[0:SEG, :] = xn
    xan_ref[SEG:2 * SEG, :] = jnp.zeros((SEG, D), f32)
    h_ref[8:24, :] = _pk(_ln(xn))
    end_step(0, oa, 0)
    cp_x1.wait()

    jax.lax.fori_loop(1, nsteps, step, 0, unroll=UNROLL)
    b_qkv()
    for c_ in range(2): b_attn(NSEG + 2, 1, 16 * c_, 16)
    b2_finish(NSEG + 2)
    cp_out(NSEG - 1).start()
    def wait_out(s, c):
        cp_out(s).wait()
        return c
    jax.lax.fori_loop(0, min(nsteps - 3, NSEG - 1) + 1 if nsteps > 3 else 1, wait_out, 0)

@functools.partial(jax.jit, static_argnames=("A_seg_len",))
def pallas_interleave_layers__memory_aug_recurrent_mem_tr__sliding_local_dilated__prompt_kernel(
        A_x, A_mem0, A_Wq, A_Wk, A_Wv, A_Wo, A_seg_len, B_x, B_wqkv, B_wo):
    assert A_seg_len == SEG
    del B_x
    nsteps = NSEG + 2
    x = A_x.reshape(S, D)
    mem0 = A_mem0.reshape(M, D)
    tr = lambda w: jnp.transpose(w, (1, 2, 0)).reshape(H * DH, D)
    wo = A_Wo.reshape(H * DH, D)
    hbm = pl.BlockSpec(memory_space=pl.ANY)
    out = pl.pallas_call(
        functools.partial(kernel, nsteps),
        out_shape=jax.ShapeDtypeStruct((S, D), bf16),
        in_specs=[hbm] * 8,
        out_specs=hbm,
        scratch_shapes=[
            pltpu.VMEM((H * DH // 2, D), u32), pltpu.VMEM((H * DH // 2, D), u32), pltpu.VMEM((H * DH // 2, D), u32), pltpu.VMEM((H * DH // 2, D), u32),
            pltpu.VMEM((D // 2, 3 * D), u32), pltpu.VMEM((D, D), bf16),
            pltpu.VMEM((D // 2, 3 * D), u32), pltpu.VMEM((D // 2, D), u32),
            pltpu.VMEM((S, D), bf16), pltpu.VMEM((M, D), bf16), pltpu.VMEM((S, D), bf16),
            pltpu.VMEM((40, D), u32), pltpu.VMEM((NPAIR, 3, 40, PW), u32), pltpu.VMEM((NPAIR, 40, PW), u32),
            pltpu.VMEM((64, D), f32), pltpu.VMEM((64, D), f32),
            pltpu.VMEM((2, 48, D), f32), pltpu.VMEM((2, 48, D), f32),
            pltpu.VMEM((64, D), f32), pltpu.VMEM((64, D), f32), pltpu.VMEM((64, D), f32),
            pltpu.VMEM((32, D), u32),
            pltpu.VMEM((24 + 8 * NPRE, D), u32), pltpu.VMEM((NPAIR, 3, 8 * NPRE, PW), u32), pltpu.VMEM((5, D, 128), f32),
            pltpu.SemaphoreType.DMA((NPAIR,)), pltpu.SemaphoreType.DMA((9,)), pltpu.SemaphoreType.DMA((1,)),
        ],
        compiler_params=pltpu.CompilerParams(vmem_limit_bytes=100 * 1024 * 1024),
    )(x, mem0, tr(A_Wq), tr(A_Wk), tr(A_Wv), wo, B_wqkv, B_wo)
    return out.reshape(1, S, D)
```

```python
import functools
import jax
import jax.numpy as jnp
import numpy as np
from jax.experimental import pallas as pl
from jax.experimental.pallas import tpu as pltpu

S = 2048; D = 640; H = 32; DH = 192; M = 8; SEG = 32; NSEG = S // SEG
NPAIR = H // 2; PW = 2 * DH
BH = 32; BDH = D // BH; BW = 8; BDIL = 2
LOG2E = 1.4426950408889634
NEG = -1e30
f32 = jnp.float32; bf16 = jnp.bfloat16; u32 = jnp.uint32

SCHED = {
    (0, 'post'): ['bqkv'],
    (12, 'post'): ['bhist'],
    (5, 'post'): ['b1fin'],
    (13, 'post'): ['hcopy', ('wo', 0, 5)],
    (14, 'k'): [('wo', 5, 10)],
    (14, 'post'): [('wo', 10, 14)],
    (15, 'post'): [('wo', 14, 16), 'b2fin'],
}
BDEP = {1: [(0, 0, 8)], 2: [(0, 8, 8)], 3: [(0, 16, 8)], 4: [(0, 24, 8)], 8: [(1, 0, 8)], 9: [(1, 8, 8)], 10: [(1, 16, 8)], 11: [(1, 24, 8)]}
NPRE = 16
WUNROLL = 1
HYB = 1
HALF = 1
UNROLL = 1
ORDER = 'B'

def _dot(a, b):
    return jnp.dot(a, b, preferred_element_type=f32)
def _dot_nt(a, b):
    return lax_dot(a, b, (((1,), (1,)), ((), ())))
def lax_dot(a, b, dn):
    return jax.lax.dot_general(a, b, dn, preferred_element_type=f32)

def _recip(x):
    r = pl.reciprocal(x, approx=True)
    return r * (2.0 - x * r)

def _ln(x):
    m = jnp.mean(x, axis=-1, keepdims=True)
    xc = x - m
    v = jnp.mean(xc * xc, axis=-1, keepdims=True)
    return xc * jax.lax.rsqrt(v + 1e-5)

def _perm_mat():
    r = jax.lax.broadcasted_iota(jnp.int32, (D, D), 0)
    c = jax.lax.broadcasted_iota(jnp.int32, (D, D), 1)
    h = c % BH
    d = c // BH
    return (r == h * BDH + d).astype(bf16)

def _pk(x):
    return pltpu.bitcast(x.astype(bf16), u32)
def _up(x):
    return pltpu.bitcast(x, bf16)

def kernel(nsteps, x_hbm, mem0_hbm, wq_hbm, wk_hbm, wv_hbm, wo_hbm, bqkv_hbm, bwo_hbm, out_hbm,
           wq, wk, wv, wo, bqkv_raw, bwo_raw, bqkv_p, bwo_p, x_ref, mem0_ref, out_ref,
           h_ref, qkv_ref, o_ref, xa_ref, xb_ref, kb_ref, vb_ref, xan_ref, bq_ref, bo_ref, hn_ref, hp_ref, pre_ref, wof_ref,
           sem_w, sem_m, sem_o):
    RW = PW // 2
    ws = (wq, wk, wv)
    ws_hbm = (wq_hbm.bitcast(u32), wk_hbm.bitcast(u32), wv_hbm.bitcast(u32))
    NWO = 4
    RO = H * DH // 2 // NWO
    def cp_w(j, g):
        sl = pl.ds(pl.multiple_of(g * RW, RW), RW) if not isinstance(g, int) else pl.ds(g * RW, RW)
        return pltpu.make_async_copy(ws_hbm[j].at[sl], ws[j].at[sl], sem_w.at[g])
    X0R = (NPRE + 2) * SEG
    cp_x0 = pltpu.make_async_copy(x_hbm.at[0:X0R], x_ref.at[0:X0R], sem_m.at[0])
    cp_mem = pltpu.make_async_copy(mem0_hbm, mem0_ref, sem_m.at[1])
    cp_bqkv = pltpu.make_async_copy(bqkv_hbm.bitcast(u32), bqkv_raw, sem_m.at[2])
    cp_bwo = pltpu.make_async_copy(bwo_hbm, bwo_raw, sem_m.at[3])
    def cp_wo(i):
        sl = pl.ds(pl.multiple_of(i * RO, RO), RO) if not isinstance(i, int) else pl.ds(i * RO, RO)
        return pltpu.make_async_copy(wo_hbm.bitcast(u32).at[sl], wo.at[sl], sem_m.at[4 + i])
    cp_x1 = pltpu.make_async_copy(x_hbm.at[X0R:S], x_ref.at[X0R:S], sem_m.at[4 + NWO])
    def cp_out(s):
        sl = pl.ds(pl.multiple_of(s * SEG, SEG), SEG) if not isinstance(s, int) else pl.ds(s * SEG, SEG)
        return pltpu.make_async_copy(out_ref.at[sl], out_hbm.at[sl], sem_o.at[0])

    cp_bwo.start(); cp_x0.start(); cp_mem.start(); cp_bqkv.start()
    for g in range(NPAIR):
        for j in range(3): cp_w(j, g).start()
    for i_ in range(NWO): cp_wo(i_).start()
    cp_x1.start()

    xb_ref[...] = jnp.zeros((2 * SEG, D), f32)
    kb_ref[...] = jnp.zeros(kb_ref.shape, f32)
    vb_ref[...] = jnp.zeros(vb_ref.shape, f32)
    xa_ref[SEG:2 * SEG, :] = jnp.zeros((SEG, D), f32)
    h_ref[24:40, :] = jnp.zeros((16, D), u32)
    cp_x0.wait(); cp_mem.wait()
    mem0 = mem0_ref[...]
    mem00 = jnp.concatenate([mem0.astype(f32), mem0.astype(f32)], axis=0)
    h_ref[0:8, :] = _pk(mem00)
    x00 = x_ref[0:SEG, :].astype(f32)
    h_ref[8:24, :] = _pk(_ln(x00))
    xa_ref[0:SEG, :] = x00
    hp_ref[0:8, :] = _pk(mem00)
    hp_ref[8:24, :] = _pk(_ln(x00))
    for i_ in range(NPRE):
        hp_ref[24 + 8 * i_:32 + 8 * i_, :] = _pk(_ln(x_ref[(i_ + 2) * SEG:(i_ + 2) * SEG + 16, :].astype(f32)))

    cp_bwo.wait()
    def cvt_wo(i, c):
        r = pl.ds(pl.multiple_of(i * 64, 64), 64)
        v_ = bwo_raw[r, :].astype(f32)
        for k_ in range(5): wof_ref[k_, r, :] = v_[:, k_ * 128:(k_ + 1) * 128]
        return c
    jax.lax.fori_loop(0, D // 64, cvt_wo, 0)
    def perm_wo(d, c):
        blk = jnp.concatenate([wof_ref[k_, pl.ds(d, BH, stride=BDH), :] for k_ in range(5)], axis=1)
        bwo_p[pl.ds(pl.multiple_of(d * (BH // 2), BH // 2), BH // 2), :] = _pk(blk)
        return c
    jax.lax.fori_loop(0, BDH, perm_wo, 0)

    lane8 = jax.lax.broadcasted_iota(jnp.int32, (8, 128), 1)
    def perm_unit(u):
        j = u // 40
        r = pl.ds(pl.multiple_of((u - 40 * j) * 8, 8), 8)
        srcs = [bqkv_raw[r, pl.ds(pl.multiple_of(j * D + k_ * 128, 128), 128)] for k_ in range(5)]
        for n in range(5):
            col = lane8 + n * 128
            s = (col % BH) * BDH + col // BH
            acc = None
            for k_ in range(5):
                g_ = jnp.take_along_axis(srcs[k_], s % 128, axis=1)
                acc = g_ if acc is None else jnp.where(s // 128 == k_, g_, acc)
            bqkv_p[r, pl.ds(pl.multiple_of(j * D + n * 128, 128), 128)] = acc

    lane = jax.lax.broadcasted_iota(jnp.int32, (48, 128), 1)
    lo64 = lane < 64
    rr = jax.lax.broadcasted_iota(jnp.int32, (48, 96), 0)
    cc = jax.lax.broadcasted_iota(jnp.int32, (48, 96), 1)
    ck = jnp.where(cc >= 48, cc - 48, cc)
    first = cc < 48
    def smask(l):
        memk = (ck >= 8 * l) & (ck < 8 * l + 8)
        tokk = (ck >= 16) & ((rr < 16) | (ck <= rr))
        return jnp.where(memk | tokk, 0.0, NEG).astype(f32)
    bias = [smask(0), smask(1)]
    row16 = jax.lax.broadcasted_iota(jnp.int32, (16, PW), 0)
    sc = (DH ** -0.5) * LOG2E

    def bd(a):
        z = jnp.zeros((48, 128), bf16)
        a0, a1, a2 = a[:, 0:128], a[:, 128:256], a[:, 256:384]
        top = jnp.concatenate([a0, jnp.where(lo64, a1, z), z], axis=1)
        bot = jnp.concatenate([z, jnp.where(lo64, z, a1), a2], axis=1)
        return jnp.concatenate([top, bot], axis=0)

    def lhs_h(var, lh):
        if var == 'full':
            return _up(h_ref[...])
        if var == 'v64':
            return _up(jnp.concatenate([h_ref[0:8, :], h_ref[16:40, :]], axis=0))
        return _up(jnp.concatenate([h_ref[0:8, :], h_ref[pl.ds(pl.multiple_of(8 + 16 * lh, 8), 16), :]], axis=0))
    def proj(g, j, var='full', lh=None):
        sl = pl.ds(pl.multiple_of(g * RW, RW), RW) if not isinstance(g, int) else pl.ds(g * RW, RW)
        y = _pk(_dot_nt(lhs_h(var, lh), _up(ws[j][sl, :])))
        if var == 'full': qkv_ref[g, j] = y
        elif var == 'v64':
            qkv_ref[g, j, 0:8, :] = y[0:8]
            qkv_ref[g, j, 16:40, :] = y[8:32]
        else: qkv_ref[g, j, 0:24, :] = y
    def rows(j, g, l, pre=None):
        if l is None: return _up(qkv_ref[g, j, 0:24, :])
        if l == 0 and pre is not None:
            return jnp.concatenate([_up(qkv_ref[g, j, 0:8, :]), _up(pre_ref[g, j, pl.ds(pl.multiple_of(8 * pre, 8), 8), :]),
                                    _up(qkv_ref[g, j, 16:24, :])], axis=0)
        return jnp.concatenate([_up(qkv_ref[g, j, 0:8, :]), _up(qkv_ref[g, j, 8 + 16 * l:24 + 16 * l, :])], axis=0)
    def qk(g, l, pre=None):
        return _dot_nt(rows(0, g, l, pre), bd(rows(1, g, l, pre)))
    def sm(s, bias_l):
        s = s * sc + bias_l
        m0 = jnp.max(jnp.where(first, s, NEG), axis=1, keepdims=True)
        m1 = jnp.max(jnp.where(first, NEG, s), axis=1, keepdims=True)
        p = jnp.exp2(s - jnp.where(first, m0, m1))
        s0 = jnp.sum(jnp.where(first, p, 0.0), axis=1, keepdims=True)
        s1 = jnp.sum(jnp.where(first, 0.0, p), axis=1, keepdims=True)
        p = p * _recip(jnp.where(first, s0, s1))
        return p.astype(bf16)
    def pv(g, ps, pre=None):
        if len(ps) == 1:
            o_ref[g, 0:24, :] = _pk(_dot(ps[0], bd(rows(2, g, None))))
            return
        os_ = [_dot(ps[l], bd(rows(2, g, l, pre))) for l in range(2)]
        om = jnp.where(row16 < 8, os_[0][0:16], os_[1][0:16])
        o = jnp.concatenate([om, os_[0][16:48], os_[1][16:48]], axis=0)
        o_ref[g] = _pk(o)

    h0c = [cc < 48, (cc < 16) | (cc >= 64)]
    row96 = jax.lax.broadcasted_iota(jnp.int32, (16, 96), 0)
    def parts(j, g, pre):
        m_ = _up(qkv_ref[g, j, 0:8, :])
        if pre is None:
            t1 = _up(qkv_ref[g, j, 8:24, :])
        else:
            t1 = jnp.concatenate([_up(pre_ref[g, j, pl.ds(pl.multiple_of(8 * pre, 8), 8), :]), _up(qkv_ref[g, j, 16:24, :])], axis=0)
        t2 = _up(qkv_ref[g, j, 24:40, :])
        return m_, t1, t2
    def lo_(a): return jnp.where(lo64[0:a.shape[0]], a, jnp.zeros_like(a))
    def hi_(a): return jnp.where(lo64[0:a.shape[0]], jnp.zeros_like(a), a)
    def rhs3(j, g, pre):
        m_, t1, t2 = parts(j, g, pre)
        z16 = jnp.zeros((16, 128), bf16)
        cat = lambda *xs: jnp.concatenate(xs, axis=0)
        r0 = cat(m_[:, 0:128], t1[:, 0:128], z16, t2[:, 0:128])
        r2 = cat(z16, t2[:, 256:384], m_[:, 256:384], t1[:, 256:384])
        m1, a1, b1 = m_[:, 128:256], t1[:, 128:256], t2[:, 128:256]
        rt0 = cat(lo_(m1), lo_(a1), hi_(m1), hi_(a1))
        rt1 = cat(lo_(m1), hi_(b1), hi_(m1), lo_(b1))
        return r0, r2, rt0, rt1
    def qk2(g, pre):
        m_, t1, t2 = parts(0, g, pre)
        q = jnp.concatenate([m_, t1, t2], axis=0)
        r0, r2, rt0, rt1 = rhs3(1, g, pre)
        a0 = _dot_nt(q[:, 0:128], r0)
        a2 = _dot_nt(q[:, 256:384], r2)
        q0 = q[0:48, 128:256]
        q1 = jnp.concatenate([q[0:16, 128:256], q[48:80, 128:256]], axis=0)
        s0 = jnp.where(h0c[0], a0[0:48], a2[0:48]) + _dot_nt(q0, rt0)
        a0l = jnp.concatenate([a0[0:16], a0[48:80]], axis=0)
        a2l = jnp.concatenate([a2[0:16], a2[48:80]], axis=0)
        s1 = jnp.where(h0c[1], a0l, a2l) + _dot_nt(q1, rt1)
        return s0, s1
    def sm2(s, bias_l, hc):
        s = s * sc + bias_l
        m0 = jnp.max(jnp.where(hc, s, NEG), axis=1, keepdims=True)
        m1 = jnp.max(jnp.where(hc, NEG, s), axis=1, keepdims=True)
        p = jnp.exp2(s - jnp.where(hc, m0, m1))
        s0 = jnp.sum(jnp.where(hc, p, 0.0), axis=1, keepdims=True)
        s1 = jnp.sum(jnp.where(hc, 0.0, p), axis=1, keepdims=True)
        return p * _recip(jnp.where(hc, s0, s1))
    def pv2(g, ps, pre):
        p0, p1 = ps
        r0, r2, rt0, rt1 = rhs3(2, g, pre)
        pa = [jnp.where(h0c[0], p0, 0.0), jnp.where(h0c[1], p1, 0.0)]
        pb = [jnp.where(h0c[0], 0.0, p0), jnp.where(h0c[1], 0.0, p1)]
        def stack(x):
            mm = jnp.where(row96 < 8, x[0][0:16], x[1][0:16])
            return jnp.concatenate([mm, x[0][16:48], x[1][16:48]], axis=0).astype(bf16)
        o0 = _dot(stack(pa), r0)
        o2 = _dot(stack(pb), r2)
        t0 = _dot(p0.astype(bf16), rt0)
        t1 = _dot(p1.astype(bf16), rt1)
        om = jnp.where(row16[:, 0:128] < 8, t0[0:16], t1[0:16])
        o1 = jnp.concatenate([om, t0[16:48], t1[16:48]], axis=0)
        o_ref[g] = _pk(jnp.concatenate([o0, o1, o2], axis=1))

    rC = jax.lax.broadcasted_iota(jnp.int32, (16, 128), 0)
    bsc = (BDH ** -0.5) * LOG2E

    def b_qkv():
        y = _dot(_ln(xb_ref[...]).astype(bf16), _up(bqkv_p[...]))
        bq_ref[...] = y[:, 0:D]
        for l in range(2):
            kb_ref[l, 16:48, :] = y[32 * l:32 * l + 32, D:2 * D]
            vb_ref[l, 16:48, :] = y[32 * l:32 * l + 32, 2 * D:3 * D]
    def b_attn(t, l, r0, nr):
        q = bq_ref[32 * l + r0:32 * l + r0 + nr, :]
        seg = t - 1 - 2 * l
        pos = seg * SEG + r0 + rC[0:nr]
        lg = []
        for w in range(BW):
            off = 16 - BDIL * w + r0
            pr = q * kb_ref[l, off:off + nr, :]
            a = pr[:, 0:128] + pr[:, 128:256] + pr[:, 256:384] + pr[:, 384:512] + pr[:, 512:640]
            a = a + pltpu.roll(a, 64, 1)
            a = a + pltpu.roll(a, 32, 1)
            a = a * bsc
            if w > 0:
                a = jnp.where(pos >= BDIL * w, a, NEG)
            lg.append(a)
        m = lg[0]
        for w in range(1, BW): m = jnp.maximum(m, lg[w])
        ps = [jnp.exp2(a - m) for a in lg]
        den = ps[0]
        for w in range(1, BW): den = den + ps[w]
        inv = _recip(den)
        acc = None
        for w in range(BW):
            off = 16 - BDIL * w + r0
            pw = ps[w] * inv
            pw5 = jnp.concatenate([pw] * 5, axis=1)
            tt = pw5 * vb_ref[l, off:off + nr, :]
            acc = tt if acc is None else acc + tt
        bo_ref[32 * l + r0:32 * l + r0 + nr, :] = acc
        z = acc[0:8, 0:128]
        for rr_ in range(nr // 8):
            for cc_ in range(5):
                if rr_ or cc_: z = jnp.maximum(z, acc[8 * rr_:8 * rr_ + 8, 128 * cc_:128 * cc_ + 128])
        return z
    def b_hist():
        for l in range(2):
            kb_ref[l, 0:16, :] = kb_ref[l, 32:48, :]
            vb_ref[l, 0:16, :] = vb_ref[l, 32:48, :]
    def b_out(l):
        return xb_ref[32 * l:32 * l + 32, :] + _dot(bo_ref[32 * l:32 * l + 32, :].astype(bf16), _up(bwo_p[...]))
    def b1_finish(t):
        x2 = b_out(0)
        xn = x_ref[pl.ds(pl.multiple_of(jnp.minimum(t + 1, NSEG - 1) * SEG, SEG), SEG), :].astype(f32)
        xan_ref[0:SEG, :] = xn
        xan_ref[SEG:2 * SEG, :] = x2
        hn_ref[0:16, :] = _pk(_ln(xn))
        hn_ref[16:32, :] = _pk(_ln(x2))
    def b2_finish(t):
        x4 = b_out(1)
        out_ref[pl.ds(pl.multiple_of(jnp.maximum(t - 3, 0) * SEG, SEG), SEG), :] = x4.astype(bf16)
    def wo_part(g0, g1, half=False):
        o = jnp.concatenate([_up(o_ref[g, 0:24, :] if half else o_ref[g]) for g in range(g0, g1)], axis=1)
        return _dot(o, _up(wo[g0 * PW // 2:g1 * PW // 2, :]))

    def step_body(t, var):
        st = {}
        pp = {}
        half = var == 'half'
        lh = jnp.where(t < 2, 0, 1) if half else None
        bias_h = smask(lh) if half else None
        pre = jnp.clip(t - 2, 0, NPRE - 1) if var == 'v64' else None
        def ex(i, pos):
            for name in SCHED.get((i, pos), ()): run_extra(name, t, st, half)
        for i in range(-2, NPAIR):
            g2, g1, g0 = i + 2, i + 1, i
            ex(i, 'pre')
            if g2 < NPAIR: proj(g2, 0, var, lh)
            ex(i, 'q')
            if g2 < NPAIR: proj(g2, 1, var, lh)
            ex(i, 'k')
            if g2 < NPAIR: proj(g2, 2, var, lh)
            ex(i, 'v')
            if 0 <= g1 < NPAIR:
                if half:
                    pp[g1] = [sm(qk(g1, None), bias_h)]
                elif HYB:
                    s_ = qk2(g1, pre)
                    pp[g1] = [sm2(s_[0], bias[0], h0c[0]), sm2(s_[1], bias[1], h0c[1])]
                else:
                    s_ = [qk(g1, 0, pre), qk(g1, 1, pre)]
                    pp[g1] = [sm(s_[0], bias[0]), sm(s_[1], bias[1])]
            if 0 <= g0:
                pg = pp.pop(g0)
                for (l_, r0_, nr_) in BDEP.get(g0, ()):
                    z = b_attn(t, l_, r0_, nr_)
                    p0 = jnp.where(t < 0, z[:, 0:96].astype(pg[0].dtype), pg[0][0:8])
                    pg[0] = jnp.concatenate([p0, pg[0][8:]], axis=0)
                if HYB and not half: pv2(g0, pg, pre)
                else: pv(g0, pg, pre)
            ex(i, 'post')
        end_step(t, st['oa'], lh)

    def step(t, c):
        @pl.when(t == 1)
        def _():
            cp_x1.wait()
        is_half = (t < 2) | (t >= NSEG)
        is_v64 = (t >= 2) & (t < NPRE + 2)
        pl.when(is_half)(lambda: step_body(t, 'half'))
        pl.when(is_v64)(lambda: step_body(t, 'v64'))
        pl.when(jnp.logical_not(is_half | is_v64))(lambda: step_body(t, 'full'))
        @pl.when(t >= 3)
        def _():
            cp_out(jnp.maximum(t - 3, 0)).start()
        return c

    def end_step(t, oa, lh=None):
        if lh is None:
            xb_ref[...] = xa_ref[...] + oa[16:80]
        else:
            sl = pl.ds(pl.multiple_of(SEG * lh, SEG), SEG) if not isinstance(lh, int) else pl.ds(SEG * lh, SEG)
            xb_ref[sl, :] = xa_ref[sl, :] + oa[16:48]
        xa_ref[...] = xan_ref[...]
        r16 = jax.lax.broadcasted_iota(jnp.int32, (16, D), 0)
        memn = jnp.where((r16 >= 8) & (t < 2), mem00, oa[0:16])
        h_ref[0:8, :] = _pk(memn)

    def run_extra(name, t, st, half):
        if name == 'bqkv': b_qkv()
        elif name[0] == 'battn': b_attn(t, name[1], name[2], name[3])
        elif name == 'bhist': b_hist()
        elif name == 'hcopy': h_ref[8:40, :] = hn_ref[...]
        elif name == 'b1fin': b1_finish(t)
        elif name == 'b2fin': b2_finish(t)
        elif name[0] == 'wo':
            part = wo_part(name[1], name[2], half)
            st['oa'] = part if 'oa' not in st else st['oa'] + part
        else: raise ValueError(name)

    def wproj(g, j):
        sl = pl.ds(pl.multiple_of(g * RW, RW), RW)
        y = _pk(_dot_nt(_up(hp_ref[...]), _up(ws[j][sl, :])))
        qkv_ref[g, j, 0:24, :] = y[0:24]
        pre_ref[g, j] = y[24:]
    for j in range(3): qkv_ref[0, j, 0:24, :] = jnp.zeros((24, PW), u32)
    cp_bqkv.wait()
    def pair0(g, c):
        gp = jnp.maximum(g - 1, 0)
        for j in range(3): cp_w(j, g).wait()
        vb = bd(rows(2, gp, None))
        p = sm(qk(gp, None), bias[0])
        wproj(g, 0); wproj(g, 1)
        o_ref[gp, 0:24, :] = _pk(_dot(p, vb))
        wproj(g, 2)
        for k_ in range(8): perm_unit(jnp.minimum(8 * g + k_, 119))
        return c
    jax.lax.fori_loop(0, NPAIR, pair0, 0, unroll=WUNROLL)
    pv(NPAIR - 1, [sm(qk(NPAIR - 1, None), bias[0])])
    xan_ref[0:48, :] = jnp.zeros((48, D), f32)
    def wo0(i, c):
        cp_wo(i).wait()
        GP = NPAIR // NWO
        o = jnp.concatenate([_up(o_ref[i * GP + g, 0:24, :]) for g in range(GP)], axis=1)
        xan_ref[0:48, :] += _dot(o, _up(wo[pl.ds(pl.multiple_of(i * RO, RO), RO), :]))
        return c
    jax.lax.fori_loop(0, NWO, wo0, 0)
    oa = xan_ref[0:48, :]
    xn = x_ref[SEG:2 * SEG, :].astype(f32)
    xan_ref[0:SEG, :] = xn
    xan_ref[SEG:2 * SEG, :] = jnp.zeros((SEG, D), f32)
    h_ref[8:24, :] = _pk(_ln(xn))
    end_step(0, oa, 0)

    jax.lax.fori_loop(1, nsteps, step, 0, unroll=UNROLL)
    b_qkv()
    for c_ in range(2): b_attn(NSEG + 2, 1, 16 * c_, 16)
    b2_finish(NSEG + 2)
    cp_out(NSEG - 1).start()
    def wait_out(s, c):
        cp_out(s).wait()
        return c
    jax.lax.fori_loop(0, min(nsteps - 3, NSEG - 1) + 1 if nsteps > 3 else 1, wait_out, 0)

@functools.partial(jax.jit, static_argnames=("A_seg_len",))
def pallas_interleave_layers__memory_aug_recurrent_mem_tr__sliding_local_dilated__prompt_kernel(
        A_x, A_mem0, A_Wq, A_Wk, A_Wv, A_Wo, A_seg_len, B_x, B_wqkv, B_wo):
    assert A_seg_len == SEG
    del B_x
    nsteps = NSEG + 2
    x = A_x.reshape(S, D)
    mem0 = A_mem0.reshape(M, D)
    tr = lambda w: jnp.transpose(w, (1, 2, 0)).reshape(H * DH, D)
    wo = A_Wo.reshape(H * DH, D)
    hbm = pl.BlockSpec(memory_space=pl.ANY)
    out = pl.pallas_call(
        functools.partial(kernel, nsteps),
        out_shape=jax.ShapeDtypeStruct((S, D), bf16),
        in_specs=[hbm] * 8,
        out_specs=hbm,
        scratch_shapes=[
            pltpu.VMEM((H * DH // 2, D), u32), pltpu.VMEM((H * DH // 2, D), u32), pltpu.VMEM((H * DH // 2, D), u32), pltpu.VMEM((H * DH // 2, D), u32),
            pltpu.VMEM((D // 2, 3 * D), u32), pltpu.VMEM((D, D), bf16),
            pltpu.VMEM((D // 2, 3 * D), u32), pltpu.VMEM((D // 2, D), u32),
            pltpu.VMEM((S, D), bf16), pltpu.VMEM((M, D), bf16), pltpu.VMEM((S, D), bf16),
            pltpu.VMEM((40, D), u32), pltpu.VMEM((NPAIR, 3, 40, PW), u32), pltpu.VMEM((NPAIR, 40, PW), u32),
            pltpu.VMEM((64, D), f32), pltpu.VMEM((64, D), f32),
            pltpu.VMEM((2, 48, D), f32), pltpu.VMEM((2, 48, D), f32),
            pltpu.VMEM((64, D), f32), pltpu.VMEM((64, D), f32), pltpu.VMEM((64, D), f32),
            pltpu.VMEM((32, D), u32),
            pltpu.VMEM((24 + 8 * NPRE, D), u32), pltpu.VMEM((NPAIR, 3, 8 * NPRE, PW), u32), pltpu.VMEM((5, D, 128), f32),
            pltpu.SemaphoreType.DMA((NPAIR,)), pltpu.SemaphoreType.DMA((9,)), pltpu.SemaphoreType.DMA((1,)),
        ],
        compiler_params=pltpu.CompilerParams(vmem_limit_bytes=100 * 1024 * 1024),
    )(x, mem0, tr(A_Wq), tr(A_Wk), tr(A_Wv), wo, B_wqkv, B_wo)
    return out.reshape(1, S, D)
```

```python
import functools
import jax
import jax.numpy as jnp
import numpy as np
from jax.experimental import pallas as pl
from jax.experimental.pallas import tpu as pltpu

S = 2048; D = 640; H = 32; DH = 192; M = 8; SEG = 32; NSEG = S // SEG
NPAIR = H // 2; PW = 2 * DH
BH = 32; BDH = D // BH; BW = 8; BDIL = 2
LOG2E = 1.4426950408889634
NEG = -1e30
f32 = jnp.float32; bf16 = jnp.bfloat16; u32 = jnp.uint32

SCHED = {
    (0, 'post'): ['bqkv'],
    (12, 'post'): ['bhist'],
    (8, 'post'): ['b1fin'],
    (13, 'post'): ['hcopy', ('wo', 0, 5)],
    (14, 'k'): [('wo', 5, 10)],
    (14, 'post'): [('wo', 10, 14)],
    (15, 'post'): [('wo', 14, 16), 'b2fin'],
}
BDEP = {2: [(0, 0, 8)], 4: [(0, 8, 8)], 6: [(0, 16, 8)], 7: [(0, 24, 8)], 9: [(1, 0, 8)], 10: [(1, 8, 8)], 11: [(1, 16, 8)], 12: [(1, 24, 8)]}
NPRE = 18
WUNROLL = 1
HYB = 1
HALF = 1
UNROLL = 1
ORDER = 'qkvSP'

def _dot(a, b):
    return jnp.dot(a, b, preferred_element_type=f32)
def _dot_nt(a, b):
    return lax_dot(a, b, (((1,), (1,)), ((), ())))
def lax_dot(a, b, dn):
    return jax.lax.dot_general(a, b, dn, preferred_element_type=f32)

def _recip(x):
    r = pl.reciprocal(x, approx=True)
    return r * (2.0 - x * r)

def _ln(x):
    m = jnp.mean(x, axis=-1, keepdims=True)
    xc = x - m
    v = jnp.mean(xc * xc, axis=-1, keepdims=True)
    return xc * jax.lax.rsqrt(v + 1e-5)

def _perm_mat():
    r = jax.lax.broadcasted_iota(jnp.int32, (D, D), 0)
    c = jax.lax.broadcasted_iota(jnp.int32, (D, D), 1)
    h = c % BH
    d = c // BH
    return (r == h * BDH + d).astype(bf16)

def _pk(x):
    return pltpu.bitcast(x.astype(bf16), u32)
def _up(x):
    return pltpu.bitcast(x, bf16)

def kernel(nsteps, x_hbm, mem0_hbm, wq_hbm, wk_hbm, wv_hbm, wo_hbm, bqkv_hbm, bwo_hbm, out_hbm,
           wq, wk, wv, wo, bqkv_raw, bwo_raw, bqkv_p, bwo_p, x_ref, mem0_ref, out_ref,
           h_ref, qkv_ref, o_ref, xa_ref, xb_ref, kb_ref, vb_ref, xan_ref, bq_ref, bo_ref, hn_ref, hp_ref, pre_ref,
           sem_w, sem_m, sem_o, sem_b):
    RW = PW // 2
    ws = (wq, wk, wv)
    ws_hbm = (wq_hbm.bitcast(u32), wk_hbm.bitcast(u32), wv_hbm.bitcast(u32))
    NWO = 4
    RO = H * DH // 2 // NWO
    def cp_w(j, g):
        sl = pl.ds(pl.multiple_of(g * RW, RW), RW) if not isinstance(g, int) else pl.ds(g * RW, RW)
        return pltpu.make_async_copy(ws_hbm[j].at[sl], ws[j].at[sl], sem_w.at[g])
    X0R = (NPRE + 2) * SEG
    cp_x0 = pltpu.make_async_copy(x_hbm.at[0:X0R], x_ref.at[0:X0R], sem_m.at[0])
    cp_mem = pltpu.make_async_copy(mem0_hbm, mem0_ref, sem_m.at[1])
    BQR = (0, 104, 208, 320)
    cp_bqkv = [pltpu.make_async_copy(bqkv_hbm.bitcast(u32).at[BQR[i_]:BQR[i_ + 1]], bqkv_raw.at[BQR[i_]:BQR[i_ + 1]], sem_b.at[i_])
               for i_ in range(3)]
    cp_bwo = [pltpu.make_async_copy(bwo_hbm.bitcast(u32).at[:, k_ * 128:(k_ + 1) * 128], bwo_raw.at[k_, 0:D // 2, :], sem_b.at[3 + k_])
              for k_ in range(5)]
    def cp_wo(i):
        sl = pl.ds(pl.multiple_of(i * RO, RO), RO) if not isinstance(i, int) else pl.ds(i * RO, RO)
        return pltpu.make_async_copy(wo_hbm.bitcast(u32).at[sl], wo.at[sl], sem_m.at[4 + i])
    cp_x1 = pltpu.make_async_copy(x_hbm.at[X0R:S], x_ref.at[X0R:S], sem_m.at[4 + NWO])
    def cp_out(s):
        sl = pl.ds(pl.multiple_of(s * SEG, SEG), SEG) if not isinstance(s, int) else pl.ds(s * SEG, SEG)
        return pltpu.make_async_copy(out_ref.at[sl], out_hbm.at[sl], sem_o.at[0])

    cp_x0.start(); cp_mem.start()
    for g in range(NPAIR):
        if g == 3: cp_bqkv[0].start()
        if g == 5:
            for c_ in cp_bwo: c_.start()
        if g == 6: cp_bqkv[1].start()
        if g == 9: cp_bqkv[2].start()
        for j in range(3): cp_w(j, g).start()
    for i_ in range(NWO): cp_wo(i_).start()
    cp_x1.start()

    bqkv_raw[D // 2:D // 2 + 8, :] = jnp.zeros((8, 3 * D), u32)
    for k_ in range(5): bwo_raw[k_, D // 2:D, :] = jnp.zeros((D // 2, 128), u32)
    xb_ref[...] = jnp.zeros((2 * SEG, D), f32)
    kb_ref[...] = jnp.zeros(kb_ref.shape, f32)
    vb_ref[...] = jnp.zeros(vb_ref.shape, f32)
    xa_ref[SEG:2 * SEG, :] = jnp.zeros((SEG, D), f32)
    h_ref[24:40, :] = jnp.zeros((16, D), u32)
    cp_x0.wait(); cp_mem.wait()
    mem0 = mem0_ref[...]
    mem00 = jnp.concatenate([mem0.astype(f32), mem0.astype(f32)], axis=0)
    h_ref[0:8, :] = _pk(mem00)
    x00 = x_ref[0:SEG, :].astype(f32)
    h_ref[8:24, :] = _pk(_ln(x00))
    xa_ref[0:SEG, :] = x00
    hp_ref[0:8, :] = _pk(mem00)
    hp_ref[8:24, :] = _pk(_ln(x00))
    for i_ in range(NPRE):
        hp_ref[24 + 8 * i_:32 + 8 * i_, :] = _pk(_ln(x_ref[(i_ + 2) * SEG:(i_ + 2) * SEG + 16, :].astype(f32)))

    def perm_wo_unit(e, valid):
        base = jnp.where(valid, e, D // 2)
        w = jnp.concatenate([bwo_raw[k_, pl.ds(base, BH, stride=BDH // 2), :] for k_ in range(5)], axis=1)
        lo = pltpu.bitcast(w << 16, f32)
        hi = pltpu.bitcast(w & jnp.uint32(0xFFFF0000), f32)
        dst = pl.multiple_of(jnp.where(valid, e * BH, D // 2), BH)
        bwo_p[pl.ds(dst, BH // 2), :] = _pk(lo)
        bwo_p[pl.ds(dst + BH // 2, BH // 2), :] = _pk(hi)
    lane8 = jax.lax.broadcasted_iota(jnp.int32, (8, 128), 1)
    def perm_unit(u, valid):
        rg = u // 3
        j = u - 3 * rg
        r = pl.ds(pl.multiple_of(jnp.where(valid, rg * 8, D // 2), 8), 8)
        srcs = [bqkv_raw[r, pl.ds(pl.multiple_of(j * D + k_ * 128, 128), 128)] for k_ in range(5)]
        for n in range(5):
            col = lane8 + n * 128
            s = (col % BH) * BDH + col // BH
            acc = None
            for k_ in range(5):
                g_ = jnp.take_along_axis(srcs[k_], s % 128, axis=1)
                acc = g_ if acc is None else jnp.where(s // 128 == k_, g_, acc)
            bqkv_p[r, pl.ds(pl.multiple_of(j * D + n * 128, 128), 128)] = acc

    lane = jax.lax.broadcasted_iota(jnp.int32, (48, 128), 1)
    lo64 = lane < 64
    rr = jax.lax.broadcasted_iota(jnp.int32, (48, 96), 0)
    cc = jax.lax.broadcasted_iota(jnp.int32, (48, 96), 1)
    ck = jnp.where(cc >= 48, cc - 48, cc)
    first = cc < 48
    def smask(l):
        memk = (ck >= 8 * l) & (ck < 8 * l + 8)
        tokk = (ck >= 16) & ((rr < 16) | (ck <= rr))
        return jnp.where(memk | tokk, 0.0, NEG).astype(f32)
    bias = [smask(0), smask(1)]
    row16 = jax.lax.broadcasted_iota(jnp.int32, (16, PW), 0)
    sc = (DH ** -0.5) * LOG2E

    def bd(a):
        z = jnp.zeros((48, 128), bf16)
        a0, a1, a2 = a[:, 0:128], a[:, 128:256], a[:, 256:384]
        top = jnp.concatenate([a0, jnp.where(lo64, a1, z), z], axis=1)
        bot = jnp.concatenate([z, jnp.where(lo64, z, a1), a2], axis=1)
        return jnp.concatenate([top, bot], axis=0)

    def lhs_h(var, lh):
        if var == 'full':
            return _up(h_ref[...])
        if var == 'v64':
            return _up(jnp.concatenate([h_ref[0:8, :], h_ref[16:40, :]], axis=0))
        return _up(jnp.concatenate([h_ref[0:8, :], h_ref[pl.ds(pl.multiple_of(8 + 16 * lh, 8), 16), :]], axis=0))
    def proj(g, j, var='full', lh=None):
        sl = pl.ds(pl.multiple_of(g * RW, RW), RW) if not isinstance(g, int) else pl.ds(g * RW, RW)
        y = _pk(_dot_nt(lhs_h(var, lh), _up(ws[j][sl, :])))
        if var == 'full': qkv_ref[g, j] = y
        elif var == 'v64':
            qkv_ref[g, j, 0:8, :] = y[0:8]
            qkv_ref[g, j, 16:40, :] = y[8:32]
        else: qkv_ref[g, j, 0:24, :] = y
    def rows(j, g, l, pre=None):
        if l is None: return _up(qkv_ref[g, j, 0:24, :])
        if l == 0 and pre is not None:
            return jnp.concatenate([_up(qkv_ref[g, j, 0:8, :]), _up(pre_ref[g, j, pl.ds(pl.multiple_of(8 * pre, 8), 8), :]),
                                    _up(qkv_ref[g, j, 16:24, :])], axis=0)
        return jnp.concatenate([_up(qkv_ref[g, j, 0:8, :]), _up(qkv_ref[g, j, 8 + 16 * l:24 + 16 * l, :])], axis=0)
    def qk(g, l, pre=None):
        return _dot_nt(rows(0, g, l, pre), bd(rows(1, g, l, pre)))
    def sm(s, bias_l):
        s = s * sc + bias_l
        m0 = jnp.max(jnp.where(first, s, NEG), axis=1, keepdims=True)
        m1 = jnp.max(jnp.where(first, NEG, s), axis=1, keepdims=True)
        p = jnp.exp2(s - jnp.where(first, m0, m1))
        s0 = jnp.sum(jnp.where(first, p, 0.0), axis=1, keepdims=True)
        s1 = jnp.sum(jnp.where(first, 0.0, p), axis=1, keepdims=True)
        p = p * _recip(jnp.where(first, s0, s1))
        return p.astype(bf16)
    def pv(g, ps, pre=None):
        if len(ps) == 1:
            o_ref[g, 0:24, :] = _pk(_dot(ps[0], bd(rows(2, g, None))))
            return
        os_ = [_dot(ps[l], bd(rows(2, g, l, pre))) for l in range(2)]
        om = jnp.where(row16 < 8, os_[0][0:16], os_[1][0:16])
        o = jnp.concatenate([om, os_[0][16:48], os_[1][16:48]], axis=0)
        o_ref[g] = _pk(o)

    h0c = [cc < 48, (cc < 16) | (cc >= 64)]
    row96 = jax.lax.broadcasted_iota(jnp.int32, (16, 96), 0)
    def parts(j, g, pre):
        m_ = _up(qkv_ref[g, j, 0:8, :])
        if pre is None:
            t1 = _up(qkv_ref[g, j, 8:24, :])
        else:
            t1 = jnp.concatenate([_up(pre_ref[g, j, pl.ds(pl.multiple_of(8 * pre, 8), 8), :]), _up(qkv_ref[g, j, 16:24, :])], axis=0)
        t2 = _up(qkv_ref[g, j, 24:40, :])
        return m_, t1, t2
    def lo_(a): return jnp.where(lo64[0:a.shape[0]], a, jnp.zeros_like(a))
    def hi_(a): return jnp.where(lo64[0:a.shape[0]], jnp.zeros_like(a), a)
    def rhs3(j, g, pre):
        m_, t1, t2 = parts(j, g, pre)
        z16 = jnp.zeros((16, 128), bf16)
        cat = lambda *xs: jnp.concatenate(xs, axis=0)
        r0 = cat(m_[:, 0:128], t1[:, 0:128], z16, t2[:, 0:128])
        r2 = cat(z16, t2[:, 256:384], m_[:, 256:384], t1[:, 256:384])
        m1, a1, b1 = m_[:, 128:256], t1[:, 128:256], t2[:, 128:256]
        rt0 = cat(lo_(m1), lo_(a1), hi_(m1), hi_(a1))
        rt1 = cat(lo_(m1), hi_(b1), hi_(m1), lo_(b1))
        return r0, r2, rt0, rt1
    def qk2(g, pre):
        m_, t1, t2 = parts(0, g, pre)
        q = jnp.concatenate([m_, t1, t2], axis=0)
        r0, r2, rt0, rt1 = rhs3(1, g, pre)
        a0 = _dot_nt(q[:, 0:128], r0)
        a2 = _dot_nt(q[:, 256:384], r2)
        q0 = q[0:48, 128:256]
        q1 = jnp.concatenate([q[0:16, 128:256], q[48:80, 128:256]], axis=0)
        s0 = jnp.where(h0c[0], a0[0:48], a2[0:48]) + _dot_nt(q0, rt0)
        a0l = jnp.concatenate([a0[0:16], a0[48:80]], axis=0)
        a2l = jnp.concatenate([a2[0:16], a2[48:80]], axis=0)
        s1 = jnp.where(h0c[1], a0l, a2l) + _dot_nt(q1, rt1)
        return s0, s1
    def sm2(s, bias_l, hc):
        s = s * sc + bias_l
        m0 = jnp.max(jnp.where(hc, s, NEG), axis=1, keepdims=True)
        m1 = jnp.max(jnp.where(hc, NEG, s), axis=1, keepdims=True)
        p = jnp.exp2(s - jnp.where(hc, m0, m1))
        s0 = jnp.sum(jnp.where(hc, p, 0.0), axis=1, keepdims=True)
        s1 = jnp.sum(jnp.where(hc, 0.0, p), axis=1, keepdims=True)
        return p * _recip(jnp.where(hc, s0, s1))
    def pv2(g, ps, pre):
        p0, p1 = ps
        r0, r2, rt0, rt1 = rhs3(2, g, pre)
        pa = [jnp.where(h0c[0], p0, 0.0), jnp.where(h0c[1], p1, 0.0)]
        pb = [jnp.where(h0c[0], 0.0, p0), jnp.where(h0c[1], 0.0, p1)]
        def stack(x):
            mm = jnp.where(row96 < 8, x[0][0:16], x[1][0:16])
            return jnp.concatenate([mm, x[0][16:48], x[1][16:48]], axis=0).astype(bf16)
        o0 = _dot(stack(pa), r0)
        o2 = _dot(stack(pb), r2)
        t0 = _dot(p0.astype(bf16), rt0)
        t1 = _dot(p1.astype(bf16), rt1)
        om = jnp.where(row16[:, 0:128] < 8, t0[0:16], t1[0:16])
        o1 = jnp.concatenate([om, t0[16:48], t1[16:48]], axis=0)
        o_ref[g] = _pk(jnp.concatenate([o0, o1, o2], axis=1))

    rC = jax.lax.broadcasted_iota(jnp.int32, (16, 128), 0)
    bsc = (BDH ** -0.5) * LOG2E

    def b_qkv(layers=(0, 1)):
        r0 = 32 * layers[0]; r1 = 32 * layers[-1] + 32
        y = _dot(_ln(xb_ref[r0:r1, :]).astype(bf16), _up(bqkv_p[0:D // 2, :]))
        bq_ref[r0:r1, :] = y[:, 0:D]
        for l in layers:
            kb_ref[l, 16:48, :] = y[32 * l - r0:32 * l - r0 + 32, D:2 * D]
            vb_ref[l, 16:48, :] = y[32 * l - r0:32 * l - r0 + 32, 2 * D:3 * D]
    def b_attn(t, l, r0, nr):
        q = bq_ref[32 * l + r0:32 * l + r0 + nr, :]
        seg = t - 1 - 2 * l
        pos = seg * SEG + r0 + rC[0:nr]
        lg = []
        for w in range(BW):
            off = 16 - BDIL * w + r0
            pr = q * kb_ref[l, off:off + nr, :]
            a = pr[:, 0:128] + pr[:, 128:256] + pr[:, 256:384] + pr[:, 384:512] + pr[:, 512:640]
            a = a + pltpu.roll(a, 64, 1)
            a = a + pltpu.roll(a, 32, 1)
            a = a * bsc
            if w > 0:
                a = jnp.where(pos >= BDIL * w, a, NEG)
            lg.append(a)
        m = lg[0]
        for w in range(1, BW): m = jnp.maximum(m, lg[w])
        ps = [jnp.exp2(a - m) for a in lg]
        den = ps[0]
        for w in range(1, BW): den = den + ps[w]
        inv = _recip(den)
        acc = None
        for w in range(BW):
            off = 16 - BDIL * w + r0
            pw = ps[w] * inv
            pw5 = jnp.concatenate([pw] * 5, axis=1)
            tt = pw5 * vb_ref[l, off:off + nr, :]
            acc = tt if acc is None else acc + tt
        bo_ref[32 * l + r0:32 * l + r0 + nr, :] = acc
        z = acc[0:8, 0:128]
        for rr_ in range(nr // 8):
            for cc_ in range(5):
                if rr_ or cc_: z = jnp.maximum(z, acc[8 * rr_:8 * rr_ + 8, 128 * cc_:128 * cc_ + 128])
        return z
    def b_hist():
        for l in range(2):
            kb_ref[l, 0:16, :] = kb_ref[l, 32:48, :]
            vb_ref[l, 0:16, :] = vb_ref[l, 32:48, :]
    def b_out(l):
        return xb_ref[32 * l:32 * l + 32, :] + _dot(bo_ref[32 * l:32 * l + 32, :].astype(bf16), _up(bwo_p[0:D // 2, :]))
    def b1_finish(t):
        x2 = b_out(0)
        xn = x_ref[pl.ds(pl.multiple_of(jnp.minimum(t + 1, NSEG - 1) * SEG, SEG), SEG), :].astype(f32)
        xan_ref[0:SEG, :] = xn
        xan_ref[SEG:2 * SEG, :] = x2
        hn_ref[0:16, :] = _pk(_ln(xn))
        hn_ref[16:32, :] = _pk(_ln(x2))
    def b2_finish(t):
        x4 = b_out(1)
        out_ref[pl.ds(pl.multiple_of(jnp.maximum(t - 3, 0) * SEG, SEG), SEG), :] = x4.astype(bf16)
    def wo_part(g0, g1, half=False):
        o = jnp.concatenate([_up(o_ref[g, 0:24, :] if half else o_ref[g]) for g in range(g0, g1)], axis=1)
        return _dot(o, _up(wo[g0 * PW // 2:g1 * PW // 2, :]))

    def step_body(t, var):
        st = {}
        pp = {}
        half = var == 'half'
        lh = jnp.where(t < 2, 0, 1) if half else None
        bias_h = smask(lh) if half else None
        pre = jnp.clip(t - 2, 0, NPRE - 1) if var == 'v64' else None
        def ex(i, pos):
            for name in SCHED.get((i, pos), ()): run_extra(name, t, st, half)
        for i in range(-2, NPAIR):
            g2, g1, g0 = i + 2, i + 1, i
            def do_proj(j):
                if g2 < NPAIR: proj(g2, j, var, lh)
                ex(i, 'qkv'[j])
            def do_qk():
                if 0 <= g1 < NPAIR:
                    if half:
                        pp[g1] = [sm(qk(g1, None), bias_h)]
                    else:
                        s_ = qk2(g1, pre)
                        pp[g1] = [sm2(s_[0], bias[0], h0c[0]), sm2(s_[1], bias[1], h0c[1])]
            def do_pv():
                if 0 <= g0:
                    pg = pp.pop(g0)
                    for (l_, r0_, nr_) in BDEP.get(g0, ()):
                        z = b_attn(t, l_, r0_, nr_)
                        p0 = jnp.where(t < 0, z[:, 0:96].astype(pg[0].dtype), pg[0][0:8])
                        pg[0] = jnp.concatenate([p0, pg[0][8:]], axis=0)
                    if half: pv(g0, pg, pre)
                    else: pv2(g0, pg, pre)
            ex(i, 'pre')
            for ch in ORDER:
                if ch == 'S': do_qk()
                elif ch == 'P': do_pv()
                else: do_proj('qkv'.index(ch))
            ex(i, 'post')
        end_step(t, st['oa'], lh)

    def step(t, c):
        @pl.when(t == 1)
        def _():
            cp_x1.wait()
        is_half = (t < 2) | (t >= NSEG)
        is_v64 = (t >= 2) & (t < NPRE + 2)
        pl.when(is_half)(lambda: step_body(t, 'half'))
        pl.when(is_v64)(lambda: step_body(t, 'v64'))
        pl.when(jnp.logical_not(is_half | is_v64))(lambda: step_body(t, 'full'))
        @pl.when(t >= 3)
        def _():
            cp_out(jnp.maximum(t - 3, 0)).start()
        return c

    def end_step(t, oa, lh=None):
        if lh is None:
            xb_ref[...] = xa_ref[...] + oa[16:80]
        else:
            sl = pl.ds(pl.multiple_of(SEG * lh, SEG), SEG) if not isinstance(lh, int) else pl.ds(SEG * lh, SEG)
            xb_ref[sl, :] = xa_ref[sl, :] + oa[16:48]
        xa_ref[...] = xan_ref[...]
        r16 = jax.lax.broadcasted_iota(jnp.int32, (16, D), 0)
        memn = jnp.where((r16 >= 8) & (t < 2), mem00, oa[0:16])
        h_ref[0:8, :] = _pk(memn)

    def run_extra(name, t, st, half):
        if name == 'bqkv': b_qkv()
        elif name[0] == 'battn': b_attn(t, name[1], name[2], name[3])
        elif name == 'bhist': b_hist()
        elif name == 'hcopy': h_ref[8:40, :] = hn_ref[...]
        elif name == 'b1fin': b1_finish(t)
        elif name == 'b2fin': b2_finish(t)
        elif name[0] == 'wo':
            part = wo_part(name[1], name[2], half)
            st['oa'] = part if 'oa' not in st else st['oa'] + part
        else: raise ValueError(name)

    def wproj(g, j):
        sl = pl.ds(pl.multiple_of(g * RW, RW), RW)
        y = _pk(_dot_nt(_up(hp_ref[...]), _up(ws[j][sl, :])))
        qkv_ref[g, j, 0:24, :] = y[0:24]
        pre_ref[g, j] = y[24:]
    for j in range(3): qkv_ref[0, j, 0:24, :] = jnp.zeros((24, PW), u32)
    def pair0(g, c):
        gp = jnp.maximum(g - 1, 0)
        for i_, g_ in enumerate((3, 6, 10)):
            pl.when(g == g_)(cp_bqkv[i_].wait)
        @pl.when(g == 6)
        def _():
            for c_ in cp_bwo: c_.wait()
        for j in range(3): cp_w(j, g).wait()
        vb = bd(rows(2, gp, None))
        p = sm(qk(gp, None), bias[0])
        wproj(g, 0); wproj(g, 1)
        o_ref[gp, 0:24, :] = _pk(_dot(p, vb))
        wproj(g, 2)
        for k_ in range(10): perm_unit(jnp.clip(10 * (g - 3) + k_, 0, 119), g >= 3)
        perm_wo_unit(jnp.clip(g - 6, 0, 9), g >= 6)
        return c
    jax.lax.fori_loop(0, NPAIR, pair0, 0, unroll=WUNROLL)
    pv(NPAIR - 1, [sm(qk(NPAIR - 1, None), bias[0])])
    for i_ in range(NWO): cp_wo(i_).wait()
    oa = wo_part(0, NPAIR, True)
    xn = x_ref[SEG:2 * SEG, :].astype(f32)
    xan_ref[0:SEG, :] = xn
    xan_ref[SEG:2 * SEG, :] = jnp.zeros((SEG, D), f32)
    h_ref[8:24, :] = _pk(_ln(xn))
    end_step(0, oa, 0)

    jax.lax.fori_loop(1, nsteps, step, 0, unroll=UNROLL)
    b_qkv((1,))
    for c_ in range(2): b_attn(NSEG + 2, 1, 16 * c_, 16)
    b2_finish(NSEG + 2)
    cp_out(NSEG - 1).start()
    def wait_out(s, c):
        cp_out(s).wait()
        return c
    jax.lax.fori_loop(0, min(nsteps - 3, NSEG - 1) + 1 if nsteps > 3 else 1, wait_out, 0)

@functools.partial(jax.jit, static_argnames=("A_seg_len",))
def pallas_interleave_layers__memory_aug_recurrent_mem_tr__sliding_local_dilated__prompt_kernel(
        A_x, A_mem0, A_Wq, A_Wk, A_Wv, A_Wo, A_seg_len, B_x, B_wqkv, B_wo):
    assert A_seg_len == SEG
    del B_x
    nsteps = NSEG + 2
    x = A_x.reshape(S, D)
    mem0 = A_mem0.reshape(M, D)
    tr = lambda w: jnp.transpose(w, (1, 2, 0)).reshape(H * DH, D)
    wo = A_Wo.reshape(H * DH, D)
    hbm = pl.BlockSpec(memory_space=pl.ANY)
    out = pl.pallas_call(
        functools.partial(kernel, nsteps),
        out_shape=jax.ShapeDtypeStruct((S, D), bf16),
        in_specs=[hbm] * 8,
        out_specs=hbm,
        scratch_shapes=[
            pltpu.VMEM((H * DH // 2, D), u32), pltpu.VMEM((H * DH // 2, D), u32), pltpu.VMEM((H * DH // 2, D), u32), pltpu.VMEM((H * DH // 2, D), u32),
            pltpu.VMEM((D // 2 + 8, 3 * D), u32), pltpu.VMEM((5, D, 128), u32),
            pltpu.VMEM((D // 2 + 8, 3 * D), u32), pltpu.VMEM((D // 2 + 32, D), u32),
            pltpu.VMEM((S, D), bf16), pltpu.VMEM((M, D), bf16), pltpu.VMEM((S, D), bf16),
            pltpu.VMEM((40, D), u32), pltpu.VMEM((NPAIR, 3, 40, PW), u32), pltpu.VMEM((NPAIR, 40, PW), u32),
            pltpu.VMEM((64, D), f32), pltpu.VMEM((64, D), f32),
            pltpu.VMEM((2, 48, D), f32), pltpu.VMEM((2, 48, D), f32),
            pltpu.VMEM((64, D), f32), pltpu.VMEM((64, D), f32), pltpu.VMEM((64, D), f32),
            pltpu.VMEM((32, D), u32),
            pltpu.VMEM((24 + 8 * NPRE, D), u32), pltpu.VMEM((NPAIR, 3, 8 * NPRE, PW), u32),
            pltpu.SemaphoreType.DMA((NPAIR,)), pltpu.SemaphoreType.DMA((9,)), pltpu.SemaphoreType.DMA((1,)), pltpu.SemaphoreType.DMA((8,)),
        ],
        compiler_params=pltpu.CompilerParams(vmem_limit_bytes=100 * 1024 * 1024),
    )(x, mem0, tr(A_Wq), tr(A_Wk), tr(A_Wv), wo, B_wqkv, B_wo)
    return out.reshape(1, S, D)
```

```python
import functools
import jax
import jax.numpy as jnp
import numpy as np
from jax.experimental import pallas as pl
from jax.experimental.pallas import tpu as pltpu

S = 2048; D = 640; H = 32; DH = 192; M = 8; SEG = 32; NSEG = S // SEG
NPAIR = H // 2; PW = 2 * DH
BH = 32; BDH = D // BH; BW = 8; BDIL = 2
LOG2E = 1.4426950408889634
NEG = -1e30
f32 = jnp.float32; bf16 = jnp.bfloat16; u32 = jnp.uint32

def _sched(bq, b1, bh, hc, cuts, wpos, b2):
    s = {}
    s.setdefault(bq, []).append('bqkv')
    s.setdefault((b1, 'post'), []).append('b1fin')
    s.setdefault((bh, 'post'), []).append('bhist')
    s.setdefault((hc, 'post'), []).append('hcopy')
    cs = [0] + list(cuts) + [NPAIR]
    for (g0, g1), p in zip(zip(cs, cs[1:]), wpos):
        s.setdefault(p, []).append(('wo', g0, g1))
    s.setdefault(b2, []).append('b2fin')
    return s
def _bdep(l0, l1):
    d = {}
    for i, g in enumerate(l0): d.setdefault(g, []).append((0, 8 * i, 8))
    for i, g in enumerate(l1): d.setdefault(g, []).append((1, 8 * i, 8))
    return d
_WP = ((13, 'post'), (14, 'k'), (14, 'post'), (15, 'post'))
SCHED = {
    'half': _sched((0, 'pre'), 8, 11, 13, (4, 8, 13), _WP, (15, 'post')),
    'v64': _sched((0, 'post'), 8, 11, 13, (4, 8, 13), _WP, (15, 'post')),
    'full': _sched((0, 'post'), 8, 12, 13, (4, 8, 13), _WP, (15, 'post')),
}
BDEP = {
    'half': _bdep((3, 4, 5, 7), (9, 10, 11, 11)),
    'v64': _bdep((3, 5, 7, 8), (9, 10, 11, 11)),
    'full': _bdep((3, 4, 5, 7), (9, 10, 11, 12)),
}
ORDER = 'qkvSP'
ORDER = 'qkvSP'
NPRE = 18

def _dot(a, b):
    return jnp.dot(a, b, preferred_element_type=f32)
def _dot_nt(a, b):
    return lax_dot(a, b, (((1,), (1,)), ((), ())))
def lax_dot(a, b, dn):
    return jax.lax.dot_general(a, b, dn, preferred_element_type=f32)

def _recip(x):
    r = pl.reciprocal(x, approx=True)
    return r * (2.0 - x * r)

def _ln(x):
    m = jnp.mean(x, axis=-1, keepdims=True)
    xc = x - m
    v = jnp.mean(xc * xc, axis=-1, keepdims=True)
    return xc * jax.lax.rsqrt(v + 1e-5)

def _perm_mat():
    r = jax.lax.broadcasted_iota(jnp.int32, (D, D), 0)
    c = jax.lax.broadcasted_iota(jnp.int32, (D, D), 1)
    h = c % BH
    d = c // BH
    return (r == h * BDH + d).astype(bf16)

def _pk(x):
    return pltpu.bitcast(x.astype(bf16), u32)
def _up(x):
    return pltpu.bitcast(x, bf16)

def kernel(nsteps, x_hbm, mem0_hbm, wq_hbm, wk_hbm, wv_hbm, wo_hbm, bqkv_hbm, bwo_hbm, out_hbm,
           wq, wk, wv, wo, bqkv_raw, bwo_raw, bqkv_p, bwo_p, x_ref, mem0_ref, out_ref,
           h_ref, qkv_ref, o_ref, xa_ref, xb_ref, kb_ref, vb_ref, xan_ref, bq_ref, bo_ref, hn_ref, hp_ref, pre_ref,
           sem_w, sem_m, sem_o, sem_b):
    RW = PW // 2
    ws = (wq, wk, wv)
    ws_hbm = (wq_hbm.bitcast(u32), wk_hbm.bitcast(u32), wv_hbm.bitcast(u32))
    NWO = 4
    RO = H * DH // 2 // NWO
    def cp_w(j, g):
        sl = pl.ds(pl.multiple_of(g * RW, RW), RW) if not isinstance(g, int) else pl.ds(g * RW, RW)
        return pltpu.make_async_copy(ws_hbm[j].at[sl], ws[j].at[sl], sem_w.at[g])
    X0R = (NPRE + 2) * SEG
    cp_x0 = pltpu.make_async_copy(x_hbm.at[0:X0R], x_ref.at[0:X0R], sem_m.at[0])
    cp_mem = pltpu.make_async_copy(mem0_hbm, mem0_ref, sem_m.at[1])
    BQR = (0, 104, 208, 320)
    cp_bqkv = [pltpu.make_async_copy(bqkv_hbm.bitcast(u32).at[BQR[i_]:BQR[i_ + 1]], bqkv_raw.at[BQR[i_]:BQR[i_ + 1]], sem_b.at[i_])
               for i_ in range(3)]
    cp_bwo = [pltpu.make_async_copy(bwo_hbm.bitcast(u32).at[:, k_ * 128:(k_ + 1) * 128], bwo_raw.at[k_, 0:D // 2, :], sem_b.at[3 + k_])
              for k_ in range(5)]
    def cp_wo(i):
        sl = pl.ds(pl.multiple_of(i * RO, RO), RO) if not isinstance(i, int) else pl.ds(i * RO, RO)
        return pltpu.make_async_copy(wo_hbm.bitcast(u32).at[sl], wo.at[sl], sem_m.at[4 + i])
    cp_x1 = pltpu.make_async_copy(x_hbm.at[X0R:S], x_ref.at[X0R:S], sem_m.at[4 + NWO])
    def cp_out(s):
        sl = pl.ds(pl.multiple_of(s * SEG, SEG), SEG) if not isinstance(s, int) else pl.ds(s * SEG, SEG)
        return pltpu.make_async_copy(out_ref.at[sl], out_hbm.at[sl], sem_o.at[0])

    cp_x0.start(); cp_mem.start()
    for g in range(NPAIR):
        if g == 3: cp_bqkv[0].start()
        if g == 5:
            for c_ in cp_bwo: c_.start()
        if g == 6: cp_bqkv[1].start()
        if g == 9: cp_bqkv[2].start()
        for j in range(3): cp_w(j, g).start()
    for i_ in range(NWO): cp_wo(i_).start()
    cp_x1.start()

    bqkv_raw[D // 2:D // 2 + 8, :] = jnp.zeros((8, 3 * D), u32)
    for k_ in range(5): bwo_raw[k_, D // 2:D, :] = jnp.zeros((D // 2, 128), u32)
    xb_ref[...] = jnp.zeros((2 * SEG, D), f32)
    kb_ref[...] = jnp.zeros(kb_ref.shape, f32)
    vb_ref[...] = jnp.zeros(vb_ref.shape, f32)
    xa_ref[SEG:2 * SEG, :] = jnp.zeros((SEG, D), f32)
    h_ref[24:40, :] = jnp.zeros((16, D), u32)
    cp_x0.wait(); cp_mem.wait()
    mem0 = mem0_ref[...]
    mem00 = jnp.concatenate([mem0.astype(f32), mem0.astype(f32)], axis=0)
    h_ref[0:8, :] = _pk(mem00)
    x00 = x_ref[0:SEG, :].astype(f32)
    h_ref[8:24, :] = _pk(_ln(x00))
    xa_ref[0:SEG, :] = x00
    hp_ref[0:8, :] = _pk(mem00)
    hp_ref[8:24, :] = _pk(_ln(x00))
    for i_ in range(NPRE):
        hp_ref[24 + 8 * i_:32 + 8 * i_, :] = _pk(_ln(x_ref[(i_ + 2) * SEG:(i_ + 2) * SEG + 16, :].astype(f32)))

    def perm_wo_unit(e, valid):
        base = jnp.where(valid, e, D // 2)
        w = jnp.concatenate([bwo_raw[k_, pl.ds(base, BH, stride=BDH // 2), :] for k_ in range(5)], axis=1)
        lo = pltpu.bitcast(w << 16, f32)
        hi = pltpu.bitcast(w & jnp.uint32(0xFFFF0000), f32)
        dst = pl.multiple_of(jnp.where(valid, e * BH, D // 2), BH)
        bwo_p[pl.ds(dst, BH // 2), :] = _pk(lo)
        bwo_p[pl.ds(dst + BH // 2, BH // 2), :] = _pk(hi)
    lane8 = jax.lax.broadcasted_iota(jnp.int32, (8, 128), 1)
    def perm_unit(u, valid):
        rg = u // 3
        j = u - 3 * rg
        r = pl.ds(pl.multiple_of(jnp.where(valid, rg * 8, D // 2), 8), 8)
        srcs = [bqkv_raw[r, pl.ds(pl.multiple_of(j * D + k_ * 128, 128), 128)] for k_ in range(5)]
        for n in range(5):
            col = lane8 + n * 128
            s = (col % BH) * BDH + col // BH
            acc = None
            for k_ in range(5):
                g_ = jnp.take_along_axis(srcs[k_], s % 128, axis=1)
                acc = g_ if acc is None else jnp.where(s // 128 == k_, g_, acc)
            bqkv_p[r, pl.ds(pl.multiple_of(j * D + n * 128, 128), 128)] = acc

    lane = jax.lax.broadcasted_iota(jnp.int32, (48, 128), 1)
    lo64 = lane < 64
    rr = jax.lax.broadcasted_iota(jnp.int32, (48, 96), 0)
    cc = jax.lax.broadcasted_iota(jnp.int32, (48, 96), 1)
    ck = jnp.where(cc >= 48, cc - 48, cc)
    first = cc < 48
    def smask(l):
        memk = (ck >= 8 * l) & (ck < 8 * l + 8)
        tokk = (ck >= 16) & ((rr < 16) | (ck <= rr))
        return jnp.where(memk | tokk, 0.0, NEG).astype(f32)
    bias = [smask(0), smask(1)]
    row16 = jax.lax.broadcasted_iota(jnp.int32, (16, PW), 0)
    sc = (DH ** -0.5) * LOG2E

    def bd(a):
        z = jnp.zeros((48, 128), bf16)
        a0, a1, a2 = a[:, 0:128], a[:, 128:256], a[:, 256:384]
        top = jnp.concatenate([a0, jnp.where(lo64, a1, z), z], axis=1)
        bot = jnp.concatenate([z, jnp.where(lo64, z, a1), a2], axis=1)
        return jnp.concatenate([top, bot], axis=0)

    def lhs_h(var, lh):
        if var == 'full':
            return _up(h_ref[...])
        if var == 'v64':
            return _up(jnp.concatenate([h_ref[0:8, :], h_ref[16:40, :]], axis=0))
        return _up(jnp.concatenate([h_ref[0:8, :], h_ref[pl.ds(pl.multiple_of(8 + 16 * lh, 8), 16), :]], axis=0))
    def proj(g, j, var='full', lh=None):
        sl = pl.ds(pl.multiple_of(g * RW, RW), RW) if not isinstance(g, int) else pl.ds(g * RW, RW)
        y = _pk(_dot_nt(lhs_h(var, lh), _up(ws[j][sl, :])))
        if var == 'full': qkv_ref[g, j] = y
        elif var == 'v64':
            qkv_ref[g, j, 0:8, :] = y[0:8]
            qkv_ref[g, j, 16:40, :] = y[8:32]
        else: qkv_ref[g, j, 0:24, :] = y
    def rows(j, g, l, pre=None):
        if l is None: return _up(qkv_ref[g, j, 0:24, :])
        if l == 0 and pre is not None:
            return jnp.concatenate([_up(qkv_ref[g, j, 0:8, :]), _up(pre_ref[g, j, pl.ds(pl.multiple_of(8 * pre, 8), 8), :]),
                                    _up(qkv_ref[g, j, 16:24, :])], axis=0)
        return jnp.concatenate([_up(qkv_ref[g, j, 0:8, :]), _up(qkv_ref[g, j, 8 + 16 * l:24 + 16 * l, :])], axis=0)
    def qk(g, l, pre=None):
        return _dot_nt(rows(0, g, l, pre), bd(rows(1, g, l, pre)))
    def sm(s, bias_l):
        s = s * sc + bias_l
        m0 = jnp.max(jnp.where(first, s, NEG), axis=1, keepdims=True)
        m1 = jnp.max(jnp.where(first, NEG, s), axis=1, keepdims=True)
        p = jnp.exp2(s - jnp.where(first, m0, m1))
        s0 = jnp.sum(jnp.where(first, p, 0.0), axis=1, keepdims=True)
        s1 = jnp.sum(jnp.where(first, 0.0, p), axis=1, keepdims=True)
        p = p * _recip(jnp.where(first, s0, s1))
        return p.astype(bf16)
    def pv(g, ps, pre=None):
        if len(ps) == 1:
            o_ref[g, 0:24, :] = _pk(_dot(ps[0], bd(rows(2, g, None))))
            return
        os_ = [_dot(ps[l], bd(rows(2, g, l, pre))) for l in range(2)]
        om = jnp.where(row16 < 8, os_[0][0:16], os_[1][0:16])
        o = jnp.concatenate([om, os_[0][16:48], os_[1][16:48]], axis=0)
        o_ref[g] = _pk(o)

    h0c = [cc < 48, (cc < 16) | (cc >= 64)]
    row96 = jax.lax.broadcasted_iota(jnp.int32, (16, 96), 0)
    def parts(j, g, pre):
        m_ = _up(qkv_ref[g, j, 0:8, :])
        if pre is None:
            t1 = _up(qkv_ref[g, j, 8:24, :])
        else:
            t1 = jnp.concatenate([_up(pre_ref[g, j, pl.ds(pl.multiple_of(8 * pre, 8), 8), :]), _up(qkv_ref[g, j, 16:24, :])], axis=0)
        t2 = _up(qkv_ref[g, j, 24:40, :])
        return m_, t1, t2
    def lo_(a): return jnp.where(lo64[0:a.shape[0]], a, jnp.zeros_like(a))
    def hi_(a): return jnp.where(lo64[0:a.shape[0]], jnp.zeros_like(a), a)
    def rhs3(j, g, pre):
        m_, t1, t2 = parts(j, g, pre)
        z16 = jnp.zeros((16, 128), bf16)
        cat = lambda *xs: jnp.concatenate(xs, axis=0)
        r0 = cat(m_[:, 0:128], t1[:, 0:128], z16, t2[:, 0:128])
        r2 = cat(z16, t2[:, 256:384], m_[:, 256:384], t1[:, 256:384])
        m1, a1, b1 = m_[:, 128:256], t1[:, 128:256], t2[:, 128:256]
        rt0 = cat(lo_(m1), lo_(a1), hi_(m1), hi_(a1))
        rt1 = cat(lo_(m1), hi_(b1), hi_(m1), lo_(b1))
        return r0, r2, rt0, rt1
    def qk2(g, pre):
        m_, t1, t2 = parts(0, g, pre)
        q = jnp.concatenate([m_, t1, t2], axis=0)
        r0, r2, rt0, rt1 = rhs3(1, g, pre)
        a0 = _dot_nt(q[:, 0:128], r0)
        a2 = _dot_nt(q[:, 256:384], r2)
        q0 = q[0:48, 128:256]
        q1 = jnp.concatenate([q[0:16, 128:256], q[48:80, 128:256]], axis=0)
        s0 = jnp.where(h0c[0], a0[0:48], a2[0:48]) + _dot_nt(q0, rt0)
        a0l = jnp.concatenate([a0[0:16], a0[48:80]], axis=0)
        a2l = jnp.concatenate([a2[0:16], a2[48:80]], axis=0)
        s1 = jnp.where(h0c[1], a0l, a2l) + _dot_nt(q1, rt1)
        return s0, s1
    def sm2(s, bias_l, hc):
        s = s * sc + bias_l
        m0 = jnp.max(jnp.where(hc, s, NEG), axis=1, keepdims=True)
        m1 = jnp.max(jnp.where(hc, NEG, s), axis=1, keepdims=True)
        p = jnp.exp2(s - jnp.where(hc, m0, m1))
        s0 = jnp.sum(jnp.where(hc, p, 0.0), axis=1, keepdims=True)
        s1 = jnp.sum(jnp.where(hc, 0.0, p), axis=1, keepdims=True)
        return p * _recip(jnp.where(hc, s0, s1))
    def pv2(g, ps, pre):
        p0, p1 = ps
        r0, r2, rt0, rt1 = rhs3(2, g, pre)
        pa = [jnp.where(h0c[0], p0, 0.0), jnp.where(h0c[1], p1, 0.0)]
        pb = [jnp.where(h0c[0], 0.0, p0), jnp.where(h0c[1], 0.0, p1)]
        def stack(x):
            mm = jnp.where(row96 < 8, x[0][0:16], x[1][0:16])
            return jnp.concatenate([mm, x[0][16:48], x[1][16:48]], axis=0).astype(bf16)
        o0 = _dot(stack(pa), r0)
        o2 = _dot(stack(pb), r2)
        t0 = _dot(p0.astype(bf16), rt0)
        t1 = _dot(p1.astype(bf16), rt1)
        om = jnp.where(row16[:, 0:128] < 8, t0[0:16], t1[0:16])
        o1 = jnp.concatenate([om, t0[16:48], t1[16:48]], axis=0)
        o_ref[g] = _pk(jnp.concatenate([o0, o1, o2], axis=1))

    rC = jax.lax.broadcasted_iota(jnp.int32, (16, 128), 0)
    bsc = (BDH ** -0.5) * LOG2E

    def b_qkv(layers=(0, 1)):
        r0 = 32 * layers[0]; r1 = 32 * layers[-1] + 32
        y = _dot(_ln(xb_ref[r0:r1, :]).astype(bf16), _up(bqkv_p[0:D // 2, :]))
        bq_ref[r0:r1, :] = y[:, 0:D]
        for l in layers:
            kb_ref[l, 16:48, :] = y[32 * l - r0:32 * l - r0 + 32, D:2 * D]
            vb_ref[l, 16:48, :] = y[32 * l - r0:32 * l - r0 + 32, 2 * D:3 * D]
    def b_attn(t, l, r0, nr):
        q = bq_ref[32 * l + r0:32 * l + r0 + nr, :]
        seg = t - 1 - 2 * l
        pos = seg * SEG + r0 + rC[0:nr]
        lg = []
        for w in range(BW):
            off = 16 - BDIL * w + r0
            pr = q * kb_ref[l, off:off + nr, :]
            a = pr[:, 0:128] + pr[:, 128:256] + pr[:, 256:384] + pr[:, 384:512] + pr[:, 512:640]
            a = a + pltpu.roll(a, 64, 1)
            a = a + pltpu.roll(a, 32, 1)
            a = a * bsc
            if w > 0:
                a = jnp.where(pos >= BDIL * w, a, NEG)
            lg.append(a)
        m = lg[0]
        for w in range(1, BW): m = jnp.maximum(m, lg[w])
        ps = [jnp.exp2(a - m) for a in lg]
        den = ps[0]
        for w in range(1, BW): den = den + ps[w]
        inv = _recip(den)
        acc = None
        for w in range(BW):
            off = 16 - BDIL * w + r0
            pw = ps[w] * inv
            pw5 = jnp.concatenate([pw] * 5, axis=1)
            tt = pw5 * vb_ref[l, off:off + nr, :]
            acc = tt if acc is None else acc + tt
        bo_ref[32 * l + r0:32 * l + r0 + nr, :] = acc
        z = acc[0:8, 0:128]
        for rr_ in range(nr // 8):
            for cc_ in range(5):
                if rr_ or cc_: z = jnp.maximum(z, acc[8 * rr_:8 * rr_ + 8, 128 * cc_:128 * cc_ + 128])
        return z
    def b_hist():
        for l in range(2):
            kb_ref[l, 0:16, :] = kb_ref[l, 32:48, :]
            vb_ref[l, 0:16, :] = vb_ref[l, 32:48, :]
    def b_out(l):
        return xb_ref[32 * l:32 * l + 32, :] + _dot(bo_ref[32 * l:32 * l + 32, :].astype(bf16), _up(bwo_p[0:D // 2, :]))
    def b1_finish(t):
        x2 = b_out(0)
        xn = x_ref[pl.ds(pl.multiple_of(jnp.minimum(t + 1, NSEG - 1) * SEG, SEG), SEG), :].astype(f32)
        xan_ref[0:SEG, :] = xn
        xan_ref[SEG:2 * SEG, :] = x2
        hn_ref[0:16, :] = _pk(_ln(xn))
        hn_ref[16:32, :] = _pk(_ln(x2))
    def b2_finish(t):
        x4 = b_out(1)
        out_ref[pl.ds(pl.multiple_of(jnp.maximum(t - 3, 0) * SEG, SEG), SEG), :] = x4.astype(bf16)
    def wo_part(g0, g1, half=False):
        o = jnp.concatenate([_up(o_ref[g, 0:24, :] if half else o_ref[g]) for g in range(g0, g1)], axis=1)
        return _dot(o, _up(wo[g0 * PW // 2:g1 * PW // 2, :]))

    def step_body(t, var):
        st = {}
        pp = {}
        half = var == 'half'
        lh = jnp.where(t < 2, 0, 1) if half else None
        bias_h = smask(lh) if half else None
        pre = jnp.clip(t - 2, 0, NPRE - 1) if var == 'v64' else None
        def ex(i, pos):
            for name in SCHED[var].get((i, pos), ()): run_extra(name, t, st, half)
        for i in range(-2, NPAIR):
            g2, g1, g0 = i + 2, i + 1, i
            def do_proj(j):
                if g2 < NPAIR: proj(g2, j, var, lh)
                ex(i, 'qkv'[j])
            def do_qk():
                if 0 <= g1 < NPAIR:
                    if half:
                        pp[g1] = [sm(qk(g1, None), bias_h)]
                    else:
                        s_ = qk2(g1, pre)
                        pp[g1] = [sm2(s_[0], bias[0], h0c[0]), sm2(s_[1], bias[1], h0c[1])]
            def do_pv():
                if 0 <= g0:
                    pg = pp.pop(g0)
                    for (l_, r0_, nr_) in BDEP[var].get(g0, ()):
                        z = b_attn(t, l_, r0_, nr_)
                        p0 = jnp.where(t < 0, z[:, 0:96].astype(pg[0].dtype), pg[0][0:8])
                        pg[0] = jnp.concatenate([p0, pg[0][8:]], axis=0)
                    if half: pv(g0, pg, pre)
                    else: pv2(g0, pg, pre)
            ex(i, 'pre')
            for ch in ORDER:
                if ch == 'S': do_qk()
                elif ch == 'P': do_pv()
                else: do_proj('qkv'.index(ch))
            ex(i, 'post')
        end_step(t, st['oa'], lh)

    def step(t, c):
        @pl.when(t == 1)
        def _():
            cp_x1.wait()
        is_half = (t < 2) | (t >= NSEG)
        is_v64 = (t >= 2) & (t < NPRE + 2)
        pl.when(is_half)(lambda: step_body(t, 'half'))
        pl.when(is_v64)(lambda: step_body(t, 'v64'))
        pl.when(jnp.logical_not(is_half | is_v64))(lambda: step_body(t, 'full'))
        @pl.when(t >= 3)
        def _():
            cp_out(jnp.maximum(t - 3, 0)).start()
        return c

    def end_step(t, oa, lh=None):
        if lh is None:
            xb_ref[...] = xa_ref[...] + oa[16:80]
        else:
            sl = pl.ds(pl.multiple_of(SEG * lh, SEG), SEG) if not isinstance(lh, int) else pl.ds(SEG * lh, SEG)
            xb_ref[sl, :] = xa_ref[sl, :] + oa[16:48]
        xa_ref[...] = xan_ref[...]
        r16 = jax.lax.broadcasted_iota(jnp.int32, (16, D), 0)
        memn = jnp.where((r16 >= 8) & (t < 2), mem00, oa[0:16])
        h_ref[0:8, :] = _pk(memn)

    def run_extra(name, t, st, half):
        if name == 'bqkv': b_qkv()
        elif name[0] == 'battn': b_attn(t, name[1], name[2], name[3])
        elif name == 'bhist': b_hist()
        elif name == 'hcopy': h_ref[8:40, :] = hn_ref[...]
        elif name == 'b1fin': b1_finish(t)
        elif name == 'b2fin': b2_finish(t)
        elif name[0] == 'wo':
            part = wo_part(name[1], name[2], half)
            st['oa'] = part if 'oa' not in st else st['oa'] + part
        else: raise ValueError(name)

    def wproj(g, j):
        sl = pl.ds(pl.multiple_of(g * RW, RW), RW)
        y = _pk(_dot_nt(_up(hp_ref[...]), _up(ws[j][sl, :])))
        qkv_ref[g, j, 0:24, :] = y[0:24]
        pre_ref[g, j] = y[24:]
    for j in range(3): qkv_ref[0, j, 0:24, :] = jnp.zeros((24, PW), u32)
    def pair0(g, c):
        gp = jnp.maximum(g - 1, 0)
        for i_, g_ in enumerate((3, 6, 10)):
            pl.when(g == g_)(cp_bqkv[i_].wait)
        @pl.when(g == 6)
        def _():
            for c_ in cp_bwo: c_.wait()
        for j in range(3): cp_w(j, g).wait()
        vb = bd(rows(2, gp, None))
        p = sm(qk(gp, None), bias[0])
        wproj(g, 0); wproj(g, 1)
        o_ref[gp, 0:24, :] = _pk(_dot(p, vb))
        wproj(g, 2)
        for k_ in range(10): perm_unit(jnp.clip(10 * (g - 3) + k_, 0, 119), g >= 3)
        perm_wo_unit(jnp.clip(g - 6, 0, 9), g >= 6)
        return c
    jax.lax.fori_loop(0, NPAIR, pair0, 0, unroll=1)
    pv(NPAIR - 1, [sm(qk(NPAIR - 1, None), bias[0])])
    for i_ in range(NWO): cp_wo(i_).wait()
    oa = wo_part(0, NPAIR, True)
    xn = x_ref[SEG:2 * SEG, :].astype(f32)
    xan_ref[0:SEG, :] = xn
    xan_ref[SEG:2 * SEG, :] = jnp.zeros((SEG, D), f32)
    h_ref[8:24, :] = _pk(_ln(xn))
    end_step(0, oa, 0)

    jax.lax.fori_loop(1, nsteps, step, 0, unroll=1)
    b_qkv((1,))
    for c_ in range(2): b_attn(NSEG + 2, 1, 16 * c_, 16)
    b2_finish(NSEG + 2)
    cp_out(NSEG - 1).start()
    def wait_out(s, c):
        cp_out(s).wait()
        return c
    jax.lax.fori_loop(0, min(nsteps - 3, NSEG - 1) + 1 if nsteps > 3 else 1, wait_out, 0)

@functools.partial(jax.jit, static_argnames=("A_seg_len",))
def pallas_interleave_layers__memory_aug_recurrent_mem_tr__sliding_local_dilated__prompt_kernel(
        A_x, A_mem0, A_Wq, A_Wk, A_Wv, A_Wo, A_seg_len, B_x, B_wqkv, B_wo):
    assert A_seg_len == SEG
    del B_x
    nsteps = NSEG + 2
    x = A_x.reshape(S, D)
    mem0 = A_mem0.reshape(M, D)
    tr = lambda w: jnp.transpose(w, (1, 2, 0)).reshape(H * DH, D)
    wo = A_Wo.reshape(H * DH, D)
    hbm = pl.BlockSpec(memory_space=pl.ANY)
    out = pl.pallas_call(
        functools.partial(kernel, nsteps),
        out_shape=jax.ShapeDtypeStruct((S, D), bf16),
        in_specs=[hbm] * 8,
        out_specs=hbm,
        scratch_shapes=[
            pltpu.VMEM((H * DH // 2, D), u32), pltpu.VMEM((H * DH // 2, D), u32), pltpu.VMEM((H * DH // 2, D), u32), pltpu.VMEM((H * DH // 2, D), u32),
            pltpu.VMEM((D // 2 + 8, 3 * D), u32), pltpu.VMEM((5, D, 128), u32),
            pltpu.VMEM((D // 2 + 8, 3 * D), u32), pltpu.VMEM((D // 2 + 32, D), u32),
            pltpu.VMEM((S, D), bf16), pltpu.VMEM((M, D), bf16), pltpu.VMEM((S, D), bf16),
            pltpu.VMEM((40, D), u32), pltpu.VMEM((NPAIR, 3, 40, PW), u32), pltpu.VMEM((NPAIR, 40, PW), u32),
            pltpu.VMEM((64, D), f32), pltpu.VMEM((64, D), f32),
            pltpu.VMEM((2, 48, D), f32), pltpu.VMEM((2, 48, D), f32),
            pltpu.VMEM((64, D), f32), pltpu.VMEM((64, D), f32), pltpu.VMEM((64, D), f32),
            pltpu.VMEM((32, D), u32),
            pltpu.VMEM((24 + 8 * NPRE, D), u32), pltpu.VMEM((NPAIR, 3, 8 * NPRE, PW), u32),
            pltpu.SemaphoreType.DMA((NPAIR,)), pltpu.SemaphoreType.DMA((9,)), pltpu.SemaphoreType.DMA((1,)), pltpu.SemaphoreType.DMA((8,)),
        ],
        compiler_params=pltpu.CompilerParams(vmem_limit_bytes=100 * 1024 * 1024),
    )(x, mem0, tr(A_Wq), tr(A_Wk), tr(A_Wv), wo, B_wqkv, B_wo)
    return out.reshape(1, S, D)
```

```python
import functools
import jax
import jax.numpy as jnp
import numpy as np
from jax.experimental import pallas as pl
from jax.experimental.pallas import tpu as pltpu

S = 2048; D = 640; H = 32; DH = 192; M = 8; SEG = 32; NSEG = S // SEG
NPAIR = H // 2; PW = 2 * DH
BH = 32; BDH = D // BH; BW = 8; BDIL = 2
LOG2E = 1.4426950408889634
NEG = -1e30
f32 = jnp.float32; bf16 = jnp.bfloat16; u32 = jnp.uint32

def _sched(bq, b1, bh, hc, cuts, wpos, b2):
    s = {}
    s.setdefault(bq, []).append('bqkv')
    s.setdefault((b1, 'post'), []).append('b1fin')
    s.setdefault((bh, 'post'), []).append('bhist')
    s.setdefault((hc, 'post'), []).append('hcopy')
    cs = [0] + list(cuts) + [NPAIR]
    for (g0, g1), p in zip(zip(cs, cs[1:]), wpos):
        s.setdefault(p, []).append(('wo', g0, g1))
    s.setdefault(b2, []).append('b2fin')
    return s
def _bdep(l0, l1):
    d = {}
    for i, g in enumerate(l0): d.setdefault(g, []).append((0, 8 * i, 8))
    for i, g in enumerate(l1): d.setdefault(g, []).append((1, 8 * i, 8))
    return d
_WP = ((13, 'post'), (14, 'k'), (14, 'post'), (15, 'post'))
SCHED = {
    'half': _sched((0, 'pre'), 8, 11, 13, (4, 8, 13), _WP, (15, 'post')),
    'v64': _sched((0, 'post'), 8, 11, 13, (4, 8, 13), _WP, (15, 'post')),
    'full': _sched((0, 'post'), 8, 12, 13, (4, 8, 13), _WP, (15, 'post')),
}
BDEP = {
    'half': _bdep((3, 4, 5, 7), (9, 10, 11, 11)),
    'v64': _bdep((3, 5, 7, 8), (9, 10, 11, 11)),
    'full': _bdep((3, 4, 5, 7), (9, 10, 11, 12)),
}
ORDER = 'qkvSP'
ORDER = 'qkvSP'
NPRE = 9

def _dot(a, b):
    return jnp.dot(a, b, preferred_element_type=f32)
def _dot_nt(a, b):
    return lax_dot(a, b, (((1,), (1,)), ((), ())))
def lax_dot(a, b, dn):
    return jax.lax.dot_general(a, b, dn, preferred_element_type=f32)

def _recip(x):
    r = pl.reciprocal(x, approx=True)
    return r * (2.0 - x * r)

def _ln(x):
    m = jnp.mean(x, axis=-1, keepdims=True)
    xc = x - m
    v = jnp.mean(xc * xc, axis=-1, keepdims=True)
    return xc * jax.lax.rsqrt(v + 1e-5)

def _perm_mat():
    r = jax.lax.broadcasted_iota(jnp.int32, (D, D), 0)
    c = jax.lax.broadcasted_iota(jnp.int32, (D, D), 1)
    h = c % BH
    d = c // BH
    return (r == h * BDH + d).astype(bf16)

def _pk(x):
    return pltpu.bitcast(x.astype(bf16), u32)
def _up(x):
    return pltpu.bitcast(x, bf16)

def kernel(nsteps, x_hbm, mem0_hbm, wq_hbm, wk_hbm, wv_hbm, wo_hbm, bqkv_hbm, bwo_hbm, out_hbm,
           wq, wk, wv, wo, bqkv_raw, bwo_raw, bqkv_p, bwo_p, x_ref, mem0_ref, out_ref,
           h_ref, qkv_ref, o_ref, xa_ref, xb_ref, kb_ref, vb_ref, xan_ref, bq_ref, bo_ref, hn_ref, hp_ref, pre_ref, wn_ref,
           sem_w, sem_m, sem_o, sem_b):
    RW = PW // 2
    ws = (wq, wk, wv)
    ws_hbm = (wq_hbm.bitcast(u32), wk_hbm.bitcast(u32), wv_hbm.bitcast(u32))
    NWO = 4
    RO = H * DH // 2 // NWO
    def cp_w(j, g):
        sl = pl.ds(pl.multiple_of(g * RW, RW), RW) if not isinstance(g, int) else pl.ds(g * RW, RW)
        return pltpu.make_async_copy(ws_hbm[j].at[sl], ws[j].at[sl], sem_w.at[g])
    X0R = (NPRE + 2) * SEG
    cp_x0 = pltpu.make_async_copy(x_hbm.at[0:X0R], x_ref.at[0:X0R], sem_m.at[0])
    cp_mem = pltpu.make_async_copy(mem0_hbm, mem0_ref, sem_m.at[1])
    BQR = (0, 104, 208, 320)
    cp_bqkv = [pltpu.make_async_copy(bqkv_hbm.bitcast(u32).at[BQR[i_]:BQR[i_ + 1]], bqkv_raw.at[BQR[i_]:BQR[i_ + 1]], sem_b.at[i_])
               for i_ in range(3)]
    cp_bwo = [pltpu.make_async_copy(bwo_hbm.bitcast(u32).at[:, k_ * 128:(k_ + 1) * 128], bwo_raw.at[k_, 0:D // 2, :], sem_b.at[3 + k_])
              for k_ in range(5)]
    def cp_wo(i):
        sl = pl.ds(pl.multiple_of(i * RO, RO), RO) if not isinstance(i, int) else pl.ds(i * RO, RO)
        return pltpu.make_async_copy(wo_hbm.bitcast(u32).at[sl], wo.at[sl], sem_m.at[4 + i])
    cp_x1 = pltpu.make_async_copy(x_hbm.at[X0R:S], x_ref.at[X0R:S], sem_m.at[4 + NWO])
    def cp_out(s):
        sl = pl.ds(pl.multiple_of(s * SEG, SEG), SEG) if not isinstance(s, int) else pl.ds(s * SEG, SEG)
        return pltpu.make_async_copy(out_ref.at[sl], out_hbm.at[sl], sem_o.at[0])

    cp_x0.start(); cp_mem.start()
    for g in range(NPAIR):
        if g == 3: cp_bqkv[0].start()
        if g == 5:
            for c_ in cp_bwo: c_.start()
        if g == 6: cp_bqkv[1].start()
        if g == 9: cp_bqkv[2].start()
        for j in range(3): cp_w(j, g).start()
    for i_ in range(NWO): cp_wo(i_).start()
    cp_x1.start()

    bqkv_raw[D // 2:D // 2 + 8, :] = jnp.zeros((8, 3 * D), u32)
    for k_ in range(5): bwo_raw[k_, D // 2:D, :] = jnp.zeros((D // 2, 128), u32)
    xb_ref[...] = jnp.zeros((2 * SEG, D), f32)
    kb_ref[...] = jnp.zeros(kb_ref.shape, f32)
    vb_ref[...] = jnp.zeros(vb_ref.shape, f32)
    xa_ref[SEG:2 * SEG, :] = jnp.zeros((SEG, D), f32)
    h_ref[24:40, :] = jnp.zeros((16, D), u32)
    cp_x0.wait(); cp_mem.wait()
    mem0 = mem0_ref[...]
    mem00 = jnp.concatenate([mem0.astype(f32), mem0.astype(f32)], axis=0)
    h_ref[0:8, :] = _pk(mem00)
    x00 = x_ref[0:SEG, :].astype(f32)
    h_ref[8:24, :] = _pk(_ln(x00))
    xa_ref[0:SEG, :] = x00
    hp_ref[0:8, :] = _pk(mem00)
    hp_ref[8:24, :] = _pk(_ln(x00))
    for i_ in range(NPRE):
        hp_ref[24 + 16 * i_:40 + 16 * i_, :] = _pk(_ln(x_ref[(i_ + 2) * SEG:(i_ + 3) * SEG, :].astype(f32)))

    def perm_wo_unit(e, valid):
        base = jnp.where(valid, e, D // 2)
        w = jnp.concatenate([bwo_raw[k_, pl.ds(base, BH, stride=BDH // 2), :] for k_ in range(5)], axis=1)
        lo = pltpu.bitcast(w << 16, f32)
        hi = pltpu.bitcast(w & jnp.uint32(0xFFFF0000), f32)
        dst = pl.multiple_of(jnp.where(valid, e * BH, D // 2), BH)
        bwo_p[pl.ds(dst, BH // 2), :] = _pk(lo)
        bwo_p[pl.ds(dst + BH // 2, BH // 2), :] = _pk(hi)
    lane8 = jax.lax.broadcasted_iota(jnp.int32, (8, 128), 1)
    def perm_unit(u, valid):
        rg = u // 3
        j = u - 3 * rg
        r = pl.ds(pl.multiple_of(jnp.where(valid, rg * 8, D // 2), 8), 8)
        srcs = [bqkv_raw[r, pl.ds(pl.multiple_of(j * D + k_ * 128, 128), 128)] for k_ in range(5)]
        for n in range(5):
            col = lane8 + n * 128
            s = (col % BH) * BDH + col // BH
            acc = None
            for k_ in range(5):
                g_ = jnp.take_along_axis(srcs[k_], s % 128, axis=1)
                acc = g_ if acc is None else jnp.where(s // 128 == k_, g_, acc)
            bqkv_p[r, pl.ds(pl.multiple_of(j * D + n * 128, 128), 128)] = acc

    lane = jax.lax.broadcasted_iota(jnp.int32, (48, 128), 1)
    lo64 = lane < 64
    rr = jax.lax.broadcasted_iota(jnp.int32, (48, 96), 0)
    cc = jax.lax.broadcasted_iota(jnp.int32, (48, 96), 1)
    ck = jnp.where(cc >= 48, cc - 48, cc)
    first = cc < 48
    def smask(l):
        memk = (ck >= 8 * l) & (ck < 8 * l + 8)
        tokk = (ck >= 16) & ((rr < 16) | (ck <= rr))
        return jnp.where(memk | tokk, 0.0, NEG).astype(f32)
    bias = [smask(0), smask(1)]
    row16 = jax.lax.broadcasted_iota(jnp.int32, (16, PW), 0)
    sc = (DH ** -0.5) * LOG2E

    def bd(a):
        z = jnp.zeros((48, 128), bf16)
        a0, a1, a2 = a[:, 0:128], a[:, 128:256], a[:, 256:384]
        top = jnp.concatenate([a0, jnp.where(lo64, a1, z), z], axis=1)
        bot = jnp.concatenate([z, jnp.where(lo64, z, a1), a2], axis=1)
        return jnp.concatenate([top, bot], axis=0)

    def lhs_h(var, lh):
        if var == 'full':
            return _up(h_ref[...])
        if var == 'v64':
            return _up(jnp.concatenate([h_ref[0:8, :], h_ref[24:40, :]], axis=0))
        return _up(jnp.concatenate([h_ref[0:8, :], h_ref[pl.ds(pl.multiple_of(8 + 16 * lh, 8), 16), :]], axis=0))
    def proj(g, j, var='full', lh=None):
        y = _pk(_dot(lhs_h(var, lh), _up(wn_ref[g, j])))
        if var == 'full': qkv_ref[g, j] = y
        elif var == 'v64':
            qkv_ref[g, j, 0:8, :] = y[0:8]
            qkv_ref[g, j, 24:40, :] = y[8:24]
        else: qkv_ref[g, j, 0:24, :] = y
    def rows(j, g, l, pre=None):
        if l is None: return _up(qkv_ref[g, j, 0:24, :])
        return jnp.concatenate([_up(qkv_ref[g, j, 0:8, :]), _up(qkv_ref[g, j, 8 + 16 * l:24 + 16 * l, :])], axis=0)
    def qk(g, l, pre=None):
        return _dot_nt(rows(0, g, l, pre), bd(rows(1, g, l, pre)))
    def sm(s, bias_l):
        s = s * sc + bias_l
        m0 = jnp.max(jnp.where(first, s, NEG), axis=1, keepdims=True)
        m1 = jnp.max(jnp.where(first, NEG, s), axis=1, keepdims=True)
        p = jnp.exp2(s - jnp.where(first, m0, m1))
        s0 = jnp.sum(jnp.where(first, p, 0.0), axis=1, keepdims=True)
        s1 = jnp.sum(jnp.where(first, 0.0, p), axis=1, keepdims=True)
        p = p * _recip(jnp.where(first, s0, s1))
        return p.astype(bf16)
    def pv(g, ps, pre=None):
        if len(ps) == 1:
            o_ref[g, 0:24, :] = _pk(_dot(ps[0], bd(rows(2, g, None))))
            return
        os_ = [_dot(ps[l], bd(rows(2, g, l, pre))) for l in range(2)]
        om = jnp.where(row16 < 8, os_[0][0:16], os_[1][0:16])
        o = jnp.concatenate([om, os_[0][16:48], os_[1][16:48]], axis=0)
        o_ref[g] = _pk(o)

    h0c = [cc < 48, (cc < 16) | (cc >= 64)]
    row96 = jax.lax.broadcasted_iota(jnp.int32, (16, 96), 0)
    def parts(j, g, pre):
        m_ = _up(qkv_ref[g, j, 0:8, :])
        if pre is None:
            t1 = _up(qkv_ref[g, j, 8:24, :])
        else:
            t1 = _up(pre_ref[g, j, pl.ds(pl.multiple_of(16 * pre, 16), 16), :])
        t2 = _up(qkv_ref[g, j, 24:40, :])
        return m_, t1, t2
    def lo_(a): return jnp.where(lo64[0:a.shape[0]], a, jnp.zeros_like(a))
    def hi_(a): return jnp.where(lo64[0:a.shape[0]], jnp.zeros_like(a), a)
    def rhs3(j, g, pre):
        m_, t1, t2 = parts(j, g, pre)
        z16 = jnp.zeros((16, 128), bf16)
        cat = lambda *xs: jnp.concatenate(xs, axis=0)
        r0 = cat(m_[:, 0:128], t1[:, 0:128], z16, t2[:, 0:128])
        r2 = cat(z16, t2[:, 256:384], m_[:, 256:384], t1[:, 256:384])
        m1, a1, b1 = m_[:, 128:256], t1[:, 128:256], t2[:, 128:256]
        rt0 = cat(lo_(m1), lo_(a1), hi_(m1), hi_(a1))
        rt1 = cat(lo_(m1), hi_(b1), hi_(m1), lo_(b1))
        return r0, r2, rt0, rt1
    def qk2(g, pre):
        m_, t1, t2 = parts(0, g, pre)
        q = jnp.concatenate([m_, t1, t2], axis=0)
        r0, r2, rt0, rt1 = rhs3(1, g, pre)
        a0 = _dot_nt(q[:, 0:128], r0)
        a2 = _dot_nt(q[:, 256:384], r2)
        q0 = q[0:48, 128:256]
        q1 = jnp.concatenate([q[0:16, 128:256], q[48:80, 128:256]], axis=0)
        s0 = jnp.where(h0c[0], a0[0:48], a2[0:48]) + _dot_nt(q0, rt0)
        a0l = jnp.concatenate([a0[0:16], a0[48:80]], axis=0)
        a2l = jnp.concatenate([a2[0:16], a2[48:80]], axis=0)
        s1 = jnp.where(h0c[1], a0l, a2l) + _dot_nt(q1, rt1)
        return s0, s1
    def sm2(s, bias_l, hc):
        s = s * sc + bias_l
        m0 = jnp.max(jnp.where(hc, s, NEG), axis=1, keepdims=True)
        m1 = jnp.max(jnp.where(hc, NEG, s), axis=1, keepdims=True)
        p = jnp.exp2(s - jnp.where(hc, m0, m1))
        s0 = jnp.sum(jnp.where(hc, p, 0.0), axis=1, keepdims=True)
        s1 = jnp.sum(jnp.where(hc, 0.0, p), axis=1, keepdims=True)
        return p * _recip(jnp.where(hc, s0, s1))
    def pv2(g, ps, pre):
        p0, p1 = ps
        r0, r2, rt0, rt1 = rhs3(2, g, pre)
        pa = [jnp.where(h0c[0], p0, 0.0), jnp.where(h0c[1], p1, 0.0)]
        pb = [jnp.where(h0c[0], 0.0, p0), jnp.where(h0c[1], 0.0, p1)]
        def stack(x):
            mm = jnp.where(row96 < 8, x[0][0:16], x[1][0:16])
            return jnp.concatenate([mm, x[0][16:48], x[1][16:48]], axis=0).astype(bf16)
        o0 = _dot(stack(pa), r0)
        o2 = _dot(stack(pb), r2)
        t0 = _dot(p0.astype(bf16), rt0)
        t1 = _dot(p1.astype(bf16), rt1)
        om = jnp.where(row16[:, 0:128] < 8, t0[0:16], t1[0:16])
        o1 = jnp.concatenate([om, t0[16:48], t1[16:48]], axis=0)
        o_ref[g] = _pk(jnp.concatenate([o0, o1, o2], axis=1))

    rC = jax.lax.broadcasted_iota(jnp.int32, (16, 128), 0)
    bsc = (BDH ** -0.5) * LOG2E

    def b_qkv(layers=(0, 1)):
        r0 = 32 * layers[0]; r1 = 32 * layers[-1] + 32
        y = _dot(_ln(xb_ref[r0:r1, :]).astype(bf16), _up(bqkv_p[0:D // 2, :]))
        bq_ref[r0:r1, :] = y[:, 0:D]
        for l in layers:
            kb_ref[l, 16:48, :] = y[32 * l - r0:32 * l - r0 + 32, D:2 * D]
            vb_ref[l, 16:48, :] = y[32 * l - r0:32 * l - r0 + 32, 2 * D:3 * D]
    def b_attn(t, l, r0, nr):
        q = bq_ref[32 * l + r0:32 * l + r0 + nr, :]
        seg = t - 1 - 2 * l
        pos = seg * SEG + r0 + rC[0:nr]
        lg = []
        for w in range(BW):
            off = 16 - BDIL * w + r0
            pr = q * kb_ref[l, off:off + nr, :]
            a = pr[:, 0:128] + pr[:, 128:256] + pr[:, 256:384] + pr[:, 384:512] + pr[:, 512:640]
            a = a + pltpu.roll(a, 64, 1)
            a = a + pltpu.roll(a, 32, 1)
            a = a * bsc
            if w > 0:
                a = jnp.where(pos >= BDIL * w, a, NEG)
            lg.append(a)
        m = lg[0]
        for w in range(1, BW): m = jnp.maximum(m, lg[w])
        ps = [jnp.exp2(a - m) for a in lg]
        den = ps[0]
        for w in range(1, BW): den = den + ps[w]
        inv = _recip(den)
        acc = None
        for w in range(BW):
            off = 16 - BDIL * w + r0
            pw = ps[w] * inv
            pw5 = jnp.concatenate([pw] * 5, axis=1)
            tt = pw5 * vb_ref[l, off:off + nr, :]
            acc = tt if acc is None else acc + tt
        bo_ref[32 * l + r0:32 * l + r0 + nr, :] = acc
        z = acc[0:8, 0:128]
        for rr_ in range(nr // 8):
            for cc_ in range(5):
                if rr_ or cc_: z = jnp.maximum(z, acc[8 * rr_:8 * rr_ + 8, 128 * cc_:128 * cc_ + 128])
        return z
    def b_hist():
        for l in range(2):
            kb_ref[l, 0:16, :] = kb_ref[l, 32:48, :]
            vb_ref[l, 0:16, :] = vb_ref[l, 32:48, :]
    def b_out(l):
        return xb_ref[32 * l:32 * l + 32, :] + _dot(bo_ref[32 * l:32 * l + 32, :].astype(bf16), _up(bwo_p[0:D // 2, :]))
    def b1_finish(t):
        x2 = b_out(0)
        xn = x_ref[pl.ds(pl.multiple_of(jnp.minimum(t + 1, NSEG - 1) * SEG, SEG), SEG), :].astype(f32)
        xan_ref[0:SEG, :] = xn
        xan_ref[SEG:2 * SEG, :] = x2
        hn_ref[0:16, :] = _pk(_ln(xn))
        hn_ref[16:32, :] = _pk(_ln(x2))
    def b2_finish(t):
        x4 = b_out(1)
        out_ref[pl.ds(pl.multiple_of(jnp.maximum(t - 3, 0) * SEG, SEG), SEG), :] = x4.astype(bf16)
    def wo_part(g0, g1, half=False):
        o = jnp.concatenate([_up(o_ref[g, 0:24, :] if half else o_ref[g]) for g in range(g0, g1)], axis=1)
        return _dot(o, _up(wo[g0 * PW // 2:g1 * PW // 2, :]))

    def step_body(t, var):
        st = {}
        pp = {}
        half = var == 'half'
        lh = jnp.where(t < 2, 0, 1) if half else None
        bias_h = smask(lh) if half else None
        pre = jnp.clip(t - 2, 0, NPRE - 1) if var == 'v64' else None
        def ex(i, pos):
            for name in SCHED[var].get((i, pos), ()): run_extra(name, t, st, half)
        for i in range(-2, NPAIR):
            g2, g1, g0 = i + 2, i + 1, i
            def do_proj(j):
                if g2 < NPAIR: proj(g2, j, var, lh)
                ex(i, 'qkv'[j])
            def do_qk():
                if 0 <= g1 < NPAIR:
                    if half:
                        pp[g1] = [sm(qk(g1, None), bias_h)]
                    else:
                        s_ = qk2(g1, pre)
                        pp[g1] = [sm2(s_[0], bias[0], h0c[0]), sm2(s_[1], bias[1], h0c[1])]
            def do_pv():
                if 0 <= g0:
                    pg = pp.pop(g0)
                    for (l_, r0_, nr_) in BDEP[var].get(g0, ()):
                        z = b_attn(t, l_, r0_, nr_)
                        p0 = jnp.where(t < 0, z[:, 0:96].astype(pg[0].dtype), pg[0][0:8])
                        pg[0] = jnp.concatenate([p0, pg[0][8:]], axis=0)
                    if half: pv(g0, pg, pre)
                    else: pv2(g0, pg, pre)
            ex(i, 'pre')
            for ch in ORDER:
                if ch == 'S': do_qk()
                elif ch == 'P': do_pv()
                else: do_proj('qkv'.index(ch))
            ex(i, 'post')
        end_step(t, st['oa'], lh)

    def make_step(var):
        def step(t, c):
            step_body(t, var)
            @pl.when(t >= 3)
            def _():
                cp_out(jnp.maximum(t - 3, 0)).start()
            return c
        return step

    def phase(ph, c):
        lo = jnp.where(ph == 0, 1, NSEG)
        hi = jnp.where(ph == 0, 2, nsteps)
        jax.lax.fori_loop(lo, hi, make_step('half'), 0)
        @pl.when(ph == 0)
        def _():
            cp_x1.wait()
            jax.lax.fori_loop(2, min(NPRE + 2, nsteps), make_step('v64'), 0)
            jax.lax.fori_loop(NPRE + 2, min(NSEG, nsteps), make_step('full'), 0)
        return c

    def end_step(t, oa, lh=None):
        if lh is None:
            xb_ref[...] = xa_ref[...] + oa[16:80]
        else:
            sl = pl.ds(pl.multiple_of(SEG * lh, SEG), SEG) if not isinstance(lh, int) else pl.ds(SEG * lh, SEG)
            xb_ref[sl, :] = xa_ref[sl, :] + oa[16:48]
        xa_ref[...] = xan_ref[...]
        r16 = jax.lax.broadcasted_iota(jnp.int32, (16, D), 0)
        memn = jnp.where((r16 >= 8) & (t < 2), mem00, oa[0:16])
        h_ref[0:8, :] = _pk(memn)

    def run_extra(name, t, st, half):
        if name == 'bqkv': b_qkv()
        elif name[0] == 'battn': b_attn(t, name[1], name[2], name[3])
        elif name == 'bhist': b_hist()
        elif name == 'hcopy': h_ref[8:40, :] = hn_ref[...]
        elif name == 'b1fin': b1_finish(t)
        elif name == 'b2fin': b2_finish(t)
        elif name[0] == 'wo':
            part = wo_part(name[1], name[2], half)
            st['oa'] = part if 'oa' not in st else st['oa'] + part
        else: raise ValueError(name)

    def wproj(g, j):
        sl = pl.ds(pl.multiple_of(g * RW, RW), RW)
        y = _pk(_dot_nt(_up(hp_ref[...]), _up(ws[j][sl, :])))
        qkv_ref[g, j, 0:24, :] = y[0:24]
        pre_ref[g, j] = y[24:]
    for j in range(3): qkv_ref[0, j, 0:24, :] = jnp.zeros((24, PW), u32)
    def pair0(g, c):
        gp = jnp.maximum(g - 1, 0)
        for i_, g_ in enumerate((3, 6, 10)):
            pl.when(g == g_)(cp_bqkv[i_].wait)
        @pl.when(g == 6)
        def _():
            for c_ in cp_bwo: c_.wait()
        for j in range(3): cp_w(j, g).wait()
        vb = bd(rows(2, gp, None))
        p = sm(qk(gp, None), bias[0])
        wproj(g, 0); wproj(g, 1)
        o_ref[gp, 0:24, :] = _pk(_dot(p, vb))
        wproj(g, 2)
        for j in range(3):
            wn_ref[g, j] = _pk(_up(ws[j][pl.ds(pl.multiple_of(g * RW, RW), RW), :]).T)
        for k_ in range(10): perm_unit(jnp.clip(10 * (g - 3) + k_, 0, 119), g >= 3)
        perm_wo_unit(jnp.clip(g - 6, 0, 9), g >= 6)
        return c
    jax.lax.fori_loop(0, NPAIR, pair0, 0, unroll=1)
    pv(NPAIR - 1, [sm(qk(NPAIR - 1, None), bias[0])])
    for i_ in range(NWO): cp_wo(i_).wait()
    oa = wo_part(0, NPAIR, True)
    xn = x_ref[SEG:2 * SEG, :].astype(f32)
    xan_ref[0:SEG, :] = xn
    xan_ref[SEG:2 * SEG, :] = jnp.zeros((SEG, D), f32)
    h_ref[8:24, :] = _pk(_ln(xn))
    end_step(0, oa, 0)

    jax.lax.fori_loop(0, 2, phase, 0)
    b_qkv((1,))
    for c_ in range(2): b_attn(NSEG + 2, 1, 16 * c_, 16)
    b2_finish(NSEG + 2)
    cp_out(NSEG - 1).start()
    def wait_out(s, c):
        cp_out(s).wait()
        return c
    jax.lax.fori_loop(0, min(nsteps - 3, NSEG - 1) + 1 if nsteps > 3 else 1, wait_out, 0)

@functools.partial(jax.jit, static_argnames=("A_seg_len",))
def pallas_interleave_layers__memory_aug_recurrent_mem_tr__sliding_local_dilated__prompt_kernel(
        A_x, A_mem0, A_Wq, A_Wk, A_Wv, A_Wo, A_seg_len, B_x, B_wqkv, B_wo):
    assert A_seg_len == SEG
    del B_x
    nsteps = NSEG + 2
    x = A_x.reshape(S, D)
    mem0 = A_mem0.reshape(M, D)
    tr = lambda w: jnp.transpose(w, (1, 2, 0)).reshape(H * DH, D)
    wo = A_Wo.reshape(H * DH, D)
    hbm = pl.BlockSpec(memory_space=pl.ANY)
    out = pl.pallas_call(
        functools.partial(kernel, nsteps),
        out_shape=jax.ShapeDtypeStruct((S, D), bf16),
        in_specs=[hbm] * 8,
        out_specs=hbm,
        scratch_shapes=[
            pltpu.VMEM((H * DH // 2, D), u32), pltpu.VMEM((H * DH // 2, D), u32), pltpu.VMEM((H * DH // 2, D), u32), pltpu.VMEM((H * DH // 2, D), u32),
            pltpu.VMEM((D // 2 + 8, 3 * D), u32), pltpu.VMEM((5, D, 128), u32),
            pltpu.VMEM((D // 2 + 8, 3 * D), u32), pltpu.VMEM((D // 2 + 32, D), u32),
            pltpu.VMEM((S, D), bf16), pltpu.VMEM((M, D), bf16), pltpu.VMEM((S, D), bf16),
            pltpu.VMEM((40, D), u32), pltpu.VMEM((NPAIR, 3, 40, PW), u32), pltpu.VMEM((NPAIR, 40, PW), u32),
            pltpu.VMEM((64, D), f32), pltpu.VMEM((64, D), f32),
            pltpu.VMEM((2, 48, D), f32), pltpu.VMEM((2, 48, D), f32),
            pltpu.VMEM((64, D), f32), pltpu.VMEM((64, D), f32), pltpu.VMEM((64, D), f32),
            pltpu.VMEM((32, D), u32),
            pltpu.VMEM((24 + 16 * NPRE, D), u32), pltpu.VMEM((NPAIR, 3, 16 * NPRE, PW), u32),
            pltpu.VMEM((NPAIR, 3, D // 2, PW), u32),
            pltpu.SemaphoreType.DMA((NPAIR,)), pltpu.SemaphoreType.DMA((9,)), pltpu.SemaphoreType.DMA((1,)), pltpu.SemaphoreType.DMA((8,)),
        ],
        compiler_params=pltpu.CompilerParams(vmem_limit_bytes=100 * 1024 * 1024),
    )(x, mem0, tr(A_Wq), tr(A_Wk), tr(A_Wv), wo, B_wqkv, B_wo)
    return out.reshape(1, S, D)
```

```python
import functools
import jax
import jax.numpy as jnp
from jax.experimental import pallas as pl
from jax.experimental.pallas import tpu as pltpu

S = 2048; D = 640; H = 32; DH = 192; M = 8; SEG = 32; NSEG = S // SEG
NPAIR = H // 2; PW = 2 * DH
BH = 32; BDH = D // BH; BW = 8; BDIL = 2
LOG2E = 1.4426950408889634
NEG = -1e30
f32 = jnp.float32; bf16 = jnp.bfloat16; u32 = jnp.uint32; i32 = jnp.int32
NPRE = 9


def _sched(bq, b1, bh, hc, cuts, wpos, b2):
    s = {}
    s.setdefault(bq, []).append('bqkv')
    s.setdefault((b1, 'post'), []).append('b1fin')
    s.setdefault((bh, 'post'), []).append('bhist')
    s.setdefault((hc, 'post'), []).append('hcopy')
    cs = [0] + list(cuts) + [NPAIR]
    for (g0, g1), p in zip(zip(cs, cs[1:]), wpos):
        s.setdefault(p, []).append(('wo', g0, g1))
    s.setdefault(b2, []).append('b2fin')
    return s


def _bdep(l0, l1):
    d = {}
    for i, g in enumerate(l0): d.setdefault(g, []).append((0, 8 * i, 8))
    for i, g in enumerate(l1): d.setdefault(g, []).append((1, 8 * i, 8))
    return d


_WP = ((13, 'post'), (14, 'k'), (14, 'post'), (15, 'post'))
SCHED = {
    'half': _sched((0, 'pre'), 8, 11, 13, (4, 8, 13), _WP, (15, 'post')),
    'pre': _sched((0, 'post'), 8, 11, 13, (4, 8, 13), _WP, (15, 'post')),
    'full': _sched((0, 'post'), 8, 12, 13, (4, 8, 13), _WP, (15, 'post')),
}
BDEP = {
    'half': _bdep((3, 4, 5, 7), (9, 10, 11, 11)),
    'pre': _bdep((3, 5, 7, 8), (9, 10, 11, 11)),
    'full': _bdep((3, 4, 5, 7), (9, 10, 11, 12)),
}


def _dot(a, b):
    return jnp.dot(a, b, preferred_element_type=f32)


def _dot_nt(a, b):
    return jax.lax.dot_general(a, b, (((1,), (1,)), ((), ())), preferred_element_type=f32)


def _recip(x):
    r = pl.reciprocal(x, approx=True)
    return r * (2.0 - x * r)


def _ln(x):
    m = jnp.mean(x, axis=-1, keepdims=True)
    xc = x - m
    v = jnp.mean(xc * xc, axis=-1, keepdims=True)
    return xc * jax.lax.rsqrt(v + 1e-5)


def _pk(x):
    return pltpu.bitcast(x.astype(bf16), u32)


def _up(x):
    return pltpu.bitcast(x, bf16)


def _ds(start, size, mult):
    return pl.ds(start, size) if isinstance(start, int) else pl.ds(pl.multiple_of(start, mult), size)


def kernel(x_hbm, mem0_hbm, wq_hbm, wk_hbm, wv_hbm, wo_hbm, bqkv_hbm, bwo_hbm, out_hbm,
           wq, wk, wv, wn_ref, wo, bqkv_raw, bwo_raw, bqkv_p, bwo_p, x_ref, mem0_ref, out_ref,
           h_ref, hn_ref, hp_ref, xa_ref, xan_ref, xb_ref, qkv_ref, pre_ref, o_ref,
           bq_ref, kb_ref, vb_ref, bo_ref,
           sem_w, sem_m, sem_b, sem_o):
    RW = PW // 2
    ws = (wq, wk, wv)
    ws_hbm = (wq_hbm.bitcast(u32), wk_hbm.bitcast(u32), wv_hbm.bitcast(u32))
    NWO = 4
    RO = H * DH // 2 // NWO
    X0R = (NPRE + 2) * SEG
    BQR = (0, 104, 208, 320)

    def cp_w(j, g):
        sl = _ds(g * RW, RW, RW)
        return pltpu.make_async_copy(ws_hbm[j].at[sl], ws[j].at[sl], sem_w.at[g])

    def cp_wo(i):
        sl = pl.ds(i * RO, RO)
        return pltpu.make_async_copy(wo_hbm.bitcast(u32).at[sl], wo.at[sl], sem_m.at[3 + i])

    def cp_out(s):
        sl = _ds(s * SEG, SEG, SEG)
        return pltpu.make_async_copy(out_ref.at[sl], out_hbm.at[sl], sem_o.at[0])

    cp_x0 = pltpu.make_async_copy(x_hbm.at[0:X0R], x_ref.at[0:X0R], sem_m.at[0])
    cp_mem = pltpu.make_async_copy(mem0_hbm, mem0_ref, sem_m.at[1])
    cp_x1 = pltpu.make_async_copy(x_hbm.at[X0R:S], x_ref.at[X0R:S], sem_m.at[2])
    cp_bqkv = [pltpu.make_async_copy(bqkv_hbm.bitcast(u32).at[BQR[i]:BQR[i + 1]], bqkv_raw.at[BQR[i]:BQR[i + 1]],
                                     sem_b.at[i]) for i in range(3)]
    cp_bwo = [pltpu.make_async_copy(bwo_hbm.bitcast(u32).at[:, k * 128:(k + 1) * 128], bwo_raw.at[k, 0:D // 2, :],
                                    sem_b.at[3 + k]) for k in range(5)]

    cp_x0.start(); cp_mem.start()
    for g in range(NPAIR):
        if g == 3: cp_bqkv[0].start()
        if g == 5:
            for c in cp_bwo: c.start()
        if g == 6: cp_bqkv[1].start()
        if g == 9: cp_bqkv[2].start()
        for j in range(3): cp_w(j, g).start()
    for i in range(NWO): cp_wo(i).start()
    cp_x1.start()

    bqkv_raw[D // 2:D // 2 + 8, :] = jnp.zeros((8, 3 * D), u32)
    for k in range(5): bwo_raw[k, D // 2:D, :] = jnp.zeros((D // 2, 128), u32)
    xb_ref[...] = jnp.zeros((2 * SEG, D), f32)
    kb_ref[...] = jnp.zeros(kb_ref.shape, f32)
    vb_ref[...] = jnp.zeros(vb_ref.shape, f32)
    xa_ref[SEG:2 * SEG, :] = jnp.zeros((SEG, D), f32)
    h_ref[24:40, :] = jnp.zeros((16, D), u32)
    for j in range(3): qkv_ref[0, j, 0:24, :] = jnp.zeros((24, PW), u32)
    cp_x0.wait(); cp_mem.wait()
    mem0 = mem0_ref[...].astype(f32)
    mem00 = jnp.concatenate([mem0, mem0], axis=0)
    x00 = x_ref[0:SEG, :].astype(f32)
    xa_ref[0:SEG, :] = x00
    hp_ref[0:8, :] = _pk(mem00)
    hp_ref[8:24, :] = _pk(_ln(x00))
    for i in range(NPRE):
        hp_ref[24 + 16 * i:40 + 16 * i, :] = _pk(_ln(x_ref[(i + 2) * SEG:(i + 3) * SEG, :].astype(f32)))

    def perm_wo_unit(e, valid):
        base = jnp.where(valid, e, D // 2)
        w = jnp.concatenate([bwo_raw[k, pl.ds(base, BH, stride=BDH // 2), :] for k in range(5)], axis=1)
        dst = pl.multiple_of(jnp.where(valid, e * BH, D // 2), BH)
        bwo_p[pl.ds(dst, BH // 2), :] = _pk(pltpu.bitcast(w << 16, f32))
        bwo_p[pl.ds(dst + BH // 2, BH // 2), :] = _pk(pltpu.bitcast(w & jnp.uint32(0xFFFF0000), f32))

    lane8 = jax.lax.broadcasted_iota(i32, (8, 128), 1)

    def perm_unit(u, valid):
        rg = u // 3
        j = u - 3 * rg
        r = pl.ds(pl.multiple_of(jnp.where(valid, rg * 8, D // 2), 8), 8)
        srcs = [bqkv_raw[r, pl.ds(pl.multiple_of(j * D + k * 128, 128), 128)] for k in range(5)]
        for n in range(5):
            col = lane8 + n * 128
            s = (col % BH) * BDH + col // BH
            acc = None
            for k in range(5):
                gk = jnp.take_along_axis(srcs[k], s % 128, axis=1)
                acc = gk if acc is None else jnp.where(s // 128 == k, gk, acc)
            bqkv_p[r, pl.ds(pl.multiple_of(j * D + n * 128, 128), 128)] = acc

    def lhs_h(var, lh):
        if var == 'full':
            return _up(h_ref[...])
        if var == 'pre':
            return _up(jnp.concatenate([h_ref[0:8, :], h_ref[24:40, :]], axis=0))
        return _up(jnp.concatenate([h_ref[0:8, :], h_ref[pl.ds(pl.multiple_of(8 + 16 * lh, 8), 16), :]], axis=0))

    def proj(g, j, var, lh):
        y = _pk(_dot(lhs_h(var, lh), _up(wn_ref[g, j])))
        if var == 'full':
            qkv_ref[g, j] = y
        elif var == 'pre':
            qkv_ref[g, j, 0:8, :] = y[0:8]
            qkv_ref[g, j, 24:40, :] = y[8:24]
        else:
            qkv_ref[g, j, 0:24, :] = y

    lo64 = jax.lax.broadcasted_iota(i32, (48, 128), 1) < 64
    rr = jax.lax.broadcasted_iota(i32, (48, 96), 0)
    cc = jax.lax.broadcasted_iota(i32, (48, 96), 1)
    ck = jnp.where(cc >= 48, cc - 48, cc)
    row16 = jax.lax.broadcasted_iota(i32, (16, 128), 0)
    row96 = jax.lax.broadcasted_iota(i32, (16, 96), 0)
    sc = (DH ** -0.5) * LOG2E

    def smask(l):
        memk = (ck >= 8 * l) & (ck < 8 * l + 8)
        tokk = (ck >= 16) & ((rr < 16) | (ck <= rr))
        return jnp.where(memk | tokk, 0.0, NEG).astype(f32)

    bias = [smask(0), smask(1)]
    h0c = [cc < 48, (cc < 16) | (cc >= 64)]

    def softmax2(s, bias_l, hc):
        s = s * sc + bias_l
        m0 = jnp.max(jnp.where(hc, s, NEG), axis=1, keepdims=True)
        m1 = jnp.max(jnp.where(hc, NEG, s), axis=1, keepdims=True)
        p = jnp.exp2(s - jnp.where(hc, m0, m1))
        s0 = jnp.sum(jnp.where(hc, p, 0.0), axis=1, keepdims=True)
        s1 = jnp.sum(jnp.where(hc, 0.0, p), axis=1, keepdims=True)
        return p * _recip(jnp.where(hc, s0, s1))

    def lo_(a): return jnp.where(lo64[0:a.shape[0]], a, jnp.zeros_like(a))
    def hi_(a): return jnp.where(lo64[0:a.shape[0]], jnp.zeros_like(a), a)

    def bd1(g, j):
        a = _up(qkv_ref[g, j, 0:24, :])
        z = jnp.zeros((48, 128), bf16)
        a1 = a[:, 128:256]
        top = jnp.concatenate([a[:, 0:128], lo_(a1), z], axis=1)
        bot = jnp.concatenate([z, hi_(a1), a[:, 256:384]], axis=1)
        return jnp.concatenate([top, bot], axis=0)

    def qk1(g, bias_l):
        return softmax2(_dot_nt(_up(qkv_ref[g, 0, 0:24, :]), bd1(g, 1)), bias_l, h0c[0])

    def pv1(g, p, vb=None):
        vb = bd1(g, 2) if vb is None else vb
        o_ref[g, 0:24, :] = _pk(_dot(p.astype(bf16), vb))

    def parts(j, g, pre):
        m_ = _up(qkv_ref[g, j, 0:8, :])
        t1 = _up(qkv_ref[g, j, 8:24, :] if pre is None else pre_ref[g, j, pl.ds(pl.multiple_of(16 * pre, 16), 16), :])
        return m_, t1, _up(qkv_ref[g, j, 24:40, :])

    def rhs3(j, g, pre):
        m_, t1, t2 = parts(j, g, pre)
        z16 = jnp.zeros((16, 128), bf16)
        cat = lambda *xs: jnp.concatenate(xs, axis=0)
        r0 = cat(m_[:, 0:128], t1[:, 0:128], z16, t2[:, 0:128])
        r2 = cat(z16, t2[:, 256:384], m_[:, 256:384], t1[:, 256:384])
        m1, a1, b1 = m_[:, 128:256], t1[:, 128:256], t2[:, 128:256]
        rt0 = cat(lo_(m1), lo_(a1), hi_(m1), hi_(a1))
        rt1 = cat(lo_(m1), hi_(b1), hi_(m1), lo_(b1))
        return r0, r2, rt0, rt1

    def qk2(g, pre):
        q = jnp.concatenate(parts(0, g, pre), axis=0)
        r0, r2, rt0, rt1 = rhs3(1, g, pre)
        a0 = _dot_nt(q[:, 0:128], r0)
        a2 = _dot_nt(q[:, 256:384], r2)
        q1 = jnp.concatenate([q[0:16, 128:256], q[48:80, 128:256]], axis=0)
        s0 = jnp.where(h0c[0], a0[0:48], a2[0:48]) + _dot_nt(q[0:48, 128:256], rt0)
        a0l = jnp.concatenate([a0[0:16], a0[48:80]], axis=0)
        a2l = jnp.concatenate([a2[0:16], a2[48:80]], axis=0)
        s1 = jnp.where(h0c[1], a0l, a2l) + _dot_nt(q1, rt1)
        return [softmax2(s0, bias[0], h0c[0]), softmax2(s1, bias[1], h0c[1])]

    def pv2(g, ps, pre):
        p0, p1 = ps
        r0, r2, rt0, rt1 = rhs3(2, g, pre)

        def stack(x0, x1):
            mm = jnp.where(row96 < 8, x0[0:16], x1[0:16])
            return jnp.concatenate([mm, x0[16:48], x1[16:48]], axis=0).astype(bf16)

        o0 = _dot(stack(jnp.where(h0c[0], p0, 0.0), jnp.where(h0c[1], p1, 0.0)), r0)
        o2 = _dot(stack(jnp.where(h0c[0], 0.0, p0), jnp.where(h0c[1], 0.0, p1)), r2)
        t0 = _dot(p0.astype(bf16), rt0)
        t1 = _dot(p1.astype(bf16), rt1)
        om = jnp.where(row16 < 8, t0[0:16], t1[0:16])
        o1 = jnp.concatenate([om, t0[16:48], t1[16:48]], axis=0)
        o_ref[g] = _pk(jnp.concatenate([o0, o1, o2], axis=1))

    def wo_part(g0, g1, half):
        o = jnp.concatenate([_up(o_ref[g, 0:24, :] if half else o_ref[g]) for g in range(g0, g1)], axis=1)
        return _dot(o, _up(wo[g0 * RW:g1 * RW, :]))

    rC = jax.lax.broadcasted_iota(i32, (16, 128), 0)
    bsc = (BDH ** -0.5) * LOG2E

    def b_qkv(layers=(0, 1)):
        r0 = SEG * layers[0]; r1 = SEG * layers[-1] + SEG
        y = _dot(_ln(xb_ref[r0:r1, :]).astype(bf16), _up(bqkv_p[0:D // 2, :]))
        bq_ref[r0:r1, :] = y[:, 0:D]
        for l in layers:
            kb_ref[l, 16:48, :] = y[SEG * l - r0:SEG * l - r0 + SEG, D:2 * D]
            vb_ref[l, 16:48, :] = y[SEG * l - r0:SEG * l - r0 + SEG, 2 * D:3 * D]

    def b_attn(t, l, r0, nr):
        q = bq_ref[SEG * l + r0:SEG * l + r0 + nr, :]
        pos = (t - 1 - 2 * l) * SEG + r0 + rC[0:nr]
        lg = []
        for w in range(BW):
            off = 16 - BDIL * w + r0
            pr = q * kb_ref[l, off:off + nr, :]
            a = pr[:, 0:128] + pr[:, 128:256] + pr[:, 256:384] + pr[:, 384:512] + pr[:, 512:640]
            a = a + pltpu.roll(a, 64, 1)
            a = (a + pltpu.roll(a, 32, 1)) * bsc
            lg.append(a if w == 0 else jnp.where(pos >= BDIL * w, a, NEG))
        m = lg[0]
        for w in range(1, BW): m = jnp.maximum(m, lg[w])
        ps = [jnp.exp2(a - m) for a in lg]
        den = ps[0]
        for w in range(1, BW): den = den + ps[w]
        inv = _recip(den)
        acc = None
        for w in range(BW):
            off = 16 - BDIL * w + r0
            tt = jnp.concatenate([ps[w] * inv] * 5, axis=1) * vb_ref[l, off:off + nr, :]
            acc = tt if acc is None else acc + tt
        bo_ref[SEG * l + r0:SEG * l + r0 + nr, :] = acc
        z = acc[0:8, 0:128]
        for a_ in range(nr // 8):
            for b_ in range(5):
                if a_ or b_: z = jnp.maximum(z, acc[8 * a_:8 * a_ + 8, 128 * b_:128 * b_ + 128])
        return z

    def b_hist():
        for l in range(2):
            kb_ref[l, 0:16, :] = kb_ref[l, 32:48, :]
            vb_ref[l, 0:16, :] = vb_ref[l, 32:48, :]

    def b_out(l):
        return xb_ref[SEG * l:SEG * l + SEG, :] + _dot(bo_ref[SEG * l:SEG * l + SEG, :].astype(bf16),
                                                       _up(bwo_p[0:D // 2, :]))

    def b1_finish(t):
        x2 = b_out(0)
        xn = x_ref[_ds(jnp.minimum(t + 1, NSEG - 1) * SEG, SEG, SEG), :].astype(f32)
        xan_ref[0:SEG, :] = xn
        xan_ref[SEG:2 * SEG, :] = x2
        hn_ref[0:16, :] = _pk(_ln(xn))
        hn_ref[16:32, :] = _pk(_ln(x2))

    def b2_finish(t):
        out_ref[_ds(jnp.maximum(t - 3, 0) * SEG, SEG, SEG), :] = b_out(1).astype(bf16)

    def end_step(t, oa, lh):
        if lh is None:
            xb_ref[...] = xa_ref[...] + oa[16:80]
        else:
            sl = _ds(SEG * lh, SEG, SEG)
            xb_ref[sl, :] = xa_ref[sl, :] + oa[16:48]
        xa_ref[...] = xan_ref[...]
        r16 = jax.lax.broadcasted_iota(i32, (16, D), 0)
        h_ref[0:8, :] = _pk(jnp.where((r16 >= 8) & (t < 2), mem00, oa[0:16]))

    def step_body(t, var):
        half = var == 'half'
        lh = jnp.where(t < 2, 0, 1) if half else None
        bias_h = smask(lh) if half else None
        pre = jnp.clip(t - 2, 0, NPRE - 1) if var == 'pre' else None
        st = {}
        pp = {}

        def extra(i, pos):
            for name in SCHED[var].get((i, pos), ()):
                if name == 'bqkv': b_qkv()
                elif name == 'bhist': b_hist()
                elif name == 'hcopy': h_ref[8:40, :] = hn_ref[...]
                elif name == 'b1fin': b1_finish(t)
                elif name == 'b2fin': b2_finish(t)
                else:
                    part = wo_part(name[1], name[2], half)
                    st['oa'] = part if 'oa' not in st else st['oa'] + part

        for i in range(-2, NPAIR):
            g2, g1, g0 = i + 2, i + 1, i
            extra(i, 'pre')
            for j in range(3):
                if g2 < NPAIR: proj(g2, j, var, lh)
                extra(i, 'qkv'[j])
            if 0 <= g1 < NPAIR:
                pp[g1] = [qk1(g1, bias_h)] if half else qk2(g1, pre)
            if 0 <= g0:
                pg = pp.pop(g0)
                for (l, r0, nr) in BDEP[var].get(g0, ()):
                    z = b_attn(t, l, r0, nr)
                    pg[0] = jnp.concatenate([jnp.where(t < 0, z[:, 0:96], pg[0][0:8]), pg[0][8:]], axis=0)
                if half: pv1(g0, pg[0])
                else: pv2(g0, pg, pre)
            extra(i, 'post')
        end_step(t, st['oa'], lh)

    def make_step(var):
        def step(t, c):
            step_body(t, var)
            @pl.when(t >= 3)
            def _():
                cp_out(t - 3).start()
            return c
        return step

    def warm(g, c):
        gp = jnp.maximum(g - 1, 0)
        for i, g_ in enumerate((3, 6, 10)):
            pl.when(g == g_)(cp_bqkv[i].wait)

        @pl.when(g == 6)
        def _():
            for c_ in cp_bwo: c_.wait()

        for j in range(3): cp_w(j, g).wait()
        sl = pl.ds(pl.multiple_of(g * RW, RW), RW)

        def wproj(j):
            y = _pk(_dot_nt(_up(hp_ref[...]), _up(ws[j][sl, :])))
            qkv_ref[g, j, 0:24, :] = y[0:24]
            pre_ref[g, j] = y[24:]

        vb = bd1(gp, 2)
        p = qk1(gp, bias[0])
        wproj(0); wproj(1)
        pv1(gp, p, vb)
        wproj(2)
        for j in range(3):
            wn_ref[g, j] = _pk(_up(ws[j][sl, :]).T)
        for k in range(10): perm_unit(jnp.clip(10 * (g - 3) + k, 0, 119), g >= 3)
        perm_wo_unit(jnp.clip(g - 6, 0, 9), g >= 6)
        return c

    jax.lax.fori_loop(0, NPAIR, warm, 0)
    pv1(NPAIR - 1, qk1(NPAIR - 1, bias[0]))
    for i in range(NWO): cp_wo(i).wait()
    oa = wo_part(0, NPAIR, True)
    xn = x_ref[SEG:2 * SEG, :].astype(f32)
    xan_ref[0:SEG, :] = xn
    xan_ref[SEG:2 * SEG, :] = jnp.zeros((SEG, D), f32)
    h_ref[8:24, :] = _pk(_ln(xn))
    end_step(0, oa, 0)

    def phase(ph, c):
        jax.lax.fori_loop(jnp.where(ph == 0, 1, NSEG), jnp.where(ph == 0, 2, NSEG + 2), make_step('half'), 0)

        @pl.when(ph == 0)
        def _():
            cp_x1.wait()
            jax.lax.fori_loop(2, NPRE + 2, make_step('pre'), 0)
            jax.lax.fori_loop(NPRE + 2, NSEG, make_step('full'), 0)
        return c

    jax.lax.fori_loop(0, 2, phase, 0)

    b_qkv((1,))
    for c in range(2): b_attn(NSEG + 2, 1, 16 * c, 16)
    b2_finish(NSEG + 2)
    cp_out(NSEG - 1).start()

    pltpu.make_async_copy(out_ref, out_hbm, sem_o.at[0]).wait()


@functools.partial(jax.jit, static_argnames=("A_seg_len",))
def pallas_interleave_layers__memory_aug_recurrent_mem_tr__sliding_local_dilated__prompt_kernel(
        A_x, A_mem0, A_Wq, A_Wk, A_Wv, A_Wo, A_seg_len, B_x, B_wqkv, B_wo):
    assert A_seg_len == SEG
    del B_x
    x = A_x.reshape(S, D)
    mem0 = A_mem0.reshape(M, D)
    tr = lambda w: jnp.transpose(w, (1, 2, 0)).reshape(H * DH, D)
    wo = A_Wo.reshape(H * DH, D)
    hbm = pl.BlockSpec(memory_space=pl.ANY)
    WR = H * DH // 2
    vmem = pltpu.VMEM
    out = pl.pallas_call(
        kernel,
        out_shape=jax.ShapeDtypeStruct((S, D), bf16),
        in_specs=[hbm] * 8,
        out_specs=hbm,
        scratch_shapes=[
            vmem((WR, D), u32), vmem((WR, D), u32), vmem((WR, D), u32),
            vmem((NPAIR, 3, D // 2, PW), u32), vmem((WR, D), u32),
            vmem((D // 2 + 8, 3 * D), u32), vmem((5, D, 128), u32),
            vmem((D // 2 + 8, 3 * D), u32), vmem((D // 2 + 32, D), u32),
            vmem((S, D), bf16), vmem((M, D), bf16), vmem((S, D), bf16),
            vmem((40, D), u32), vmem((32, D), u32), vmem((24 + 16 * NPRE, D), u32),
            vmem((64, D), f32), vmem((64, D), f32), vmem((64, D), f32),
            vmem((NPAIR, 3, 40, PW), u32), vmem((NPAIR, 3, 16 * NPRE, PW), u32),
            vmem((NPAIR, 40, PW), u32),
            vmem((64, D), f32), vmem((2, 48, D), f32), vmem((2, 48, D), f32), vmem((64, D), f32),
            pltpu.SemaphoreType.DMA((NPAIR,)), pltpu.SemaphoreType.DMA((7,)),
            pltpu.SemaphoreType.DMA((8,)), pltpu.SemaphoreType.DMA((1,)),
        ],
        compiler_params=pltpu.CompilerParams(vmem_limit_bytes=100 * 1024 * 1024),
    )(x, mem0, tr(A_Wq), tr(A_Wk), tr(A_Wv), wo, B_wqkv, B_wo)
    return out.reshape(1, S, D)
```

```python
import functools
import jax
import jax.numpy as jnp
from jax.experimental import pallas as pl
from jax.experimental.pallas import tpu as pltpu

S = 2048; D = 640; H = 32; DH = 192; M = 8; SEG = 32; NSEG = S // SEG
NPAIR = H // 2; PW = 2 * DH
BH = 32; BDH = D // BH; BW = 8; BDIL = 2
LOG2E = 1.4426950408889634
NEG = -1e30
f32 = jnp.float32; bf16 = jnp.bfloat16; u32 = jnp.uint32; i32 = jnp.int32
NPRE = 9


def _sched(bq, b1, bh, hc, cuts, wpos, b2):
    s = {}
    s.setdefault(bq, []).append('bqkv')
    s.setdefault((b1, 'post'), []).append('b1fin')
    s.setdefault((bh, 'post'), []).append('bhist')
    s.setdefault((hc, 'post'), []).append('hcopy')
    cs = [0] + list(cuts) + [NPAIR]
    for (g0, g1), p in zip(zip(cs, cs[1:]), wpos):
        s.setdefault(p, []).append(('wo', g0, g1))
    s.setdefault(b2, []).append('b2fin')
    return s


def _bdep(l0, l1):
    d = {}
    for i, g in enumerate(l0): d.setdefault(g, []).append((0, 8 * i, 8))
    for i, g in enumerate(l1): d.setdefault(g, []).append((1, 8 * i, 8))
    return d


_WP = ((13, 'post'), (14, 'k'), (14, 'post'), (15, 'post'))
SCHED = {
    'half': _sched((0, 'pre'), 8, 11, 13, (4, 8, 13), _WP, (15, 'post')),
    'pre': _sched((0, 'post'), 8, 11, 13, (4, 8, 13), _WP, (15, 'post')),
    'full': _sched((0, 'post'), 8, 12, 13, (4, 8, 13), _WP, (15, 'post')),
}
BDEP = {
    'half': _bdep((3, 4, 5, 7), (9, 10, 11, 11)),
    'pre': _bdep((3, 5, 7, 8), (9, 10, 11, 11)),
    'full': _bdep((3, 4, 5, 7), (9, 10, 11, 12)),
}


def _dot(a, b):
    return jnp.dot(a, b, preferred_element_type=f32)


def _dot_nt(a, b):
    return jax.lax.dot_general(a, b, (((1,), (1,)), ((), ())), preferred_element_type=f32)


def _recip(x):
    r = pl.reciprocal(x, approx=True)
    return r * (2.0 - x * r)


def _ln(x):
    m = jnp.mean(x, axis=-1, keepdims=True)
    xc = x - m
    v = jnp.mean(xc * xc, axis=-1, keepdims=True)
    return xc * jax.lax.rsqrt(v + 1e-5)


def _pk(x):
    return pltpu.bitcast(x.astype(bf16), u32)


def _up(x):
    return pltpu.bitcast(x, bf16)


def _ds(start, size, mult):
    return pl.ds(start, size) if isinstance(start, int) else pl.ds(pl.multiple_of(start, mult), size)


def kernel(x_hbm, mem0_hbm, wq_hbm, wk_hbm, wv_hbm, wo_hbm, bqkv_hbm, bwo_hbm, out_hbm,
           wq, wk, wv, wn_ref, wo, bqkv_raw, bwo_raw, bqkv_p, bwo_p, x_ref, mem0_ref, out_ref,
           h_ref, hn_ref, hp_ref, xa_ref, xan_ref, xb_ref, qkv_ref, pre_ref, o_ref,
           bq_ref, kb_ref, vb_ref, bo_ref,
           sem_w, sem_m, sem_b, sem_o):
    RW = PW // 2
    ws = (wq, wk, wv)
    ws_hbm = (wq_hbm.bitcast(u32), wk_hbm.bitcast(u32), wv_hbm.bitcast(u32))
    NWO = 4
    RO = H * DH // 2 // NWO
    X0R = (NPRE + 2) * SEG
    BQR = (0, 104, 208, 320)

    def cp_w(j, g):
        sl = _ds(g * RW, RW, RW)
        sem = sem_w.at[NPAIR + j] if (isinstance(g, int) and g == 0) else sem_w.at[g]
        return pltpu.make_async_copy(ws_hbm[j].at[sl], ws[j].at[sl], sem)

    def cp_wo(i):
        sl = pl.ds(i * RO, RO)
        return pltpu.make_async_copy(wo_hbm.bitcast(u32).at[sl], wo.at[sl], sem_m.at[3 + i])

    def cp_out(s):
        sl = _ds(s * SEG, SEG, SEG)
        return pltpu.make_async_copy(out_ref.at[sl], out_hbm.at[sl], sem_o.at[0])

    cp_x0 = pltpu.make_async_copy(x_hbm.at[0:X0R], x_ref.at[0:X0R], sem_m.at[0])
    cp_mem = pltpu.make_async_copy(mem0_hbm, mem0_ref, sem_m.at[1])
    cp_x1 = pltpu.make_async_copy(x_hbm.at[X0R:S], x_ref.at[X0R:S], sem_m.at[2])
    cp_bqkv = [pltpu.make_async_copy(bqkv_hbm.bitcast(u32).at[BQR[i]:BQR[i + 1]], bqkv_raw.at[BQR[i]:BQR[i + 1]],
                                     sem_b.at[i]) for i in range(3)]
    cp_bwo = [pltpu.make_async_copy(bwo_hbm.bitcast(u32).at[:, k * 128:(k + 1) * 128], bwo_raw.at[k, 0:D // 2, :],
                                    sem_b.at[3 + k]) for k in range(5)]

    cp_x0.start(); cp_mem.start()
    for g in range(NPAIR):
        if g == 3: cp_bqkv[0].start()
        if g == 5:
            for c in cp_bwo: c.start()
        if g == 6: cp_bqkv[1].start()
        if g == 9: cp_bqkv[2].start()
        for j in range(3): cp_w(j, g).start()
    for i in range(NWO): cp_wo(i).start()
    cp_x1.start()

    bqkv_raw[D // 2:D // 2 + 8, :] = jnp.zeros((8, 3 * D), u32)
    for k in range(5): bwo_raw[k, D // 2:D, :] = jnp.zeros((D // 2, 128), u32)
    xb_ref[...] = jnp.zeros((2 * SEG, D), f32)
    kb_ref[...] = jnp.zeros(kb_ref.shape, f32)
    vb_ref[...] = jnp.zeros(vb_ref.shape, f32)
    xa_ref[SEG:2 * SEG, :] = jnp.zeros((SEG, D), f32)
    h_ref[24:40, :] = jnp.zeros((16, D), u32)
    cp_x0.wait(); cp_mem.wait()
    mem0 = mem0_ref[...].astype(f32)
    mem00 = jnp.concatenate([mem0, mem0], axis=0)
    x00 = x_ref[0:SEG, :].astype(f32)
    xa_ref[0:SEG, :] = x00
    hp_ref[0:8, :] = _pk(mem00)
    hp_ref[8:24, :] = _pk(_ln(x00))
    for i in range(NPRE):
        hp_ref[24 + 16 * i:40 + 16 * i, :] = _pk(_ln(x_ref[(i + 2) * SEG:(i + 3) * SEG, :].astype(f32)))

    def perm_wo_unit(e, valid):
        base = jnp.where(valid, e, D // 2)
        w = jnp.concatenate([bwo_raw[k, pl.ds(base, BH, stride=BDH // 2), :] for k in range(5)], axis=1)
        dst = pl.multiple_of(jnp.where(valid, e * BH, D // 2), BH)
        bwo_p[pl.ds(dst, BH // 2), :] = _pk(pltpu.bitcast(w << 16, f32))
        bwo_p[pl.ds(dst + BH // 2, BH // 2), :] = _pk(pltpu.bitcast(w & jnp.uint32(0xFFFF0000), f32))

    lane8 = jax.lax.broadcasted_iota(i32, (8, 128), 1)

    def perm_unit(u, valid):
        rg = u // 3
        j = u - 3 * rg
        r = pl.ds(pl.multiple_of(jnp.where(valid, rg * 8, D // 2), 8), 8)
        srcs = [bqkv_raw[r, pl.ds(pl.multiple_of(j * D + k * 128, 128), 128)] for k in range(5)]
        for n in range(5):
            col = lane8 + n * 128
            s = (col % BH) * BDH + col // BH
            acc = None
            for k in range(5):
                gk = jnp.take_along_axis(srcs[k], s % 128, axis=1)
                acc = gk if acc is None else jnp.where(s // 128 == k, gk, acc)
            bqkv_p[r, pl.ds(pl.multiple_of(j * D + n * 128, 128), 128)] = acc

    def lhs_h(var, lh):
        if var == 'full':
            return _up(h_ref[...])
        if var == 'pre':
            return _up(jnp.concatenate([h_ref[0:8, :], h_ref[24:40, :]], axis=0))
        return _up(jnp.concatenate([h_ref[0:8, :], h_ref[pl.ds(pl.multiple_of(8 + 16 * lh, 8), 16), :]], axis=0))

    def proj(g, j, var, lh):
        y = _pk(_dot(lhs_h(var, lh), _up(wn_ref[g, j])))
        if var == 'full':
            qkv_ref[g, j] = y
        elif var == 'pre':
            qkv_ref[g, j, 0:8, :] = y[0:8]
            qkv_ref[g, j, 24:40, :] = y[8:24]
        else:
            qkv_ref[g, j, 0:24, :] = y

    lo64 = jax.lax.broadcasted_iota(i32, (48, 128), 1) < 64
    rr = jax.lax.broadcasted_iota(i32, (48, 96), 0)
    cc = jax.lax.broadcasted_iota(i32, (48, 96), 1)
    ck = jnp.where(cc >= 48, cc - 48, cc)
    row16 = jax.lax.broadcasted_iota(i32, (16, 128), 0)
    row96 = jax.lax.broadcasted_iota(i32, (16, 96), 0)
    sc = (DH ** -0.5) * LOG2E

    def smask(l):
        memk = (ck >= 8 * l) & (ck < 8 * l + 8)
        tokk = (ck >= 16) & ((rr < 16) | (ck <= rr))
        return jnp.where(memk | tokk, 0.0, NEG).astype(f32)

    bias = [smask(0), smask(1)]
    h0c = [cc < 48, (cc < 16) | (cc >= 64)]

    def softmax2(s, bias_l, hc):
        s = s * sc + bias_l
        m0 = jnp.max(jnp.where(hc, s, NEG), axis=1, keepdims=True)
        m1 = jnp.max(jnp.where(hc, NEG, s), axis=1, keepdims=True)
        p = jnp.exp2(s - jnp.where(hc, m0, m1))
        s0 = jnp.sum(jnp.where(hc, p, 0.0), axis=1, keepdims=True)
        s1 = jnp.sum(jnp.where(hc, 0.0, p), axis=1, keepdims=True)
        return p * _recip(jnp.where(hc, s0, s1))

    def lo_(a): return jnp.where(lo64[0:a.shape[0]], a, jnp.zeros_like(a))
    def hi_(a): return jnp.where(lo64[0:a.shape[0]], jnp.zeros_like(a), a)

    def bd1(g, j):
        a = _up(qkv_ref[g, j, 0:24, :])
        z = jnp.zeros((48, 128), bf16)
        a1 = a[:, 128:256]
        top = jnp.concatenate([a[:, 0:128], lo_(a1), z], axis=1)
        bot = jnp.concatenate([z, hi_(a1), a[:, 256:384]], axis=1)
        return jnp.concatenate([top, bot], axis=0)

    def qk1(g, bias_l):
        return softmax2(_dot_nt(_up(qkv_ref[g, 0, 0:24, :]), bd1(g, 1)), bias_l, h0c[0])

    def pv1(g, p, vb=None):
        vb = bd1(g, 2) if vb is None else vb
        o_ref[g, 0:24, :] = _pk(_dot(p.astype(bf16), vb))

    def parts(j, g, pre):
        m_ = _up(qkv_ref[g, j, 0:8, :])
        t1 = _up(qkv_ref[g, j, 8:24, :] if pre is None else pre_ref[g, j, pl.ds(pl.multiple_of(16 * pre, 16), 16), :])
        return m_, t1, _up(qkv_ref[g, j, 24:40, :])

    def rhs3(j, g, pre):
        m_, t1, t2 = parts(j, g, pre)
        z16 = jnp.zeros((16, 128), bf16)
        cat = lambda *xs: jnp.concatenate(xs, axis=0)
        r0 = cat(m_[:, 0:128], t1[:, 0:128], z16, t2[:, 0:128])
        r2 = cat(z16, t2[:, 256:384], m_[:, 256:384], t1[:, 256:384])
        m1, a1, b1 = m_[:, 128:256], t1[:, 128:256], t2[:, 128:256]
        rt0 = cat(lo_(m1), lo_(a1), hi_(m1), hi_(a1))
        rt1 = cat(lo_(m1), hi_(b1), hi_(m1), lo_(b1))
        return r0, r2, rt0, rt1

    def qk2(g, pre):
        q = jnp.concatenate(parts(0, g, pre), axis=0)
        r0, r2, rt0, rt1 = rhs3(1, g, pre)
        a0 = _dot_nt(q[:, 0:128], r0)
        a2 = _dot_nt(q[:, 256:384], r2)
        q1 = jnp.concatenate([q[0:16, 128:256], q[48:80, 128:256]], axis=0)
        s0 = jnp.where(h0c[0], a0[0:48], a2[0:48]) + _dot_nt(q[0:48, 128:256], rt0)
        a0l = jnp.concatenate([a0[0:16], a0[48:80]], axis=0)
        a2l = jnp.concatenate([a2[0:16], a2[48:80]], axis=0)
        s1 = jnp.where(h0c[1], a0l, a2l) + _dot_nt(q1, rt1)
        return [softmax2(s0, bias[0], h0c[0]), softmax2(s1, bias[1], h0c[1])]

    def pv2(g, ps, pre):
        p0, p1 = ps
        r0, r2, rt0, rt1 = rhs3(2, g, pre)

        def stack(x0, x1):
            mm = jnp.where(row96 < 8, x0[0:16], x1[0:16])
            return jnp.concatenate([mm, x0[16:48], x1[16:48]], axis=0).astype(bf16)

        o0 = _dot(stack(jnp.where(h0c[0], p0, 0.0), jnp.where(h0c[1], p1, 0.0)), r0)
        o2 = _dot(stack(jnp.where(h0c[0], 0.0, p0), jnp.where(h0c[1], 0.0, p1)), r2)
        t0 = _dot(p0.astype(bf16), rt0)
        t1 = _dot(p1.astype(bf16), rt1)
        om = jnp.where(row16 < 8, t0[0:16], t1[0:16])
        o1 = jnp.concatenate([om, t0[16:48], t1[16:48]], axis=0)
        o_ref[g] = _pk(jnp.concatenate([o0, o1, o2], axis=1))

    def wo_part(g0, g1, half):
        o = jnp.concatenate([_up(o_ref[g, 0:24, :] if half else o_ref[g]) for g in range(g0, g1)], axis=1)
        return _dot(o, _up(wo[g0 * RW:g1 * RW, :]))

    rC = jax.lax.broadcasted_iota(i32, (16, 128), 0)
    bsc = (BDH ** -0.5) * LOG2E

    def b_qkv(layers=(0, 1)):
        r0 = SEG * layers[0]; r1 = SEG * layers[-1] + SEG
        y = _dot(_ln(xb_ref[r0:r1, :]).astype(bf16), _up(bqkv_p[0:D // 2, :]))
        bq_ref[r0:r1, :] = y[:, 0:D]
        for l in layers:
            kb_ref[l, 16:48, :] = y[SEG * l - r0:SEG * l - r0 + SEG, D:2 * D]
            vb_ref[l, 16:48, :] = y[SEG * l - r0:SEG * l - r0 + SEG, 2 * D:3 * D]

    def b_attn(t, l, r0, nr):
        q = bq_ref[SEG * l + r0:SEG * l + r0 + nr, :]
        pos = (t - 1 - 2 * l) * SEG + r0 + rC[0:nr]
        lg = []
        for w in range(BW):
            off = 16 - BDIL * w + r0
            pr = q * kb_ref[l, off:off + nr, :]
            a = pr[:, 0:128] + pr[:, 128:256] + pr[:, 256:384] + pr[:, 384:512] + pr[:, 512:640]
            a = a + pltpu.roll(a, 64, 1)
            a = (a + pltpu.roll(a, 32, 1)) * bsc
            lg.append(a if w == 0 else jnp.where(pos >= BDIL * w, a, NEG))
        m = lg[0]
        for w in range(1, BW): m = jnp.maximum(m, lg[w])
        ps = [jnp.exp2(a - m) for a in lg]
        den = ps[0]
        for w in range(1, BW): den = den + ps[w]
        inv = _recip(den)
        acc = None
        for w in range(BW):
            off = 16 - BDIL * w + r0
            tt = jnp.concatenate([ps[w] * inv] * 5, axis=1) * vb_ref[l, off:off + nr, :]
            acc = tt if acc is None else acc + tt
        bo_ref[SEG * l + r0:SEG * l + r0 + nr, :] = acc
        z = acc[0:8, 0:128]
        for a_ in range(nr // 8):
            for b_ in range(5):
                if a_ or b_: z = jnp.maximum(z, acc[8 * a_:8 * a_ + 8, 128 * b_:128 * b_ + 128])
        return z

    def b_hist():
        for l in range(2):
            kb_ref[l, 0:16, :] = kb_ref[l, 32:48, :]
            vb_ref[l, 0:16, :] = vb_ref[l, 32:48, :]

    def b_out(l):
        return xb_ref[SEG * l:SEG * l + SEG, :] + _dot(bo_ref[SEG * l:SEG * l + SEG, :].astype(bf16),
                                                       _up(bwo_p[0:D // 2, :]))

    def b1_finish(t):
        x2 = b_out(0)
        xn = x_ref[_ds(jnp.minimum(t + 1, NSEG - 1) * SEG, SEG, SEG), :].astype(f32)
        xan_ref[0:SEG, :] = xn
        xan_ref[SEG:2 * SEG, :] = x2
        hn_ref[0:16, :] = _pk(_ln(xn))
        hn_ref[16:32, :] = _pk(_ln(x2))

    def b2_finish(t):
        out_ref[_ds(jnp.maximum(t - 3, 0) * SEG, SEG, SEG), :] = b_out(1).astype(bf16)

    def end_step(t, oa, lh):
        if lh is None:
            xb_ref[...] = xa_ref[...] + oa[16:80]
        else:
            sl = _ds(SEG * lh, SEG, SEG)
            xb_ref[sl, :] = xa_ref[sl, :] + oa[16:48]
        xa_ref[...] = xan_ref[...]
        r16 = jax.lax.broadcasted_iota(i32, (16, D), 0)
        h_ref[0:8, :] = _pk(jnp.where((r16 >= 8) & (t < 2), mem00, oa[0:16]))

    def step_body(t, var):
        half = var == 'half'
        lh = jnp.where(t < 2, 0, 1) if half else None
        bias_h = smask(lh) if half else None
        pre = jnp.clip(t - 2, 0, NPRE - 1) if var == 'pre' else None
        st = {}
        pp = {}

        def extra(i, pos):
            for name in SCHED[var].get((i, pos), ()):
                if name == 'bqkv': b_qkv()
                elif name == 'bhist': b_hist()
                elif name == 'hcopy': h_ref[8:40, :] = hn_ref[...]
                elif name == 'b1fin': b1_finish(t)
                elif name == 'b2fin': b2_finish(t)
                else:
                    part = wo_part(name[1], name[2], half)
                    st['oa'] = part if 'oa' not in st else st['oa'] + part

        for i in range(-2, NPAIR):
            g2, g1, g0 = i + 2, i + 1, i
            extra(i, 'pre')
            for j in range(3):
                if g2 < NPAIR: proj(g2, j, var, lh)
                extra(i, 'qkv'[j])
            if 0 <= g1 < NPAIR:
                pp[g1] = [qk1(g1, bias_h)] if half else qk2(g1, pre)
            if 0 <= g0:
                pg = pp.pop(g0)
                for (l, r0, nr) in BDEP[var].get(g0, ()):
                    z = b_attn(t, l, r0, nr)
                    pg[0] = jnp.concatenate([jnp.where(t < 0, z[:, 0:96], pg[0][0:8]), pg[0][8:]], axis=0)
                if half: pv1(g0, pg[0])
                else: pv2(g0, pg, pre)
            extra(i, 'post')
        end_step(t, st['oa'], lh)

    def make_step(var):
        def step(t, c):
            step_body(t, var)
            @pl.when(t >= 3)
            def _():
                cp_out(jnp.maximum(t - 3, 0)).start()
            return c
        return step

    def warm(g, c, first=False):
        sl = _ds(g * RW, RW, RW)

        def wproj(j):
            y = _pk(_dot_nt(_up(hp_ref[...]), _up(ws[j][sl, :])))
            qkv_ref[g, j, 0:24, :] = y[0:24]
            pre_ref[g, j] = y[24:]

        if first:
            for j in range(3):
                cp_w(j, g).wait()
                wproj(j)
        else:
            for i, g_ in enumerate((3, 6, 10)):
                pl.when(g == g_)(cp_bqkv[i].wait)

            @pl.when(g == 6)
            def _():
                for c_ in cp_bwo: c_.wait()

            for j in range(3): cp_w(j, g).wait()
            vb = bd1(g - 1, 2)
            p = qk1(g - 1, bias[0])
            wproj(0); wproj(1)
            pv1(g - 1, p, vb)
            wproj(2)
        for j in range(3):
            wn_ref[g, j] = _pk(_up(ws[j][sl, :]).T)
        if not first:
            for k in range(10): perm_unit(jnp.clip(10 * (g - 3) + k, 0, 119), g >= 3)
            perm_wo_unit(jnp.clip(g - 6, 0, 9), g >= 6)
        return c

    warm(0, 0, first=True)
    jax.lax.fori_loop(1, NPAIR, warm, 0)
    p_last = qk1(NPAIR - 1, bias[0])
    for i in range(NWO): cp_wo(i).wait()
    oa = wo_part(0, NPAIR - 1, True)
    pv1(NPAIR - 1, p_last)
    oa = oa + wo_part(NPAIR - 1, NPAIR, True)
    xn = x_ref[SEG:2 * SEG, :].astype(f32)
    xan_ref[0:SEG, :] = xn
    xan_ref[SEG:2 * SEG, :] = jnp.zeros((SEG, D), f32)
    h_ref[8:24, :] = _pk(_ln(xn))
    end_step(0, oa, 0)

    def phase(ph, c):
        jax.lax.fori_loop(jnp.where(ph == 0, 1, NSEG), jnp.where(ph == 0, 2, NSEG + 2), make_step('half'), 0)

        @pl.when(ph == 0)
        def _():
            cp_x1.wait()
            jax.lax.fori_loop(2, NPRE + 2, make_step('pre'), 0)
            jax.lax.fori_loop(NPRE + 2, NSEG, make_step('full'), 0)
        return c

    jax.lax.fori_loop(0, 2, phase, 0)

    b_qkv((1,))
    for c in range(2): b_attn(NSEG + 2, 1, 16 * c, 16)
    b2_finish(NSEG + 2)
    cp_out(NSEG - 1).start()

    pltpu.make_async_copy(out_ref, out_hbm, sem_o.at[0]).wait()


@functools.partial(jax.jit, static_argnames=("A_seg_len",))
def pallas_interleave_layers__memory_aug_recurrent_mem_tr__sliding_local_dilated__prompt_kernel(
        A_x, A_mem0, A_Wq, A_Wk, A_Wv, A_Wo, A_seg_len, B_x, B_wqkv, B_wo):
    assert A_seg_len == SEG
    del B_x
    x = A_x.reshape(S, D)
    mem0 = A_mem0.reshape(M, D)
    tr = lambda w: jnp.transpose(w, (1, 2, 0)).reshape(H * DH, D)
    wo = A_Wo.reshape(H * DH, D)
    hbm = pl.BlockSpec(memory_space=pl.ANY)
    WR = H * DH // 2
    vmem = pltpu.VMEM
    out = pl.pallas_call(
        kernel,
        out_shape=jax.ShapeDtypeStruct((S, D), bf16),
        in_specs=[hbm] * 8,
        out_specs=hbm,
        scratch_shapes=[
            vmem((WR, D), u32), vmem((WR, D), u32), vmem((WR, D), u32),
            vmem((NPAIR, 3, D // 2, PW), u32), vmem((WR, D), u32),
            vmem((D // 2 + 8, 3 * D), u32), vmem((5, D, 128), u32),
            vmem((D // 2 + 8, 3 * D), u32), vmem((D // 2 + 32, D), u32),
            vmem((S, D), bf16), vmem((M, D), bf16), vmem((S, D), bf16),
            vmem((40, D), u32), vmem((32, D), u32), vmem((24 + 16 * NPRE, D), u32),
            vmem((64, D), f32), vmem((64, D), f32), vmem((64, D), f32),
            vmem((NPAIR, 3, 40, PW), u32), vmem((NPAIR, 3, 16 * NPRE, PW), u32),
            vmem((NPAIR, 40, PW), u32),
            vmem((64, D), f32), vmem((2, 48, D), f32), vmem((2, 48, D), f32), vmem((64, D), f32),
            pltpu.SemaphoreType.DMA((NPAIR + 3,)), pltpu.SemaphoreType.DMA((7,)),
            pltpu.SemaphoreType.DMA((8,)), pltpu.SemaphoreType.DMA((1,)),
        ],
        compiler_params=pltpu.CompilerParams(vmem_limit_bytes=100 * 1024 * 1024),
    )(x, mem0, tr(A_Wq), tr(A_Wk), tr(A_Wv), wo, B_wqkv, B_wo)
    return out.reshape(1, S, D)
```

```python
import functools
import jax
import jax.numpy as jnp
from jax.experimental import pallas as pl
from jax.experimental.pallas import tpu as pltpu

S = 2048; D = 640; H = 32; DH = 192; M = 8; SEG = 32; NSEG = S // SEG
NPAIR = H // 2; PW = 2 * DH
BH = 32; BDH = D // BH; BW = 8; BDIL = 2
LOG2E = 1.4426950408889634
NEG = -1e30
f32 = jnp.float32; bf16 = jnp.bfloat16; u32 = jnp.uint32; i32 = jnp.int32
NPRE = 9


def _sched(bq, b1, bh, hc, cuts, wpos, b2):
    s = {}
    s.setdefault(bq, []).append('bqkv')
    s.setdefault((b1, 'post'), []).append('b1fin')
    s.setdefault((bh, 'post'), []).append('bhist')
    s.setdefault((hc, 'post'), []).append('hcopy')
    cs = [0] + list(cuts) + [NPAIR]
    for (g0, g1), p in zip(zip(cs, cs[1:]), wpos):
        s.setdefault(p, []).append(('wo', g0, g1))
    s.setdefault(b2, []).append('b2fin')
    return s


def _bdep(l0, l1):
    d = {}
    for i, g in enumerate(l0): d.setdefault(g, []).append((0, 8 * i, 8))
    for i, g in enumerate(l1): d.setdefault(g, []).append((1, 8 * i, 8))
    return d


_WP = ((13, 'post'), (14, 'k'), (14, 'post'), (15, 'post'))
SCHED = {
    'half': _sched((0, 'pre'), 8, 11, 13, (4, 8, 13), _WP, (15, 'post')),
    'pre': _sched((0, 'post'), 8, 11, 13, (4, 8, 13), _WP, (15, 'post')),
    'full': _sched((0, 'post'), 8, 12, 13, (4, 8, 13), _WP, (15, 'post')),
}
BDEP = {
    'half': _bdep((3, 4, 5, 7), (9, 10, 11, 11)),
    'pre': _bdep((3, 5, 7, 8), (9, 10, 11, 11)),
    'full': _bdep((3, 4, 5, 7), (9, 10, 11, 12)),
}


def _dot(a, b):
    return jnp.dot(a, b, preferred_element_type=f32)


def _dot_nt(a, b):
    return jax.lax.dot_general(a, b, (((1,), (1,)), ((), ())), preferred_element_type=f32)


def _recip(x):
    r = pl.reciprocal(x, approx=True)
    return r * (2.0 - x * r)


def _ln(x):
    m = jnp.mean(x, axis=-1, keepdims=True)
    xc = x - m
    v = jnp.mean(xc * xc, axis=-1, keepdims=True)
    return xc * jax.lax.rsqrt(v + 1e-5)


def _pk(x):
    return pltpu.bitcast(x.astype(bf16), u32)


def _up(x):
    return pltpu.bitcast(x, bf16)


def _ds(start, size, mult):
    return pl.ds(start, size) if isinstance(start, int) else pl.ds(pl.multiple_of(start, mult), size)


def kernel(x_hbm, mem0_hbm, wq_hbm, wk_hbm, wv_hbm, wo_hbm, bqkv_hbm, bwo_hbm, out_hbm,
           wq, wk, wv, wn_ref, wo, bqkv_raw, bwo_raw, bqkv_p, bwo_p, x_ref, mem0_ref, out_ref,
           h_ref, hn_ref, hp_ref, xa_ref, xan_ref, xb_ref, qkv_ref, pre_ref, o_ref,
           bq_ref, kb_ref, vb_ref, bo_ref,
           sem_w, sem_m, sem_b, sem_o):
    RW = PW // 2
    ws = (wq, wk, wv)
    ws_hbm = (wq_hbm.bitcast(u32), wk_hbm.bitcast(u32), wv_hbm.bitcast(u32))
    NWO = 4
    RO = H * DH // 2 // NWO
    X0R = (NPRE + 2) * SEG
    BQR = (0, 104, 208, 320)

    def cp_w(j, g):
        sl = _ds(g * RW, RW, RW)
        sem = sem_w.at[NPAIR + j] if (isinstance(g, int) and g == 0) else sem_w.at[g]
        return pltpu.make_async_copy(ws_hbm[j].at[sl], ws[j].at[sl], sem)

    def cp_wo(i):
        sl = pl.ds(i * RO, RO)
        return pltpu.make_async_copy(wo_hbm.bitcast(u32).at[sl], wo.at[sl], sem_m.at[3 + i])

    def cp_out(s):
        sl = _ds(s * SEG, SEG, SEG)
        return pltpu.make_async_copy(out_ref.at[sl], out_hbm.at[sl], sem_o.at[0])

    cp_x0 = pltpu.make_async_copy(x_hbm.at[0:X0R], x_ref.at[0:X0R], sem_m.at[0])
    cp_mem = pltpu.make_async_copy(mem0_hbm, mem0_ref, sem_m.at[1])
    cp_x1 = pltpu.make_async_copy(x_hbm.at[X0R:S], x_ref.at[X0R:S], sem_m.at[2])
    cp_bqkv = [pltpu.make_async_copy(bqkv_hbm.bitcast(u32).at[BQR[i]:BQR[i + 1]], bqkv_raw.at[BQR[i]:BQR[i + 1]],
                                     sem_b.at[i]) for i in range(3)]
    cp_bwo = [pltpu.make_async_copy(bwo_hbm.bitcast(u32).at[:, k * 128:(k + 1) * 128], bwo_raw.at[k, 0:D // 2, :],
                                    sem_b.at[3 + k]) for k in range(5)]

    cp_x0.start(); cp_mem.start()
    for g in range(NPAIR):
        if g == 3: cp_bqkv[0].start()
        if g == 5:
            for c in cp_bwo: c.start()
        if g == 6: cp_bqkv[1].start()
        if g == 9: cp_bqkv[2].start()
        for j in range(3): cp_w(j, g).start()
    for i in range(NWO): cp_wo(i).start()

    bqkv_raw[D // 2:D // 2 + 8, :] = jnp.zeros((8, 3 * D), u32)
    for k in range(5): bwo_raw[k, D // 2:D, :] = jnp.zeros((D // 2, 128), u32)
    xb_ref[...] = jnp.zeros((2 * SEG, D), f32)
    kb_ref[...] = jnp.zeros(kb_ref.shape, f32)
    vb_ref[...] = jnp.zeros(vb_ref.shape, f32)
    xa_ref[SEG:2 * SEG, :] = jnp.zeros((SEG, D), f32)
    h_ref[24:40, :] = jnp.zeros((16, D), u32)
    cp_x0.wait(); cp_mem.wait()
    mem0 = mem0_ref[...].astype(f32)
    mem00 = jnp.concatenate([mem0, mem0], axis=0)
    x00 = x_ref[0:SEG, :].astype(f32)
    xa_ref[0:SEG, :] = x00
    hp_ref[0:8, :] = _pk(mem00)
    hp_ref[8:24, :] = _pk(_ln(x00))
    for i in range(NPRE):
        hp_ref[24 + 16 * i:40 + 16 * i, :] = _pk(_ln(x_ref[(i + 2) * SEG:(i + 3) * SEG, :].astype(f32)))

    def perm_wo_unit(e, valid):
        base = jnp.where(valid, e, D // 2)
        w = jnp.concatenate([bwo_raw[k, pl.ds(base, BH, stride=BDH // 2), :] for k in range(5)], axis=1)
        dst = pl.multiple_of(jnp.where(valid, e * BH, D // 2), BH)
        bwo_p[pl.ds(dst, BH // 2), :] = _pk(pltpu.bitcast(w << 16, f32))
        bwo_p[pl.ds(dst + BH // 2, BH // 2), :] = _pk(pltpu.bitcast(w & jnp.uint32(0xFFFF0000), f32))

    lane8 = jax.lax.broadcasted_iota(i32, (8, 128), 1)

    def perm_unit(u, valid):
        rg = u // 3
        j = u - 3 * rg
        r = pl.ds(pl.multiple_of(jnp.where(valid, rg * 8, D // 2), 8), 8)
        srcs = [bqkv_raw[r, pl.ds(pl.multiple_of(j * D + k * 128, 128), 128)] for k in range(5)]
        for n in range(5):
            col = lane8 + n * 128
            s = (col % BH) * BDH + col // BH
            acc = None
            for k in range(5):
                gk = jnp.take_along_axis(srcs[k], s % 128, axis=1)
                acc = gk if acc is None else jnp.where(s // 128 == k, gk, acc)
            bqkv_p[r, pl.ds(pl.multiple_of(j * D + n * 128, 128), 128)] = acc

    def lhs_h(var, lh):
        if var == 'full':
            return _up(h_ref[...])
        if var == 'pre':
            return _up(jnp.concatenate([h_ref[0:8, :], h_ref[24:40, :]], axis=0))
        return _up(jnp.concatenate([h_ref[0:8, :], h_ref[pl.ds(pl.multiple_of(8 + 16 * lh, 8), 16), :]], axis=0))

    def proj(g, j, var, lh):
        y = _pk(_dot(lhs_h(var, lh), _up(wn_ref[g, j])))
        if var == 'full':
            qkv_ref[g, j] = y
        elif var == 'pre':
            qkv_ref[g, j, 0:8, :] = y[0:8]
            qkv_ref[g, j, 24:40, :] = y[8:24]
        else:
            qkv_ref[g, j, 0:24, :] = y

    lo64 = jax.lax.broadcasted_iota(i32, (48, 128), 1) < 64
    rr = jax.lax.broadcasted_iota(i32, (48, 96), 0)
    cc = jax.lax.broadcasted_iota(i32, (48, 96), 1)
    ck = jnp.where(cc >= 48, cc - 48, cc)
    row16 = jax.lax.broadcasted_iota(i32, (16, 128), 0)
    row96 = jax.lax.broadcasted_iota(i32, (16, 96), 0)
    sc = (DH ** -0.5) * LOG2E

    def smask(l):
        memk = (ck >= 8 * l) & (ck < 8 * l + 8)
        tokk = (ck >= 16) & ((rr < 16) | (ck <= rr))
        return jnp.where(memk | tokk, 0.0, NEG).astype(f32)

    bias = [smask(0), smask(1)]
    h0c = [cc < 48, (cc < 16) | (cc >= 64)]

    def softmax2(s, bias_l, hc):
        s = s * sc + bias_l
        m0 = jnp.max(jnp.where(hc, s, NEG), axis=1, keepdims=True)
        m1 = jnp.max(jnp.where(hc, NEG, s), axis=1, keepdims=True)
        p = jnp.exp2(s - jnp.where(hc, m0, m1))
        s0 = jnp.sum(jnp.where(hc, p, 0.0), axis=1, keepdims=True)
        s1 = jnp.sum(jnp.where(hc, 0.0, p), axis=1, keepdims=True)
        return p * _recip(jnp.where(hc, s0, s1))

    def lo_(a): return jnp.where(lo64[0:a.shape[0]], a, jnp.zeros_like(a))
    def hi_(a): return jnp.where(lo64[0:a.shape[0]], jnp.zeros_like(a), a)

    def bd1(g, j):
        a = _up(qkv_ref[g, j, 0:24, :])
        z = jnp.zeros((48, 128), bf16)
        a1 = a[:, 128:256]
        top = jnp.concatenate([a[:, 0:128], lo_(a1), z], axis=1)
        bot = jnp.concatenate([z, hi_(a1), a[:, 256:384]], axis=1)
        return jnp.concatenate([top, bot], axis=0)

    def qk1(g, bias_l):
        return softmax2(_dot_nt(_up(qkv_ref[g, 0, 0:24, :]), bd1(g, 1)), bias_l, h0c[0])

    def pv1(g, p, vb=None):
        vb = bd1(g, 2) if vb is None else vb
        o_ref[g, 0:24, :] = _pk(_dot(p.astype(bf16), vb))

    def parts(j, g, pre):
        m_ = _up(qkv_ref[g, j, 0:8, :])
        t1 = _up(qkv_ref[g, j, 8:24, :] if pre is None else pre_ref[g, j, pl.ds(pl.multiple_of(16 * pre, 16), 16), :])
        return m_, t1, _up(qkv_ref[g, j, 24:40, :])

    def rhs3(j, g, pre):
        m_, t1, t2 = parts(j, g, pre)
        z16 = jnp.zeros((16, 128), bf16)
        cat = lambda *xs: jnp.concatenate(xs, axis=0)
        r0 = cat(m_[:, 0:128], t1[:, 0:128], z16, t2[:, 0:128])
        r2 = cat(z16, t2[:, 256:384], m_[:, 256:384], t1[:, 256:384])
        m1, a1, b1 = m_[:, 128:256], t1[:, 128:256], t2[:, 128:256]
        rt0 = cat(lo_(m1), lo_(a1), hi_(m1), hi_(a1))
        rt1 = cat(lo_(m1), hi_(b1), hi_(m1), lo_(b1))
        return r0, r2, rt0, rt1

    def qk2(g, pre):
        q = jnp.concatenate(parts(0, g, pre), axis=0)
        r0, r2, rt0, rt1 = rhs3(1, g, pre)
        a0 = _dot_nt(q[:, 0:128], r0)
        a2 = _dot_nt(q[:, 256:384], r2)
        q1 = jnp.concatenate([q[0:16, 128:256], q[48:80, 128:256]], axis=0)
        s0 = jnp.where(h0c[0], a0[0:48], a2[0:48]) + _dot_nt(q[0:48, 128:256], rt0)
        a0l = jnp.concatenate([a0[0:16], a0[48:80]], axis=0)
        a2l = jnp.concatenate([a2[0:16], a2[48:80]], axis=0)
        s1 = jnp.where(h0c[1], a0l, a2l) + _dot_nt(q1, rt1)
        return [softmax2(s0, bias[0], h0c[0]), softmax2(s1, bias[1], h0c[1])]

    def pv2(g, ps, pre):
        p0, p1 = ps
        r0, r2, rt0, rt1 = rhs3(2, g, pre)

        def stack(x0, x1):
            mm = jnp.where(row96 < 8, x0[0:16], x1[0:16])
            return jnp.concatenate([mm, x0[16:48], x1[16:48]], axis=0).astype(bf16)

        o0 = _dot(stack(jnp.where(h0c[0], p0, 0.0), jnp.where(h0c[1], p1, 0.0)), r0)
        o2 = _dot(stack(jnp.where(h0c[0], 0.0, p0), jnp.where(h0c[1], 0.0, p1)), r2)
        t0 = _dot(p0.astype(bf16), rt0)
        t1 = _dot(p1.astype(bf16), rt1)
        om = jnp.where(row16 < 8, t0[0:16], t1[0:16])
        o1 = jnp.concatenate([om, t0[16:48], t1[16:48]], axis=0)
        o_ref[g] = _pk(jnp.concatenate([o0, o1, o2], axis=1))

    def wo_part(g0, g1, half):
        o = jnp.concatenate([_up(o_ref[g, 0:24, :] if half else o_ref[g]) for g in range(g0, g1)], axis=1)
        return _dot(o, _up(wo[g0 * RW:g1 * RW, :]))

    rC = jax.lax.broadcasted_iota(i32, (16, 128), 0)
    bsc = (BDH ** -0.5) * LOG2E

    def b_qkv(layers=(0, 1)):
        r0 = SEG * layers[0]; r1 = SEG * layers[-1] + SEG
        y = _dot(_ln(xb_ref[r0:r1, :]).astype(bf16), _up(bqkv_p[0:D // 2, :]))
        bq_ref[r0:r1, :] = y[:, 0:D]
        for l in layers:
            kb_ref[l, 16:48, :] = y[SEG * l - r0:SEG * l - r0 + SEG, D:2 * D]
            vb_ref[l, 16:48, :] = y[SEG * l - r0:SEG * l - r0 + SEG, 2 * D:3 * D]

    def b_attn(t, l, r0, nr):
        q = bq_ref[SEG * l + r0:SEG * l + r0 + nr, :]
        pos = (t - 1 - 2 * l) * SEG + r0 + rC[0:nr]
        lg = []
        for w in range(BW):
            off = 16 - BDIL * w + r0
            pr = q * kb_ref[l, off:off + nr, :]
            a = pr[:, 0:128] + pr[:, 128:256] + pr[:, 256:384] + pr[:, 384:512] + pr[:, 512:640]
            a = a + pltpu.roll(a, 64, 1)
            a = (a + pltpu.roll(a, 32, 1)) * bsc
            lg.append(a if w == 0 else jnp.where(pos >= BDIL * w, a, NEG))
        m = lg[0]
        for w in range(1, BW): m = jnp.maximum(m, lg[w])
        ps = [jnp.exp2(a - m) for a in lg]
        den = ps[0]
        for w in range(1, BW): den = den + ps[w]
        inv = _recip(den)
        acc = None
        for w in range(BW):
            off = 16 - BDIL * w + r0
            tt = jnp.concatenate([ps[w] * inv] * 5, axis=1) * vb_ref[l, off:off + nr, :]
            acc = tt if acc is None else acc + tt
        bo_ref[SEG * l + r0:SEG * l + r0 + nr, :] = acc
        z = acc[0:8, 0:128]
        for a_ in range(nr // 8):
            for b_ in range(5):
                if a_ or b_: z = jnp.maximum(z, acc[8 * a_:8 * a_ + 8, 128 * b_:128 * b_ + 128])
        return z

    def b_hist():
        for l in range(2):
            kb_ref[l, 0:16, :] = kb_ref[l, 32:48, :]
            vb_ref[l, 0:16, :] = vb_ref[l, 32:48, :]

    def b_out(l):
        a = bo_ref[SEG * l:SEG * l + SEG, :].astype(bf16)
        if l == 0:
            return xb_ref[SEG * l:SEG * l + SEG, :] + _dot(a, _up(bwo_p[0:D // 2, :]))
        acc = xb_ref[SEG * l:SEG * l + SEG, :] + _dot(a[:, 0:512], _up(bwo_p[0:256, :]))
        return acc + _dot(a[:, 512:D], _up(bwo_p[256:D // 2, :]))

    def b1_finish(t):
        x2 = b_out(0)
        xn = x_ref[_ds(jnp.minimum(t + 1, NSEG - 1) * SEG, SEG, SEG), :].astype(f32)
        xan_ref[0:SEG, :] = xn
        xan_ref[SEG:2 * SEG, :] = x2
        hn_ref[0:16, :] = _pk(_ln(xn))
        hn_ref[16:32, :] = _pk(_ln(x2))

    def b2_finish(t):
        out_ref[_ds(jnp.maximum(t - 3, 0) * SEG, SEG, SEG), :] = b_out(1).astype(bf16)

    def end_step(t, oa, lh):
        if lh is None:
            xb_ref[...] = xa_ref[...] + oa[16:80]
        else:
            sl = _ds(SEG * lh, SEG, SEG)
            xb_ref[sl, :] = xa_ref[sl, :] + oa[16:48]
        xa_ref[...] = xan_ref[...]
        r16 = jax.lax.broadcasted_iota(i32, (16, D), 0)
        h_ref[0:8, :] = _pk(jnp.where((r16 >= 8) & (t < 2), mem00, oa[0:16]))

    def step_body(t, var):
        half = var == 'half'
        lh = jnp.where(t < 2, 0, 1) if half else None
        bias_h = smask(lh) if half else None
        pre = jnp.clip(t - 2, 0, NPRE - 1) if var == 'pre' else None
        st = {}
        pp = {}

        def extra(i, pos):
            for name in SCHED[var].get((i, pos), ()):
                if name == 'bqkv': b_qkv()
                elif name == 'bhist': b_hist()
                elif name == 'hcopy': h_ref[8:40, :] = hn_ref[...]
                elif name == 'b1fin': b1_finish(t)
                elif name == 'b2fin': b2_finish(t)
                else:
                    part = wo_part(name[1], name[2], half)
                    st['oa'] = part if 'oa' not in st else st['oa'] + part

        for i in range(-2, NPAIR):
            g2, g1, g0 = i + 2, i + 1, i
            extra(i, 'pre')
            for j in range(3):
                if g2 < NPAIR: proj(g2, j, var, lh)
                extra(i, 'qkv'[j])
            if 0 <= g1 < NPAIR:
                pp[g1] = [qk1(g1, bias_h)] if half else qk2(g1, pre)
            if 0 <= g0:
                pg = pp.pop(g0)
                for (l, r0, nr) in BDEP[var].get(g0, ()):
                    z = b_attn(t, l, r0, nr)
                    pg[0] = jnp.concatenate([jnp.where(t < 0, z[:, 0:96], pg[0][0:8]), pg[0][8:]], axis=0)
                if half: pv1(g0, pg[0])
                else: pv2(g0, pg, pre)
            extra(i, 'post')
        end_step(t, st['oa'], lh)

    def make_step(var):
        def step(t, c):
            step_body(t, var)
            @pl.when(t >= 3)
            def _():
                cp_out(jnp.maximum(t - 3, 0)).start()
            return c
        return step

    def warm(g, c, first=False):
        sl = _ds(g * RW, RW, RW)

        def wproj(j):
            y = _pk(_dot_nt(_up(hp_ref[...]), _up(ws[j][sl, :])))
            qkv_ref[g, j, 0:24, :] = y[0:24]
            pre_ref[g, j] = y[24:]

        if first:
            for j in range(3):
                cp_w(j, g).wait()
                wproj(j)
        else:
            for i, g_ in enumerate((3, 6, 10)):
                pl.when(g == g_)(cp_bqkv[i].wait)

            @pl.when(g == 6)
            def _():
                for c_ in cp_bwo: c_.wait()

            for j in range(3): cp_w(j, g).wait()
            vb = bd1(g - 1, 2)
            p = qk1(g - 1, bias[0])
            wproj(0); wproj(1)
            pv1(g - 1, p, vb)
            wproj(2)
        for j in range(3):
            wn_ref[g, j] = _pk(_up(ws[j][sl, :]).T)
        if not first:
            for k in range(10): perm_unit(jnp.clip(10 * (g - 3) + k, 0, 119), g >= 3)
            perm_wo_unit(jnp.clip(g - 6, 0, 9), g >= 6)
        return c

    warm(0, 0, first=True)
    jax.lax.fori_loop(1, NPAIR, warm, 0)
    p_last = qk1(NPAIR - 1, bias[0])
    for i in range(NWO): cp_wo(i).wait()
    cp_x1.start()
    oa = wo_part(0, NPAIR - 1, True)
    pv1(NPAIR - 1, p_last)
    oa = oa + wo_part(NPAIR - 1, NPAIR, True)
    xn = x_ref[SEG:2 * SEG, :].astype(f32)
    xan_ref[0:SEG, :] = xn
    xan_ref[SEG:2 * SEG, :] = jnp.zeros((SEG, D), f32)
    h_ref[8:24, :] = _pk(_ln(xn))
    end_step(0, oa, 0)

    def phase(ph, c):
        jax.lax.fori_loop(jnp.where(ph == 0, 1, NSEG), jnp.where(ph == 0, 2, NSEG + 2), make_step('half'), 0)

        @pl.when(ph == 0)
        def _():
            cp_x1.wait()
            jax.lax.fori_loop(2, NPRE + 2, make_step('pre'), 0)
            jax.lax.fori_loop(NPRE + 2, NSEG, make_step('full'), 0)
        return c

    jax.lax.fori_loop(0, 2, phase, 0)

    b_qkv((1,))
    for c in range(2): b_attn(NSEG + 2, 1, 16 * c, 16)
    b2_finish(NSEG + 2)
    cp_out(NSEG - 1).start()

    pltpu.make_async_copy(out_ref, out_hbm, sem_o.at[0]).wait()


@functools.partial(jax.jit, static_argnames=("A_seg_len",))
def pallas_interleave_layers__memory_aug_recurrent_mem_tr__sliding_local_dilated__prompt_kernel(
        A_x, A_mem0, A_Wq, A_Wk, A_Wv, A_Wo, A_seg_len, B_x, B_wqkv, B_wo):
    assert A_seg_len == SEG
    del B_x
    x = A_x.reshape(S, D)
    mem0 = A_mem0.reshape(M, D)
    tr = lambda w: jnp.transpose(w, (1, 2, 0)).reshape(H * DH, D)
    wo = A_Wo.reshape(H * DH, D)
    hbm = pl.BlockSpec(memory_space=pl.ANY)
    WR = H * DH // 2
    vmem = pltpu.VMEM
    out = pl.pallas_call(
        kernel,
        out_shape=jax.ShapeDtypeStruct((S, D), bf16),
        in_specs=[hbm] * 8,
        out_specs=hbm,
        scratch_shapes=[
            vmem((WR, D), u32), vmem((WR, D), u32), vmem((WR, D), u32),
            vmem((NPAIR, 3, D // 2, PW), u32), vmem((WR, D), u32),
            vmem((D // 2 + 8, 3 * D), u32), vmem((5, D, 128), u32),
            vmem((D // 2 + 8, 3 * D), u32), vmem((D // 2 + 32, D), u32),
            vmem((S, D), bf16), vmem((M, D), bf16), vmem((S, D), bf16),
            vmem((40, D), u32), vmem((32, D), u32), vmem((24 + 16 * NPRE, D), u32),
            vmem((64, D), f32), vmem((64, D), f32), vmem((64, D), f32),
            vmem((NPAIR, 3, 40, PW), u32), vmem((NPAIR, 3, 16 * NPRE, PW), u32),
            vmem((NPAIR, 40, PW), u32),
            vmem((64, D), f32), vmem((2, 48, D), f32), vmem((2, 48, D), f32), vmem((64, D), f32),
            pltpu.SemaphoreType.DMA((NPAIR + 3,)), pltpu.SemaphoreType.DMA((7,)),
            pltpu.SemaphoreType.DMA((8,)), pltpu.SemaphoreType.DMA((1,)),
        ],
        compiler_params=pltpu.CompilerParams(vmem_limit_bytes=100 * 1024 * 1024),
    )(x, mem0, tr(A_Wq), tr(A_Wk), tr(A_Wv), wo, B_wqkv, B_wo)
    return out.reshape(1, S, D)
```
